```python
import jax
import jax.numpy as jnp

def _softmax(x, axis=-1):
    return jax.nn.softmax(x, axis=axis)
def _gelu(x):
    return jax.nn.gelu(x, approximate=True)
def _silu(x):
    return jax.nn.silu(x)
def _sigmoid(x):
    return jax.nn.sigmoid(x)
def _layernorm(x, axis=-1, eps=1e-5):
    m = jnp.mean(x, axis=axis, keepdims=True)
    v = jnp.var(x, axis=axis, keepdims=True)
    return (x - m) / jnp.sqrt(v + eps)
def _scatter_add(tgt, idx, src, axis=0):
    return tgt.at[idx].add(src)
def _segment_sum(src, seg, n):
    return jax.ops.segment_sum(src, seg, n)
class _Rng:
    def __init__(self, key):
        self._k = key
    def _next(self):
        self._k, sub = jax.random.split(self._k)
        return sub
    def normal(self, shape):
        return jax.random.normal(self._next(), shape, dtype=jnp.bfloat16)
    def randint(self, lo, hi, shape):
        return jax.random.randint(self._next(), shape, lo, hi, dtype=jnp.int32)
    def uniform(self, shape, lo=0.0, hi=1.0):
        return jax.random.uniform(self._next(), shape, jnp.bfloat16, lo, hi)
    def permutation(self, n):
        return jax.random.permutation(self._next(), n)


kernel_name = 'interleave_layers__sliding_block_cached__moe_arch_mod__decode'

def setup_inputs():
    _rng = _Rng(jax.random.key(int.from_bytes(__import__("os").urandom(4), "little")))
    _w = (lambda a: (lambda t: t.astype(jnp.bfloat16) if jnp.issubdtype(t.dtype, jnp.floating) else t)(jnp.asarray(a)))
    def _A_setup():
        B, Sq, D = 4, 1, 640
        Hq, Hkv, Sk, Dh = 32, 32, 4096, 192
        assert Hq % Hkv == 0, (Hq, Hkv)
        return {
            "x": _w((lambda *s: _rng.normal(s) * 0.05)(B, Sq, D)),
            "k_cache": _w((lambda *s: _rng.normal(s) * 0.05)(B, Hkv, Sk, Dh)),
            "v_cache": _w((lambda *s: _rng.normal(s) * 0.05)(B, Hkv, Sk, Dh)),
            "wq": _w((lambda *s: _rng.normal(s) * 0.05)(D, Hq * Dh) * (D ** -0.5)),
            "wo": _w((lambda *s: _rng.normal(s) * 0.05)(Hq * Dh, D) * ((Hq * Dh) ** -0.5)),
        }
    _A_in = _A_setup()

    def _B_setup():
        B, S, D, F, C = 4, 1, 640, 1536, 1
        return {
            "x": _w((lambda *s: _rng.normal(s) * 0.05)(B, S, D)),
            "w_r": _w((lambda *s: _rng.normal(s) * 0.05)(D)),
            "w_gate": _w((lambda *s: _rng.normal(s) * 0.05)(D, F)),
            "w_up": _w((lambda *s: _rng.normal(s) * 0.05)(D, F)),
            "w_down": _w((lambda *s: _rng.normal(s) * 0.05)(F, D)),
        }
    _B_in = _B_setup()

    return {
        "A_x": _A_in["x"],
        "A_k_cache": _A_in["k_cache"],
        "A_v_cache": _A_in["v_cache"],
        "A_wq": _A_in["wq"],
        "A_wo": _A_in["wo"],
        "B_x": _B_in["x"],
        "B_w_r": _B_in["w_r"],
        "B_w_gate": _B_in["w_gate"],
        "B_w_up": _B_in["w_up"],
        "B_w_down": _B_in["w_down"],
    }

def reference(A_x, A_k_cache, A_v_cache, A_wq, A_wo, B_x, B_w_r, B_w_gate, B_w_up, B_w_down):
    def _A_ref(x, k_cache, v_cache, wq, wo):
        B, Sq, D = x.shape
        Hq, Dh = 32, 192
        Hkv, Sk = k_cache.shape[1], k_cache.shape[2]
        W = min(4096, max(256, Sk // 4))
        rep = Hq // Hkv
        q = (lambda x, *d: x.transpose(*d))((x @ wq).reshape(B, Sq, Hq, Dh), 0, 2, 1, 3)
        k = jnp.repeat(k_cache[:, :, Sk - W:, :], rep, axis=1)
        v = jnp.repeat(v_cache[:, :, Sk - W:, :], rep, axis=1)
        scores = jnp.einsum("bhqd,bhkd->bhqk", q, k) * (Dh ** -0.5)
        p = _softmax(scores, axis=-1)
        o = jnp.einsum("bhqk,bhkd->bhqd", p, v)
        return (lambda x, *d: x.transpose(*d))(o, 0, 2, 1, 3).reshape(B, Sq, Hq * Dh) @ wo

    def _B_ref(x, w_r, w_gate, w_up, w_down):
        B, S, D = x.shape
        C = 1
        r = x @ w_r
        idx = jnp.argsort(-r, axis=-1)[:, :C]
        idx_e = jnp.repeat(idx.reshape(B, C, 1), D, axis=2)
        x_sel = jnp.take_along_axis(x, idx_e, axis=1)
        g = _silu(x_sel @ w_gate)
        u = x_sel @ w_up
        y = (g * u) @ w_down
        r_sel = _sigmoid(jnp.take_along_axis(r, idx, axis=1))
        y = y * r_sel.reshape(B, C, 1)
        b_off = (jnp.arange(B) * S).reshape(B, 1)
        flat_idx = (idx + b_off).reshape(B * C)
        zero = (x * 0.0).reshape(B * S, D)
        upd = _scatter_add(zero, flat_idx, y.reshape(B * C, D), axis=0)
        return x + upd.reshape(B, S, D)

    x = A_x
    x = x + _A_ref(_layernorm(x, axis=-1), A_k_cache, A_v_cache, A_wq, A_wo)
    x = x + _B_ref(_layernorm(x, axis=-1), B_w_r, B_w_gate, B_w_up, B_w_down)
    x = x + _A_ref(_layernorm(x, axis=-1), A_k_cache, A_v_cache, A_wq, A_wo)
    x = x + _B_ref(_layernorm(x, axis=-1), B_w_r, B_w_gate, B_w_up, B_w_down)
    return x
```

```python
import functools

import jax
import jax.numpy as jnp
from jax import lax
import jax.experimental.pallas as pl
import jax.experimental.pallas.tpu as pltpu

B, D = 4, 640
H, DH, SK = 32, 192, 4096
W = 1024
F = 1536
NJ = W // 128
HG = 8
NG = H // HG
GR = HG * DH
LN_EPS = 1e-5
SCALE = DH ** -0.5
F32 = jnp.float32
BF16 = jnp.bfloat16


def _layernorm(x):
    m = jnp.mean(x, axis=-1, keepdims=True)
    c = x - m
    v = jnp.mean(c * c, axis=-1, keepdims=True)
    return c * lax.rsqrt(v + LN_EPS)


def _dot(a, b):
    return jnp.dot(a, b, preferred_element_type=F32)


def _dot_nt(a, b):
    return lax.dot_general(a, b, (((1,), (1,)), ((), ())), preferred_element_type=F32)


def _kernel(x_hbm, k_hbm, v_hbm, wq_hbm, wo_hbm, wr_hbm, wg_hbm, wu_hbm, wd_hbm,
            o_ref,
            x_in, wr_in, wq_s, wo_s, wg_s, wu_s, wd_s, kbuf, vbuf,
            x_s, q1_s, p_s, out_s,
            sems):
    sem_small = sems.at[pl.ds(0, 2)]
    sem_w = sems.at[pl.ds(2, 5)]
    sem_k = sems.at[pl.ds(8, 2 * NG)]
    sem_v = sems.at[pl.ds(8 + 2 * NG, 2 * NG)]

    def w_copies(src, dst, sem):
        return [pltpu.make_async_copy(src.at[:, pl.ds(j * 128, 128)], dst.at[j], sem)
                for j in range(dst.shape[0])]

    def kv_copy(src, dst, sem, b, slot, g, j):
        rows = pl.ds(g * GR, GR)
        return pltpu.make_async_copy(
            src.at[b, rows, pl.ds(SK - W + j * 128, 128)], dst.at[slot, j, rows], sem.at[slot * NG + g])

    def start_kv(src, dst, sem, b, slot):
        for g in range(NG):
            for j in range(NJ):
                kv_copy(src, dst, sem, b, slot, g, j).start()

    def wait_kv(src, dst, sem, b, slot, g):
        for j in range(NJ):
            kv_copy(src, dst, sem, b, slot, g, j).wait()

    x_cp = pltpu.make_async_copy(x_hbm, x_in, sem_small.at[0])
    wr_cp = pltpu.make_async_copy(wr_hbm, wr_in, sem_small.at[1])
    wq_cp = w_copies(wq_hbm, wq_s, sem_w.at[0])
    wo_cp = w_copies(wo_hbm, wo_s, sem_w.at[1])
    wg_cp = w_copies(wg_hbm, wg_s, sem_w.at[2])
    wu_cp = w_copies(wu_hbm, wu_s, sem_w.at[3])
    wd_cp = w_copies(wd_hbm, wd_s, sem_w.at[4])

    x_cp.start()
    wr_cp.start()
    for c in wq_cp:
        c.start()
    start_kv(k_hbm, kbuf, sem_k, 0, 0)
    for c in wo_cp:
        c.start()
    start_kv(v_hbm, vbuf, sem_v, 0, 0)
    for c in wg_cp + wu_cp + wd_cp:
        c.start()
    start_kv(k_hbm, kbuf, sem_k, 1, 1)
    start_kv(v_hbm, vbuf, sem_v, 1, 1)

    row = lax.broadcasted_iota(jnp.int32, (HG, GR), 0)
    col = lax.broadcasted_iota(jnp.int32, (HG, GR), 1)
    diag = (col >= row * DH) & (col < (row + 1) * DH)

    def proj(a, w_s, rows=None):
        if rows is None:
            return jnp.concatenate([_dot(a, w_s[j]) for j in range(w_s.shape[0])], axis=1)
        return jnp.concatenate([_dot(a, w_s[j, rows, :]) for j in range(w_s.shape[0])], axis=1)

    def scores_softmax(qg, slot, rows):
        lhs = jnp.where(diag, qg, 0.0).astype(BF16)
        s = jnp.concatenate([_dot(lhs, kbuf[slot, j, rows, :]) for j in range(NJ)], axis=1)
        s = s * SCALE
        m = jnp.max(s, axis=-1, keepdims=True)
        e = jnp.exp(s - m)
        l = jnp.sum(e, axis=-1, keepdims=True)
        return e * (1.0 / l)

    def pv_wo(p, slot, rows):
        pb = p.astype(BF16)
        o = _dot_nt(pb[:, 0:128], vbuf[slot, 0, rows, :])
        for j in range(1, NJ):
            o = o + _dot_nt(pb[:, j * 128:(j + 1) * 128], vbuf[slot, j, rows, :])
        o = jnp.where(diag, o, 0.0).astype(BF16)
        return proj(o, wo_s, rows)

    def moe(x):
        xn = _layernorm(x)
        xb = xn.astype(BF16)
        r = jnp.sum(xb.astype(F32) * wr_in[...].astype(F32), axis=-1, keepdims=True)
        g = proj(xb, wg_s)
        u = proj(xb, wu_s)
        h = (g * jax.nn.sigmoid(g) * u).astype(BF16)
        y = proj(h, wd_s)
        return x + xn + y * jax.nn.sigmoid(r)

    x_cp.wait()
    wr_cp.wait()
    x_s[...] = jnp.zeros_like(x_s)
    x_s[0:B, :] = x_in[...].astype(F32)
    out_s[...] = jnp.zeros_like(out_s)
    xn0 = _layernorm(x_s[...]).astype(BF16)
    for c in wq_cp:
        c.wait()
    q1_s[...] = proj(xn0, wq_s).astype(BF16).astype(F32)

    def batch_body(b, carry):
        slot = b % 2

        def qk1(g, c):
            wait_kv(k_hbm, kbuf, sem_k, b, slot, g)
            off = pl.multiple_of(g * GR, GR)
            qg = jnp.broadcast_to(q1_s[pl.ds(b, 1), pl.ds(off, GR)], (HG, GR))
            p_s[g] = scores_softmax(qg, slot, pl.ds(off, GR))
            return c
        lax.fori_loop(0, NG, qk1, 0)

        @pl.when(b == 0)
        def _():
            for c in wo_cp:
                c.wait()

        def pv1(g, y):
            wait_kv(v_hbm, vbuf, sem_v, b, slot, g)
            off = pl.multiple_of(g * GR, GR)
            return y + pv_wo(p_s[g], slot, pl.ds(off, GR))
        y1 = lax.fori_loop(0, NG, pv1, jnp.zeros((HG, D), F32))

        @pl.when(b == 0)
        def _():
            for c in wg_cp + wu_cp + wd_cp:
                c.wait()

        x0 = jnp.broadcast_to(x_s[pl.ds(b, 1), :], (HG, D))
        x1 = x0 + jnp.sum(y1, axis=0, keepdims=True)
        x2 = moe(x1)

        xn2 = _layernorm(x2).astype(BF16)
        y2 = jnp.zeros((HG, D), F32)
        for g in range(NG):
            rows = pl.ds(g * GR, GR)
            nt = GR // 128
            qg = jnp.concatenate([_dot(xn2, wq_s[g * nt + j]) for j in range(nt)], axis=1)
            p = scores_softmax(qg, slot, rows)
            y2 = y2 + pv_wo(p, slot, rows)

        @pl.when(b + 2 < B)
        def _():
            start_kv(k_hbm, kbuf, sem_k, b + 2, slot)
            start_kv(v_hbm, vbuf, sem_v, b + 2, slot)

        x3 = x2 + jnp.sum(y2, axis=0, keepdims=True)
        x4 = moe(x3)
        out_s[pl.ds(b, 1), :] = x4[0:1, :]
        return carry

    lax.fori_loop(0, B, batch_body, 0)
    o_ref[...] = out_s[0:B, :].astype(o_ref.dtype)


@jax.jit
def pallas_interleave_layers__sliding_block_cached__moe_arch_mod__decode_kernel(
    A_x: jax.Array,
    A_k_cache: jax.Array,
    A_v_cache: jax.Array,
    A_wq: jax.Array,
    A_wo: jax.Array,
    B_x: jax.Array,
    B_w_r: jax.Array,
    B_w_gate: jax.Array,
    B_w_up: jax.Array,
    B_w_down: jax.Array,
):
    x = A_x.reshape(B, D)
    kt = jnp.swapaxes(A_k_cache, 2, 3).reshape(B, H * DH, SK)
    vt = jnp.swapaxes(A_v_cache, 2, 3).reshape(B, H * DH, SK)
    wr = B_w_r.reshape(1, D)

    out = pl.pallas_call(
        _kernel,
        in_specs=[pl.BlockSpec(memory_space=pl.ANY)] * 9,
        out_specs=pl.BlockSpec(memory_space=pltpu.VMEM),
        out_shape=jax.ShapeDtypeStruct((B, D), BF16),
        scratch_shapes=[
            pltpu.VMEM((B, D), BF16),
            pltpu.VMEM((1, D), BF16),
            pltpu.VMEM((H * DH // 128, D, 128), BF16),
            pltpu.VMEM((D // 128, H * DH, 128), BF16),
            pltpu.VMEM((F // 128, D, 128), BF16),
            pltpu.VMEM((F // 128, D, 128), BF16),
            pltpu.VMEM((D // 128, F, 128), BF16),
            pltpu.VMEM((2, NJ, H * DH, 128), BF16),
            pltpu.VMEM((2, NJ, H * DH, 128), BF16),
            pltpu.VMEM((8, D), F32),
            pltpu.VMEM((8, H * DH), F32),
            pltpu.VMEM((NG, HG, W), F32),
            pltpu.VMEM((8, D), F32),
            pltpu.SemaphoreType.DMA((8 + 4 * NG,)),
        ],
        compiler_params=pltpu.CompilerParams(vmem_limit_bytes=100 * 1024 * 1024),
    )(x, kt, vt, A_wq, A_wo, wr, B_w_gate, B_w_up, B_w_down)
    return out.reshape(B, 1, D)
```

```python
import jax
import jax.numpy as jnp
from jax import lax
import jax.experimental.pallas as pl
import jax.experimental.pallas.tpu as pltpu

B, D = 4, 640
H, DH, SK = 32, 192, 4096
W = 1024
F = 1536
NJ = W // 128
HG = 8
NG = H // HG
GR = HG * DH
SR = 2 * DH
NS = H // 2
PG = HG // 2
RC = 128
LN_EPS = 1e-5
SCALE = DH ** -0.5
F32 = jnp.float32
BF16 = jnp.bfloat16
U32 = jnp.uint32

V_CHUNKS = ([(g * GR, GR, 0, NJ) for g in range(NG - 1)]
            + [(s * SR, SR, 0, NJ) for s in range(NS - PG, NS - 1)]
            + [((NS - 1) * SR, SR, 0, 4), ((NS - 1) * SR, SR, 4, 3), ((NS - 1) * SR, SR, 7, 1)])
NVC = len(V_CHUNKS)

SEM_X, SEM_WR, SEM_WQ, SEM_WO, SEM_WG, SEM_WU, SEM_WD = range(7)
SEM_K = 7
SEM_V = SEM_K + 2
NSEM = SEM_V + 2 * NVC


def _dot(a, b):
    return jnp.dot(a, b, preferred_element_type=F32)


def _dot_nt(a, b):
    return lax.dot_general(a, b, (((1,), (1,)), ((), ())), preferred_element_type=F32)


def _ln_stats(x):
    m = jnp.mean(x, axis=-1, keepdims=True)
    c = x - m
    v = jnp.mean(c * c, axis=-1, keepdims=True)
    r = lax.rsqrt(v + LN_EPS)
    return m, r, c * r


def _round(x):
    return x.astype(BF16).astype(F32)


def _kernel(x_hbm, k_hbm, v_hbm, wq_hbm, wo_hbm, wr_hbm, wg_hbm, wu_hbm, wd_hbm,
            o_ref,
            x_in, wr_in, wq_s, wo_s, wg_s, wu_s, wd_s, kbuf, vbuf,
            x_s, q1_s, p_s, out_s,
            sems):

    def start_w(src, dst, sem):
        def body(r, c):
            rows = pl.ds(pl.multiple_of(r * RC, RC), RC)
            for j in range(dst.shape[0]):
                pltpu.make_async_copy(src.at[rows, pl.ds(j * 128, 128)], dst.at[j, rows],
                                      sems.at[sem]).start()
            return c
        lax.fori_loop(0, src.shape[0] // RC, body, 0)

    def wait_w(dst, sem):
        pltpu.make_async_copy(dst, dst, sems.at[sem]).wait()

    def start_chunk(src, dst, sem, b, slot, r0, nr, j0, nj):
        rows = pl.ds(r0, nr)
        for j in range(j0, j0 + nj):
            pltpu.make_async_copy(src.at[b, rows, pl.ds(SK - W + j * 128, 128)],
                                  dst.at[slot, j, rows], sems.at[sem]).start()

    def wait_chunk(dst, sem, slot, r0, nr, j0, nj):
        view = dst.at[slot, pl.ds(j0, nj), pl.ds(r0, nr)]
        pltpu.make_async_copy(view, view, sems.at[sem]).wait()

    def start_k(b, slot):
        start_chunk(k_hbm, kbuf, SEM_K + slot, b, slot, 0, H * DH, 0, NJ)

    def start_v(b, slot, c):
        start_chunk(v_hbm, vbuf, SEM_V + slot * NVC + c, b, slot, *V_CHUNKS[c])

    x_cp = pltpu.make_async_copy(x_hbm, x_in, sems.at[SEM_X])
    wr_cp = pltpu.make_async_copy(wr_hbm, wr_in, sems.at[SEM_WR])
    x_cp.start()
    wr_cp.start()
    start_w(wq_hbm, wq_s, SEM_WQ)
    start_w(wo_hbm, wo_s, SEM_WO)
    start_w(wg_hbm, wg_s, SEM_WG)
    start_w(wu_hbm, wu_s, SEM_WU)
    start_w(wd_hbm, wd_s, SEM_WD)
    start_k(0, 0)
    for c in range(NVC):
        start_v(0, 0, c)

    wq_u, wo_u, wg_u, wu_u, wd_u, k_u, v_u = (
        r.bitcast(U32) for r in (wq_s, wo_s, wg_s, wu_s, wd_s, kbuf, vbuf))

    def tile(ref_u, idx, start, size):
        if isinstance(start, int):
            rows = pl.ds(start // 2, size // 2)
        else:
            rows = pl.ds(pl.multiple_of(start // 2, 8), size // 2)
        return pltpu.bitcast(ref_u[idx + (rows, slice(None))], BF16)

    def proj(a, w_u, tiles, start, size):
        return jnp.concatenate([_dot(a, tile(w_u, (j,), start, size)) for j in tiles], axis=1)

    def ln_lhs(x):
        return jnp.concatenate([x, jnp.ones_like(x)], axis=0).astype(BF16)

    def ln_proj(lhs, mean, rstd, w_u, tiles):
        z = proj(lhs, w_u, tiles, 0, D)
        return (z[0:8] - mean * z[8:16]) * rstd

    row = lax.broadcasted_iota(jnp.int32, (HG, GR), 0)
    col = lax.broadcasted_iota(jnp.int32, (HG, GR), 1)
    diag = (col >= row * DH) & (col < (row + 1) * DH)

    def qk_lhs(qg):
        return jnp.where(diag, qg, 0.0).astype(BF16)

    def softmax(s_tiles):
        s = jnp.concatenate(s_tiles, axis=1) * SCALE
        m = jnp.max(s, axis=-1, keepdims=True)
        e = jnp.exp(s - m)
        l = jnp.sum(e, axis=-1, keepdims=True)
        return e * (1.0 / l)

    def moe(x):
        lhs = ln_lhs(x)
        mean, rstd, xn = _ln_stats(x)
        r = jnp.sum(xn * wr_in[...].astype(F32), axis=-1, keepdims=True)
        g = ln_proj(lhs, mean, rstd, wg_u, range(F // 128))
        u = ln_proj(lhs, mean, rstd, wu_u, range(F // 128))
        h = (g * jax.nn.sigmoid(g) * u).astype(BF16)
        y = proj(h, wd_u, range(D // 128), 0, F)
        return _round(x + (xn + y * jax.nn.sigmoid(r)))

    x_cp.wait()
    wr_cp.wait()
    x_s[...] = jnp.zeros_like(x_s)
    x_s[0:B, :] = x_in[...].astype(F32)
    out_s[...] = jnp.zeros_like(out_s)
    xn0 = _ln_stats(x_s[...])[2].astype(BF16)
    wait_w(wq_s, SEM_WQ)
    q1_s[...] = proj(xn0, wq_u, range(H * DH // 128), 0, D)
    wait_w(wo_s, SEM_WO)
    wait_w(wg_s, SEM_WG)
    wait_w(wu_s, SEM_WU)
    wait_w(wd_s, SEM_WD)

    srow = lax.broadcasted_iota(jnp.int32, (HG, SR), 0)
    scol = lax.broadcasted_iota(jnp.int32, (HG, SR), 1)
    shead = srow - (scol >= DH).astype(jnp.int32)
    ones = jnp.ones((8, 128), BF16)

    def batch_body(b, carry):
        slot = b % 2
        more = b + 1 < B

        def wait_v(c):
            wait_chunk(vbuf, SEM_V + slot * NVC + c, slot, *V_CHUNKS[c])

            @pl.when(more)
            def _():
                start_v(b + 1, 1 - slot, c)

        wait_chunk(kbuf, SEM_K + slot, slot, 0, H * DH, 0, NJ)

        @pl.when(more)
        def _():
            start_k(b + 1, 1 - slot)

        def qk1(g, c):
            off = pl.multiple_of(g * GR, GR)
            qg = jnp.broadcast_to(q1_s[pl.ds(b, 1), pl.ds(off, GR)], (HG, GR))
            lhs = qk_lhs(qg)
            p_s[g] = softmax([_dot(lhs, tile(k_u, (slot, j), off, GR)) for j in range(NJ)])
            return c
        lax.fori_loop(0, NG, qk1, 0)

        def pv_tiles(pb, off, js):
            o = None
            for j in js:
                t = _dot_nt(pb[:, j * 128:(j + 1) * 128], tile(v_u, (slot, j), off, SR))
                o = t if o is None else o + t
            return o

        def wo_pair(o, s, off):
            o = jnp.where(shead == 2 * (s % PG), o, 0.0).astype(BF16)
            return proj(o, wo_u, range(D // 128), off, SR)

        def pv1(s, y):
            for c in range(NVC - 3):
                @pl.when(s == V_CHUNKS[c][0] // SR)
                def _():
                    wait_v(c)
            off = pl.multiple_of(s * SR, SR)
            pb = p_s[s // PG].astype(BF16)
            return y + wo_pair(pv_tiles(pb, off, range(NJ)), s, off)
        y1 = lax.fori_loop(0, NS - 1, pv1, jnp.zeros((HG, D), F32))

        off = (NS - 1) * SR
        pb = p_s[NG - 1].astype(BF16)
        o = None
        for c in range(NVC - 3, NVC):
            wait_v(c)
            t = pv_tiles(pb, off, range(V_CHUNKS[c][2], V_CHUNKS[c][2] + V_CHUNKS[c][3]))
            o = t if o is None else o + t
        y1 = y1 + wo_pair(o, NS - 1, off)

        x0 = jnp.broadcast_to(x_s[pl.ds(b, 1), :], (HG, D))
        x1 = _round(x0 + jnp.sum(y1, axis=0, keepdims=True))
        x2 = moe(x1)

        lhs2 = ln_lhs(x2)
        mean2, rstd2, _ = _ln_stats(x2)
        nt = GR // 128

        def q_group(g):
            return qk_lhs(ln_proj(lhs2, mean2, rstd2, wq_u, range(g * nt, (g + 1) * nt)))

        def s_tile(lhs, g, j):
            return _dot(lhs, tile(k_u, (slot, j), g * GR, GR))

        def pv_pair(p, g, i):
            accs = []
            for m in (2 * i, 2 * i + 1):
                pj = [jnp.broadcast_to(p[m:m + 1, j * 128:(j + 1) * 128], (16, 128))
                      for j in range(NJ)]
                for c in range(DH // 16):
                    start = g * GR + m * DH + c * 16
                    acc = tile(v_u, (slot, 0), start, 16).astype(F32) * pj[0]
                    for j in range(1, NJ):
                        acc = acc + tile(v_u, (slot, j), start, 16).astype(F32) * pj[j]
                    accs.append(acc.astype(BF16))
            return _dot_nt(ones, jnp.concatenate(accs, axis=0)).astype(BF16)

        lhs = q_group(0)
        p = softmax([s_tile(lhs, 0, j) for j in range(NJ)])
        o_groups = []
        for g in range(1, NG):
            lhs = q_group(g)
            st, op = [], []
            for i in range(PG):
                st.append(s_tile(lhs, g, 2 * i))
                st.append(s_tile(lhs, g, 2 * i + 1))
                op.append(pv_pair(p, g - 1, i))
            o_groups.append(jnp.concatenate(op, axis=1))
            p = softmax(st)

        nd = D // 128
        y_tiles = [None] * nd

        def add_y(n, t):
            y_tiles[n] = t if y_tiles[n] is None else y_tiles[n] + t

        jobs = [(g, n) for g in range(NG - 1) for n in range(nd)]
        cuts = [7, 10, 13, 15]
        done = 0
        pend = None
        for i in range(PG):
            for g, n in jobs[done:cuts[i]]:
                add_y(n, _dot(o_groups[g], tile(wo_u, (n,), g * GR, GR)))
            done = cuts[i]
            if pend is not None:
                for n in range(nd):
                    add_y(n, _dot(pend[0], tile(wo_u, (n,), pend[1], SR)))
            pend = (pv_pair(p, NG - 1, i), (NG - 1) * GR + i * SR)
        for n in range(nd):
            add_y(n, _dot(pend[0], tile(wo_u, (n,), pend[1], SR)))

        x3 = _round(x2 + jnp.concatenate(y_tiles, axis=1))
        x4 = moe(x3)
        out_s[pl.ds(b, 1), :] = x4[0:1, :]
        return carry

    lax.fori_loop(0, B, batch_body, 0)
    o_ref[...] = out_s[0:B, :].astype(o_ref.dtype)


@jax.jit
def pallas_interleave_layers__sliding_block_cached__moe_arch_mod__decode_kernel(
    A_x: jax.Array,
    A_k_cache: jax.Array,
    A_v_cache: jax.Array,
    A_wq: jax.Array,
    A_wo: jax.Array,
    B_x: jax.Array,
    B_w_r: jax.Array,
    B_w_gate: jax.Array,
    B_w_up: jax.Array,
    B_w_down: jax.Array,
):
    x = A_x.reshape(B, D)
    kt = jnp.swapaxes(A_k_cache, 2, 3).reshape(B, H * DH, SK)
    vt = jnp.swapaxes(A_v_cache, 2, 3).reshape(B, H * DH, SK)
    wr = B_w_r.reshape(1, D)

    out = pl.pallas_call(
        _kernel,
        in_specs=[pl.BlockSpec(memory_space=pl.ANY)] * 9,
        out_specs=pl.BlockSpec(memory_space=pltpu.VMEM),
        out_shape=jax.ShapeDtypeStruct((B, D), BF16),
        scratch_shapes=[
            pltpu.VMEM((B, D), BF16),
            pltpu.VMEM((1, D), BF16),
            pltpu.VMEM((H * DH // 128, D, 128), BF16),
            pltpu.VMEM((D // 128, H * DH, 128), BF16),
            pltpu.VMEM((F // 128, D, 128), BF16),
            pltpu.VMEM((F // 128, D, 128), BF16),
            pltpu.VMEM((D // 128, F, 128), BF16),
            pltpu.VMEM((2, NJ, H * DH, 128), BF16),
            pltpu.VMEM((2, NJ, H * DH, 128), BF16),
            pltpu.VMEM((8, D), F32),
            pltpu.VMEM((8, H * DH), F32),
            pltpu.VMEM((NG, HG, W), F32),
            pltpu.VMEM((8, D), F32),
            pltpu.SemaphoreType.DMA((NSEM,)),
        ],
        compiler_params=pltpu.CompilerParams(
            vmem_limit_bytes=100 * 1024 * 1024,
            disable_bounds_checks=True,
            disable_semaphore_checks=True,
        ),
    )(x, kt, vt, A_wq, A_wo, wr, B_w_gate, B_w_up, B_w_down)
    return out.reshape(B, 1, D)
```

```python
import jax
import jax.numpy as jnp
from jax import lax
import jax.experimental.pallas as pl
import jax.experimental.pallas.tpu as pltpu

B, D = 4, 640
H, DH, SK = 32, 192, 4096
W = 1024
F = 1536
NJ = W // 128
HG = 8
NG = H // HG
GR = HG * DH
SR = 2 * DH
NS = H // 2
PG = HG // 2
RC = 128
LN_EPS = 1e-5
SCALE = DH ** -0.5
F32 = jnp.float32
BF16 = jnp.bfloat16
U32 = jnp.uint32

V_CHUNKS = ([(g * GR, GR, 0, NJ) for g in range(NG - 1)]
            + [(s * SR, SR, 0, NJ) for s in range(NS - PG, NS - 1)]
            + [((NS - 1) * SR, SR, 0, 4), ((NS - 1) * SR, SR, 4, 3), ((NS - 1) * SR, SR, 7, 1)])
NVC = len(V_CHUNKS)

SEM_X, SEM_WR, SEM_WQ, SEM_WO, SEM_WG, SEM_WU, SEM_WD = range(7)
SEM_K = 7
SEM_V = SEM_K + 2
NSEM = SEM_V + 2 * NVC


def _l2_schedule():
    nt = GR // 128
    nd = D // 128
    t_d = 110
    t_x = 300
    t_soft = 400
    t_pop = 130
    mx = []
    for g in range(NG):
        mx += [('a', g, t) for t in range(nt)] + [('b', g, j) for j in range(NJ)]
    mx += [('f', g, 0, nt, n) for g in range(NG - 1) for n in range(nd)]
    es = [(g, t) for g in range(NG) for t in range(nt)]
    fk = 2
    order, now, vpu = [], 0, 0
    b_end, avail, o_at = {}, [], {}
    last_f = [('f', NG - 1, t, t + fk, n) for t in range(0, nt, fk) for n in range(nd)]

    def start(e):
        return max(vpu, b_end[e[0]] + t_soft)

    while mx or es or last_f:
        while es and es[0][0] in b_end and (start(es[0]) <= now + t_pop or not (mx or (
                last_f and (NG - 1, last_f[0][3] - 1) in o_at))):
            e = es.pop(0)
            st = start(e)
            gate = None
            if e[1] > 0 or vpu > b_end[e[0]] + t_soft:
                cand = [j for (tt, j) in avail if tt <= st + 20]
                gate = cand[-1] if cand else None
            order.append(('e',) + e + (gate,))
            vpu = st + t_d
            o_at[e] = st + t_x
        if last_f and o_at.get((NG - 1, last_f[0][3] - 1), 1 << 30) <= now or not mx:
            if not last_f or (NG - 1, last_f[0][3] - 1) not in o_at:
                continue
            job = last_f.pop(0)
            now = max(now, o_at[NG - 1, job[3] - 1]) + 8 * fk
        else:
            job = mx.pop(0)
            now += {'a': 40, 'b': 96, 'f': 96}[job[0]]
            if job[0] == 'b' and job[2] == NJ - 1:
                b_end[job[1]] = now
        order.append(job)
        avail.append((now + t_pop, job))
    return order


def _dot(a, b):
    return jnp.dot(a, b, preferred_element_type=F32)


def _dot_nt(a, b):
    return lax.dot_general(a, b, (((1,), (1,)), ((), ())), preferred_element_type=F32)


def _ln_stats(x):
    m = jnp.mean(x, axis=-1, keepdims=True)
    c = x - m
    v = jnp.mean(c * c, axis=-1, keepdims=True)
    r = lax.rsqrt(v + LN_EPS)
    return m, r, c * r


def _round(x):
    return x.astype(BF16).astype(F32)


def _kernel(x_hbm, k_hbm, v_hbm, wq_hbm, wo_hbm, wr_hbm, wg_hbm, wu_hbm, wd_hbm,
            o_ref,
            x_in, wr_in, wq_s, wo_s, wg_s, wu_s, wd_s, kbuf, vbuf,
            x_s, q1_s, p_s, out_s,
            sems):

    def start_w(src, dst, sem):
        def body(r, c):
            rows = pl.ds(pl.multiple_of(r * RC, RC), RC)
            for j in range(dst.shape[0]):
                pltpu.make_async_copy(src.at[rows, pl.ds(j * 128, 128)], dst.at[j, rows],
                                      sems.at[sem]).start()
            return c
        lax.fori_loop(0, src.shape[0] // RC, body, 0)

    def wait_w(dst, sem):
        pltpu.make_async_copy(dst, dst, sems.at[sem]).wait()

    def start_chunk(src, dst, sem, b, slot, r0, nr, j0, nj):
        rows = pl.ds(r0, nr)
        for j in range(j0, j0 + nj):
            pltpu.make_async_copy(src.at[b, rows, pl.ds(SK - W + j * 128, 128)],
                                  dst.at[slot, j, rows], sems.at[sem]).start()

    def wait_chunk(dst, sem, slot, r0, nr, j0, nj):
        view = dst.at[slot, pl.ds(j0, nj), pl.ds(r0, nr)]
        pltpu.make_async_copy(view, view, sems.at[sem]).wait()

    def start_k(b, slot):
        start_chunk(k_hbm, kbuf, SEM_K + slot, b, slot, 0, H * DH, 0, NJ)

    def start_v(b, slot, c):
        start_chunk(v_hbm, vbuf, SEM_V + slot * NVC + c, b, slot, *V_CHUNKS[c])

    x_cp = pltpu.make_async_copy(x_hbm, x_in, sems.at[SEM_X])
    wr_cp = pltpu.make_async_copy(wr_hbm, wr_in, sems.at[SEM_WR])
    x_cp.start()
    wr_cp.start()
    start_w(wq_hbm, wq_s, SEM_WQ)
    start_w(wo_hbm, wo_s, SEM_WO)
    start_w(wg_hbm, wg_s, SEM_WG)
    start_w(wu_hbm, wu_s, SEM_WU)
    start_w(wd_hbm, wd_s, SEM_WD)
    start_k(0, 0)
    for c in range(NVC):
        start_v(0, 0, c)

    wq_u, wo_u, wg_u, wu_u, wd_u, k_u, v_u = (
        r.bitcast(U32) for r in (wq_s, wo_s, wg_s, wu_s, wd_s, kbuf, vbuf))

    def tile(ref_u, idx, start, size):
        if isinstance(start, int):
            rows = pl.ds(start // 2, size // 2)
        else:
            rows = pl.ds(pl.multiple_of(start // 2, 8), size // 2)
        return pltpu.bitcast(ref_u[idx + (rows, slice(None))], BF16)

    def proj(a, w_u, tiles, start, size):
        return jnp.concatenate([_dot(a, tile(w_u, (j,), start, size)) for j in tiles], axis=1)

    def ln_lhs(x):
        return jnp.concatenate([x, jnp.ones_like(x)], axis=0).astype(BF16)

    def ln_proj(lhs, mean, rstd, w_u, tiles):
        z = proj(lhs, w_u, tiles, 0, D)
        return (z[0:8] - mean * z[8:16]) * rstd

    row = lax.broadcasted_iota(jnp.int32, (HG, GR), 0)
    col = lax.broadcasted_iota(jnp.int32, (HG, GR), 1)
    diag = (col >= row * DH) & (col < (row + 1) * DH)

    def qk_lhs(qg):
        return jnp.where(diag, qg, 0.0).astype(BF16)

    def softmax(s_tiles):
        s = jnp.concatenate(s_tiles, axis=1) * SCALE
        m = jnp.max(s, axis=-1, keepdims=True)
        e = jnp.exp(s - m)
        l = jnp.sum(e, axis=-1, keepdims=True)
        return e * (1.0 / l)

    def moe(x):
        lhs = ln_lhs(x)
        mean, rstd, xn = _ln_stats(x)
        r = jnp.sum(xn * wr_in[...].astype(F32), axis=-1, keepdims=True)
        g = ln_proj(lhs, mean, rstd, wg_u, range(F // 128))
        u = ln_proj(lhs, mean, rstd, wu_u, range(F // 128))
        h = (g * jax.nn.sigmoid(g) * u).astype(BF16)
        y = proj(h, wd_u, range(D // 128), 0, F)
        return _round(x + (xn + y * jax.nn.sigmoid(r)))

    x_cp.wait()
    wr_cp.wait()
    x_s[...] = jnp.zeros_like(x_s)
    x_s[0:B, :] = x_in[...].astype(F32)
    out_s[...] = jnp.zeros_like(out_s)
    xn0 = _ln_stats(x_s[...])[2].astype(BF16)
    wait_w(wq_s, SEM_WQ)
    q1_s[...] = proj(xn0, wq_u, range(H * DH // 128), 0, D)
    wait_w(wo_s, SEM_WO)
    wait_w(wg_s, SEM_WG)
    wait_w(wu_s, SEM_WU)
    wait_w(wd_s, SEM_WD)

    srow = lax.broadcasted_iota(jnp.int32, (HG, SR), 0)
    scol = lax.broadcasted_iota(jnp.int32, (HG, SR), 1)
    shead = srow - (scol >= DH).astype(jnp.int32)
    ones = jnp.ones((8, 128), BF16)

    def batch_body(b, carry):
        slot = b % 2
        more = b + 1 < B

        def wait_v(c):
            wait_chunk(vbuf, SEM_V + slot * NVC + c, slot, *V_CHUNKS[c])

            @pl.when(more)
            def _():
                start_v(b + 1, 1 - slot, c)

        wait_chunk(kbuf, SEM_K + slot, slot, 0, H * DH, 0, NJ)

        @pl.when(more)
        def _():
            start_k(b + 1, 1 - slot)

        def qk1(g, c):
            off = pl.multiple_of(g * GR, GR)
            qg = jnp.broadcast_to(q1_s[pl.ds(b, 1), pl.ds(off, GR)], (HG, GR))
            lhs = qk_lhs(qg)
            p_s[g] = softmax([_dot(lhs, tile(k_u, (slot, j), off, GR)) for j in range(NJ)])
            return c
        lax.fori_loop(0, NG, qk1, 0)

        def pv_tiles(pb, off, js):
            o = None
            for j in js:
                t = _dot_nt(pb[:, j * 128:(j + 1) * 128], tile(v_u, (slot, j), off, SR))
                o = t if o is None else o + t
            return o

        def wo_pair(o, s, off):
            o = jnp.where(shead == 2 * (s % PG), o, 0.0).astype(BF16)
            return proj(o, wo_u, range(D // 128), off, SR)

        def pv1(s, y):
            for c in range(NVC - 3):
                @pl.when(s == V_CHUNKS[c][0] // SR)
                def _():
                    wait_v(c)
            off = pl.multiple_of(s * SR, SR)
            pb = p_s[s // PG].astype(BF16)
            return y + wo_pair(pv_tiles(pb, off, range(NJ)), s, off)
        y1 = lax.fori_loop(0, NS - 1, pv1, jnp.zeros((HG, D), F32))

        off = (NS - 1) * SR
        pb = p_s[NG - 1].astype(BF16)
        o = None
        for c in range(NVC - 3, NVC):
            wait_v(c)
            t = pv_tiles(pb, off, range(V_CHUNKS[c][2], V_CHUNKS[c][2] + V_CHUNKS[c][3]))
            o = t if o is None else o + t
        y1 = y1 + wo_pair(o, NS - 1, off)

        x0 = jnp.broadcast_to(x_s[pl.ds(b, 1), :], (HG, D))
        x1 = _round(x0 + jnp.sum(y1, axis=0, keepdims=True))
        x2 = moe(x1)

        lhs2 = ln_lhs(x2)
        mean2, rstd2, _ = _ln_stats(x2)
        nt = GR // 128

        nd = D // 128
        q_t, s_t, p_g, pj_h, o_t = {}, {}, {}, {}, {}
        y_tiles = [jnp.where(srow[:, 0:128] == 0, x2[:, n * 128:(n + 1) * 128], 0.0)
                   for n in range(nd)]
        true8 = (srow[:, 0:128] + b) >= 0
        res = {}
        lhs_g = {}

        def job_a(job, g, t):
            res[job] = q_t[g, t] = ln_proj(lhs2, mean2, rstd2, wq_u, [g * nt + t])

        def job_b(job, g, j):
            if g not in lhs_g:
                lhs_g[g] = qk_lhs(jnp.concatenate([q_t[g, t] for t in range(nt)], axis=1))
            res[job] = s_t[g, j] = _dot(lhs_g[g], tile(k_u, (slot, j), g * GR, GR))

        def job_e(job, g, t, gate):
            if g not in p_g:
                p_g[g] = softmax([s_t[g, j] for j in range(NJ)])
            accs = []
            for c in range(8):
                r = t * 128 + c * 16
                m = r // DH
                if (g, m) not in pj_h:
                    pj_h[g, m] = [
                        jnp.broadcast_to(p_g[g][m:m + 1, j * 128:(j + 1) * 128], (16, 128))
                        for j in range(NJ)]
                pj = pj_h[g, m]
                acc = tile(v_u, (slot, 0), g * GR + r, 16).astype(F32) * pj[0]
                for j in range(1, NJ):
                    acc = acc + tile(v_u, (slot, j), g * GR + r, 16).astype(F32) * pj[j]
                if c == 0 and gate is not None:
                    acc = jnp.concatenate([jnp.where(true8, acc[0:8], res[gate]), acc[8:16]],
                                          axis=0)
                accs.append(acc)
            a = jnp.concatenate(accs, axis=0)
            o_t[g, t] = a.T.reshape(16, 8, 128).sum(axis=0)

        def job_f(job, g, t0, t1, n):
            o = jnp.concatenate([o_t[g, t] for t in range(t0, t1)], axis=1).astype(BF16)
            y = _dot(o, tile(wo_u, (n,), g * GR + t0 * 128, (t1 - t0) * 128))
            res[job] = y_tiles[n] = y + y_tiles[n]

        for job in _l2_schedule():
            {'a': job_a, 'b': job_b, 'e': job_e, 'f': job_f}[job[0]](job, *job[1:])

        x3 = _round(jnp.broadcast_to(jnp.sum(jnp.concatenate(y_tiles, axis=1), axis=0, keepdims=True), (8, D)))
        x4 = moe(x3)
        out_s[pl.ds(b, 1), :] = x4[0:1, :]
        return carry

    lax.fori_loop(0, B, batch_body, 0)
    o_ref[...] = out_s[0:B, :].astype(o_ref.dtype)


@jax.jit
def pallas_interleave_layers__sliding_block_cached__moe_arch_mod__decode_kernel(
    A_x: jax.Array,
    A_k_cache: jax.Array,
    A_v_cache: jax.Array,
    A_wq: jax.Array,
    A_wo: jax.Array,
    B_x: jax.Array,
    B_w_r: jax.Array,
    B_w_gate: jax.Array,
    B_w_up: jax.Array,
    B_w_down: jax.Array,
):
    x = A_x.reshape(B, D)
    kt = jnp.swapaxes(A_k_cache, 2, 3).reshape(B, H * DH, SK)
    vt = jnp.swapaxes(A_v_cache, 2, 3).reshape(B, H * DH, SK)
    wr = B_w_r.reshape(1, D)

    out = pl.pallas_call(
        _kernel,
        in_specs=[pl.BlockSpec(memory_space=pl.ANY)] * 9,
        out_specs=pl.BlockSpec(memory_space=pltpu.VMEM),
        out_shape=jax.ShapeDtypeStruct((B, D), BF16),
        scratch_shapes=[
            pltpu.VMEM((B, D), BF16),
            pltpu.VMEM((1, D), BF16),
            pltpu.VMEM((H * DH // 128, D, 128), BF16),
            pltpu.VMEM((D // 128, H * DH, 128), BF16),
            pltpu.VMEM((F // 128, D, 128), BF16),
            pltpu.VMEM((F // 128, D, 128), BF16),
            pltpu.VMEM((D // 128, F, 128), BF16),
            pltpu.VMEM((2, NJ, H * DH, 128), BF16),
            pltpu.VMEM((2, NJ, H * DH, 128), BF16),
            pltpu.VMEM((8, D), F32),
            pltpu.VMEM((8, H * DH), F32),
            pltpu.VMEM((NG, HG, W), F32),
            pltpu.VMEM((8, D), F32),
            pltpu.SemaphoreType.DMA((NSEM,)),
        ],
        compiler_params=pltpu.CompilerParams(
            vmem_limit_bytes=100 * 1024 * 1024,
            disable_bounds_checks=True,
            disable_semaphore_checks=True,
        ),
    )(x, kt, vt, A_wq, A_wo, wr, B_w_gate, B_w_up, B_w_down)
    return out.reshape(B, 1, D)
```

```python
import jax
import jax.numpy as jnp
from jax import lax
import jax.experimental.pallas as pl
import jax.experimental.pallas.tpu as pltpu

B, D = 4, 640
H, DH, SK = 32, 192, 4096
W = 1024
F = 1536
NJ = W // 128
HG = 8
NG = H // HG
GR = HG * DH
SR = 2 * DH
NS = H // 2
PG = HG // 2
JW0 = (SK - W) // 128
JW = 4
LN_EPS = 1e-5
SCALE = DH ** -0.5
F32 = jnp.float32
BF16 = jnp.bfloat16
U32 = jnp.uint32

V_CHUNKS = ([(g * GR, GR, 0, NJ) for g in range(NG - 1)]
            + [(s * SR, SR, 0, NJ) for s in range(NS - PG, NS - 1)]
            + [((NS - 1) * SR, SR, 0, 4), ((NS - 1) * SR, SR, 4, 3), ((NS - 1) * SR, SR, 7, 1)])
NVC = len(V_CHUNKS)

SEM_X, SEM_WR, SEM_WQ, SEM_WO, SEM_WG, SEM_WU, SEM_WD = range(7)
SEM_K = 7
SEM_V = SEM_K + 2
NSEM = SEM_V + 2 * NVC


def _l2_schedule():
    nt = GR // 128
    nd = D // 128
    t_d = 110
    t_x = 300
    t_soft = 400
    t_pop = 130
    mx = []
    for g in range(NG):
        mx += [('a', g, t) for t in range(nt)] + [('b', g, j) for j in range(NJ)]
    mx += [('f', g, 0, nt, n) for g in range(NG - 1) for n in range(nd)]
    es = [(g, t) for g in range(NG) for t in range(nt)]
    fk = 2
    order, now, vpu = [], 0, 0
    b_end, avail, o_at = {}, [], {}
    last_f = [('f', NG - 1, t, t + fk, n) for t in range(0, nt, fk) for n in range(nd)]

    def start(e):
        return max(vpu, b_end[e[0]] + t_soft)

    while mx or es or last_f:
        while es and es[0][0] in b_end and (start(es[0]) <= now + t_pop or not (mx or (
                last_f and (NG - 1, last_f[0][3] - 1) in o_at))):
            e = es.pop(0)
            st = start(e)
            gate = None
            if e[1] > 0 or vpu > b_end[e[0]] + t_soft:
                cand = [j for (tt, j) in avail if tt <= st + 20]
                gate = cand[-1] if cand else None
            order.append(('e',) + e + (gate,))
            vpu = st + t_d
            o_at[e] = st + t_x
        if last_f and o_at.get((NG - 1, last_f[0][3] - 1), 1 << 30) <= now or not mx:
            if not last_f or (NG - 1, last_f[0][3] - 1) not in o_at:
                continue
            job = last_f.pop(0)
            now = max(now, o_at[NG - 1, job[3] - 1]) + 8 * fk
        else:
            job = mx.pop(0)
            now += {'a': 40, 'b': 96, 'f': 96}[job[0]]
            if job[0] == 'b' and job[2] == NJ - 1:
                b_end[job[1]] = now
        order.append(job)
        avail.append((now + t_pop, job))
    return order


def _dot(a, b):
    return jnp.dot(a, b, preferred_element_type=F32)


def _dot_nt(a, b):
    return lax.dot_general(a, b, (((1,), (1,)), ((), ())), preferred_element_type=F32)


def _ln_stats(x):
    m = jnp.mean(x, axis=-1, keepdims=True)
    c = x - m
    v = jnp.mean(c * c, axis=-1, keepdims=True)
    r = lax.rsqrt(v + LN_EPS)
    return m, r, c * r


def _round(x):
    return x.astype(BF16).astype(F32)


def _kernel(x_hbm, k_hbm, v_hbm, wq_hbm, wo_hbm, wr_hbm, wg_hbm, wu_hbm, wd_hbm,
            o_ref,
            x_in, wr_in, wq_s, wo_s, wg_s, wu_s, wd_s, kbuf, vbuf,
            x_s, q1_s, p_s, out_s,
            sems):

    def start_rows(src, dst, sem, r0, nr, j_src, j0, nj, jw):
        rows = pl.ds(r0 // 16, nr // 16)
        for par in range(2):
            for j in range(j0, j0 + nj, jw):
                n = min(jw, j0 + nj - j)
                pltpu.make_async_copy(src.at[rows, par, pl.ds(j_src + j, n)],
                                      dst.at[rows, pl.ds(j, n), pl.ds(par * 8, 8)],
                                      sems.at[sem]).start()

    def start_w(src, dst, sem, nr):
        for r0 in range(0, dst.shape[0] * 16, nr):
            start_rows(src, dst, sem, r0, nr, 0, 0, dst.shape[1], dst.shape[1])

    def wait_w(dst, sem):
        pltpu.make_async_copy(dst, dst, sems.at[sem]).wait()

    def wait_chunk(dst, sem, slot, r0, nr, j0, nj):
        view = dst.at[slot, pl.ds(r0 // 16, nr // 16), pl.ds(j0, nj)]
        pltpu.make_async_copy(view, view, sems.at[sem]).wait()

    def start_k(b, slot):
        for g in range(NG):
            start_rows(k_hbm.at[b], kbuf.at[slot], SEM_K + slot, g * GR, GR, JW0, 0, NJ, JW)

    def start_v(b, slot, c):
        r0, nr, j0, nj = V_CHUNKS[c]
        start_rows(v_hbm.at[b], vbuf.at[slot], SEM_V + slot * NVC + c, r0, nr, JW0, j0, nj, JW)

    x_cp = pltpu.make_async_copy(x_hbm, x_in, sems.at[SEM_X])
    wr_cp = pltpu.make_async_copy(wr_hbm, wr_in, sems.at[SEM_WR])
    x_cp.start()
    wr_cp.start()
    start_w(wq_hbm, wq_s, SEM_WQ, D)
    start_w(wo_hbm, wo_s, SEM_WO, 384)
    start_w(wg_hbm, wg_s, SEM_WG, D)
    start_w(wu_hbm, wu_s, SEM_WU, D)
    start_w(wd_hbm, wd_s, SEM_WD, 384)
    start_k(0, 0)
    for c in range(NVC):
        start_v(0, 0, c)

    wq_u, wo_u, wg_u, wu_u, wd_u, k_u, v_u = (
        r.bitcast(U32) for r in (wq_s, wo_s, wg_s, wu_s, wd_s, kbuf, vbuf))

    def tile(ref_u, idx, start, size):
        x = ref_u[idx[:-1] + (pl.ds(start // 16, size // 16), idx[-1])]
        return pltpu.bitcast(x.reshape(size // 2, 128), BF16)

    def proj(a, w_u, tiles, start, size):
        return jnp.concatenate([_dot(a, tile(w_u, (j,), start, size)) for j in tiles], axis=1)

    def ln_lhs(x):
        return jnp.concatenate([x, jnp.ones_like(x)], axis=0).astype(BF16)

    def ln_proj(lhs, mean, rstd, w_u, tiles):
        z = proj(lhs, w_u, tiles, 0, D)
        return (z[0:8] - mean * z[8:16]) * rstd

    row = lax.broadcasted_iota(jnp.int32, (HG, GR), 0)
    col = lax.broadcasted_iota(jnp.int32, (HG, GR), 1)
    diag = (col >= row * DH) & (col < (row + 1) * DH)

    def qk_lhs(qg):
        return jnp.where(diag, qg, 0.0).astype(BF16)

    def softmax(s_tiles):
        s = jnp.concatenate(s_tiles, axis=1) * SCALE
        m = jnp.max(s, axis=-1, keepdims=True)
        e = jnp.exp(s - m)
        l = jnp.sum(e, axis=-1, keepdims=True)
        return e * (1.0 / l)

    def moe(x):
        lhs = ln_lhs(x)
        mean, rstd, xn = _ln_stats(x)
        r = jnp.sum(xn * wr_in[...].astype(F32), axis=-1, keepdims=True)
        g = ln_proj(lhs, mean, rstd, wg_u, range(F // 128))
        u = ln_proj(lhs, mean, rstd, wu_u, range(F // 128))
        h = (g * jax.nn.sigmoid(g) * u).astype(BF16)
        y = proj(h, wd_u, range(D // 128), 0, F)
        return _round(x + (xn + y * jax.nn.sigmoid(r)))

    x_cp.wait()
    wr_cp.wait()
    x_s[...] = jnp.zeros_like(x_s)
    x_s[0:B, :] = x_in[...].astype(F32)
    out_s[...] = jnp.zeros_like(out_s)
    xn0 = _ln_stats(x_s[...])[2].astype(BF16)
    wait_w(wq_s, SEM_WQ)
    q1_s[...] = proj(xn0, wq_u, range(H * DH // 128), 0, D)
    wait_w(wo_s, SEM_WO)
    wait_w(wg_s, SEM_WG)
    wait_w(wu_s, SEM_WU)
    wait_w(wd_s, SEM_WD)

    srow = lax.broadcasted_iota(jnp.int32, (HG, SR), 0)
    scol = lax.broadcasted_iota(jnp.int32, (HG, SR), 1)
    shead = srow - (scol >= DH).astype(jnp.int32)

    def batch_body(b, carry):
        slot = b % 2
        more = b + 1 < B

        def wait_v(c):
            wait_chunk(vbuf, SEM_V + slot * NVC + c, slot, *V_CHUNKS[c])

            @pl.when(more)
            def _():
                start_v(b + 1, 1 - slot, c)

        wait_chunk(kbuf, SEM_K + slot, slot, 0, H * DH, 0, NJ)

        @pl.when(more)
        def _():
            start_k(b + 1, 1 - slot)

        def qk1(g, c):
            off = pl.multiple_of(g * GR, GR)
            qg = jnp.broadcast_to(q1_s[pl.ds(b, 1), pl.ds(off, GR)], (HG, GR))
            lhs = qk_lhs(qg)
            p_s[g] = softmax([_dot(lhs, tile(k_u, (slot, j), off, GR)) for j in range(NJ)])
            return c
        lax.fori_loop(0, NG, qk1, 0)

        def pv_tiles(pb, off, js):
            o = None
            for j in js:
                t = _dot_nt(pb[:, j * 128:(j + 1) * 128], tile(v_u, (slot, j), off, SR))
                o = t if o is None else o + t
            return o

        def wo_pair(o, s, off):
            o = jnp.where(shead == 2 * (s % PG), o, 0.0).astype(BF16)
            return proj(o, wo_u, range(D // 128), off, SR)

        def pv1(s, y):
            for c in range(NVC - 3):
                @pl.when(s == V_CHUNKS[c][0] // SR)
                def _():
                    wait_v(c)
            off = pl.multiple_of(s * SR, SR)
            pb = p_s[s // PG].astype(BF16)
            return y + wo_pair(pv_tiles(pb, off, range(NJ)), s, off)
        y1 = lax.fori_loop(0, NS - 1, pv1, jnp.zeros((HG, D), F32))

        off = (NS - 1) * SR
        pb = p_s[NG - 1].astype(BF16)
        o = None
        for c in range(NVC - 3, NVC):
            wait_v(c)
            t = pv_tiles(pb, off, range(V_CHUNKS[c][2], V_CHUNKS[c][2] + V_CHUNKS[c][3]))
            o = t if o is None else o + t
        y1 = y1 + wo_pair(o, NS - 1, off)

        x0 = jnp.broadcast_to(x_s[pl.ds(b, 1), :], (HG, D))
        x1 = _round(x0 + jnp.sum(y1, axis=0, keepdims=True))
        x2 = moe(x1)

        lhs2 = ln_lhs(x2)
        mean2, rstd2, _ = _ln_stats(x2)
        nt = GR // 128

        nd = D // 128
        q_t, s_t, p_g, pj_h, o_t = {}, {}, {}, {}, {}
        y_tiles = [jnp.where(srow[:, 0:128] == 0, x2[:, n * 128:(n + 1) * 128], 0.0)
                   for n in range(nd)]
        true8 = (srow[:, 0:128] + b) >= 0
        res = {}
        lhs_g = {}

        def job_a(job, g, t):
            res[job] = q_t[g, t] = ln_proj(lhs2, mean2, rstd2, wq_u, [g * nt + t])

        def job_b(job, g, j):
            if g not in lhs_g:
                lhs_g[g] = qk_lhs(jnp.concatenate([q_t[g, t] for t in range(nt)], axis=1))
            res[job] = s_t[g, j] = _dot(lhs_g[g], tile(k_u, (slot, j), g * GR, GR))

        def job_e(job, g, t, gate):
            if g not in p_g:
                p_g[g] = softmax([s_t[g, j] for j in range(NJ)])
            accs = []
            for c in range(8):
                r = t * 128 + c * 16
                m = r // DH
                if (g, m) not in pj_h:
                    pj_h[g, m] = [
                        jnp.broadcast_to(p_g[g][m:m + 1, j * 128:(j + 1) * 128], (16, 128))
                        for j in range(NJ)]
                pj = pj_h[g, m]
                acc = tile(v_u, (slot, 0), g * GR + r, 16).astype(F32) * pj[0]
                for j in range(1, NJ):
                    acc = acc + tile(v_u, (slot, j), g * GR + r, 16).astype(F32) * pj[j]
                if c == 0 and gate is not None:
                    acc = jnp.concatenate([jnp.where(true8, acc[0:8], res[gate]), acc[8:16]],
                                          axis=0)
                accs.append(acc)
            a = jnp.concatenate(accs, axis=0)
            o_t[g, t] = a.T.reshape(16, 8, 128).sum(axis=0)

        def job_f(job, g, t0, t1, n):
            o = jnp.concatenate([o_t[g, t] for t in range(t0, t1)], axis=1).astype(BF16)
            y = _dot(o, tile(wo_u, (n,), g * GR + t0 * 128, (t1 - t0) * 128))
            res[job] = y_tiles[n] = y + y_tiles[n]

        for job in _l2_schedule():
            {'a': job_a, 'b': job_b, 'e': job_e, 'f': job_f}[job[0]](job, *job[1:])

        x3 = _round(jnp.broadcast_to(jnp.sum(jnp.concatenate(y_tiles, axis=1), axis=0, keepdims=True), (8, D)))
        x4 = moe(x3)
        out_s[pl.ds(b, 1), :] = x4[0:1, :]
        return carry

    lax.fori_loop(0, B, batch_body, 0)
    o_ref[...] = out_s[0:B, :].astype(o_ref.dtype)


def _tile_view(t):
    *lead, r, c = t.shape
    n = len(lead)
    t = t.reshape(*lead, r // 16, 2, 8, c // 128, 128)
    return t.transpose(*range(n), n, n + 1, n + 3, n + 2, n + 4)


@jax.jit
def pallas_interleave_layers__sliding_block_cached__moe_arch_mod__decode_kernel(
    A_x: jax.Array,
    A_k_cache: jax.Array,
    A_v_cache: jax.Array,
    A_wq: jax.Array,
    A_wo: jax.Array,
    B_x: jax.Array,
    B_w_r: jax.Array,
    B_w_gate: jax.Array,
    B_w_up: jax.Array,
    B_w_down: jax.Array,
):
    x = A_x.reshape(B, D)
    kt = _tile_view(jnp.swapaxes(A_k_cache, 2, 3).reshape(B, H * DH, SK))
    vt = _tile_view(jnp.swapaxes(A_v_cache, 2, 3).reshape(B, H * DH, SK))
    wr = B_w_r.reshape(1, D)

    out = pl.pallas_call(
        _kernel,
        in_specs=[pl.BlockSpec(memory_space=pl.ANY)] * 9,
        out_specs=pl.BlockSpec(memory_space=pltpu.VMEM),
        out_shape=jax.ShapeDtypeStruct((B, D), BF16),
        scratch_shapes=[
            pltpu.VMEM((B, D), BF16),
            pltpu.VMEM((1, D), BF16),
            pltpu.VMEM((D // 16, H * DH // 128, 16, 128), BF16),
            pltpu.VMEM((H * DH // 16, D // 128, 16, 128), BF16),
            pltpu.VMEM((D // 16, F // 128, 16, 128), BF16),
            pltpu.VMEM((D // 16, F // 128, 16, 128), BF16),
            pltpu.VMEM((F // 16, D // 128, 16, 128), BF16),
            pltpu.VMEM((2, H * DH // 16, NJ, 16, 128), BF16),
            pltpu.VMEM((2, H * DH // 16, NJ, 16, 128), BF16),
            pltpu.VMEM((8, D), F32),
            pltpu.VMEM((8, H * DH), F32),
            pltpu.VMEM((NG, HG, W), F32),
            pltpu.VMEM((8, D), F32),
            pltpu.SemaphoreType.DMA((NSEM,)),
        ],
        compiler_params=pltpu.CompilerParams(
            vmem_limit_bytes=100 * 1024 * 1024,
            disable_bounds_checks=True,
            disable_semaphore_checks=True,
        ),
    )(x, kt, vt, _tile_view(A_wq), _tile_view(A_wo), wr,
      _tile_view(B_w_gate), _tile_view(B_w_up), _tile_view(B_w_down))
    return out.reshape(B, 1, D)
```

```python
import jax
import jax.numpy as jnp
from jax import lax
import jax.experimental.pallas as pl
import jax.experimental.pallas.tpu as pltpu

B, D = 4, 640
H, DH, SK = 32, 192, 4096
W = 1024
F = 1536
NJ = W // 128
HG = 8
NG = H // HG
GR = HG * DH
SR = 2 * DH
NS = H // 2
PG = HG // 2
JW0 = (SK - W) // 128
JW = 4
LN_EPS = 1e-5
SCALE = DH ** -0.5
F32 = jnp.float32
BF16 = jnp.bfloat16
U32 = jnp.uint32

V_CHUNKS = ([(g * GR, GR, 0, NJ) for g in range(NG - 1)]
            + [(s * SR, SR, 0, NJ) for s in range(NS - PG, NS - 1)]
            + [((NS - 1) * SR, SR, 0, 4), ((NS - 1) * SR, SR, 4, 3), ((NS - 1) * SR, SR, 7, 1)])
NVC = len(V_CHUNKS)

SEM_X, SEM_WR, SEM_WQ, SEM_WO, SEM_WG, SEM_WU, SEM_WD = range(7)
SEM_K = 7
SEM_V = SEM_K + 2
NSEM = SEM_V + 2 * NVC


def _l2_schedule():
    nt = GR // 128
    nd = D // 128
    t_d = 110
    t_x = 300
    t_soft = 400
    t_pop = 130
    mx = []
    for g in range(NG):
        mx += [('a', g, t) for t in range(nt)] + [('b', g, j) for j in range(NJ)]
    mx += [('f', g, 0, nt, n) for g in range(NG - 1) for n in range(nd)]
    es = [(g, t) for g in range(NG) for t in range(nt)]
    fk = 2
    order, now, vpu = [], 0, 0
    b_end, avail, o_at = {}, [], {}
    last_f = [('f', NG - 1, t, t + fk, n) for t in range(0, nt, fk) for n in range(nd)]

    def start(e):
        return max(vpu, b_end[e[0]] + t_soft)

    while mx or es or last_f:
        while es and es[0][0] in b_end and (start(es[0]) <= now + t_pop or not (mx or (
                last_f and (NG - 1, last_f[0][3] - 1) in o_at))):
            e = es.pop(0)
            st = start(e)
            gate = None
            if e[1] > 0 or vpu > b_end[e[0]] + t_soft:
                cand = [j for (tt, j) in avail if tt <= st + 20]
                gate = cand[-1] if cand else None
            order.append(('e',) + e + (gate,))
            vpu = st + t_d
            o_at[e] = st + t_x
        if last_f and o_at.get((NG - 1, last_f[0][3] - 1), 1 << 30) <= now or not mx:
            if not last_f or (NG - 1, last_f[0][3] - 1) not in o_at:
                continue
            job = last_f.pop(0)
            now = max(now, o_at[NG - 1, job[3] - 1]) + 8 * fk
        else:
            job = mx.pop(0)
            now += {'a': 40, 'b': 96, 'f': 96}[job[0]]
            if job[0] == 'b' and job[2] == NJ - 1:
                b_end[job[1]] = now
        order.append(job)
        avail.append((now + t_pop, job))
    return order


def _dot(a, b):
    return jnp.dot(a, b, preferred_element_type=F32)


def _dot_nt(a, b):
    return lax.dot_general(a, b, (((1,), (1,)), ((), ())), preferred_element_type=F32)


def _ln_stats(x):
    m = jnp.mean(x, axis=-1, keepdims=True)
    c = x - m
    v = jnp.mean(c * c, axis=-1, keepdims=True)
    r = lax.rsqrt(v + LN_EPS)
    return m, r, c * r


def _round(x):
    return x.astype(BF16).astype(F32)


def _kernel(x_hbm, k_hbm, v_hbm, wq_hbm, wo_hbm, wr_hbm, wg_hbm, wu_hbm, wd_hbm,
            o_ref,
            x_in, wr_in, wq_s, wo_s, wg_s, wu_s, wd_s, kbuf, vbuf,
            x_s, q1_s, p_s, out_s, wr_s,
            sems):

    def start_rows(src, dst, sem, r0, nr, j_src, j0, nj, jw):
        rows = pl.ds(r0 // 16, nr // 16)
        for par in range(2):
            for j in range(j0, j0 + nj, jw):
                n = min(jw, j0 + nj - j)
                pltpu.make_async_copy(src.at[rows, par, pl.ds(j_src + j, n)],
                                      dst.at[rows, pl.ds(j, n), pl.ds(par * 8, 8)],
                                      sems.at[sem]).start()

    def start_w(src, dst, sem, nr):
        for r0 in range(0, dst.shape[0] * 16, nr):
            start_rows(src, dst, sem, r0, nr, 0, 0, dst.shape[1], dst.shape[1])

    def wait_w(dst, sem):
        pltpu.make_async_copy(dst, dst, sems.at[sem]).wait()

    def wait_chunk(dst, sem, slot, r0, nr, j0, nj):
        view = dst.at[slot, pl.ds(r0 // 16, nr // 16), pl.ds(j0, nj)]
        pltpu.make_async_copy(view, view, sems.at[sem]).wait()

    def start_k(b, slot):
        for g in range(NG):
            start_rows(k_hbm.at[b], kbuf.at[slot], SEM_K + slot, g * GR, GR, JW0, 0, NJ, JW)

    def start_v(b, slot, c):
        r0, nr, j0, nj = V_CHUNKS[c]
        start_rows(v_hbm.at[b], vbuf.at[slot], SEM_V + slot * NVC + c, r0, nr, JW0, j0, nj, JW)

    x_cp = pltpu.make_async_copy(x_hbm, x_in, sems.at[SEM_X])
    wr_cp = pltpu.make_async_copy(wr_hbm, wr_in, sems.at[SEM_WR])
    x_cp.start()
    wr_cp.start()
    start_w(wq_hbm, wq_s, SEM_WQ, D)
    start_w(wo_hbm, wo_s, SEM_WO, 384)
    start_w(wg_hbm, wg_s, SEM_WG, D)
    start_w(wu_hbm, wu_s, SEM_WU, D)
    start_w(wd_hbm, wd_s, SEM_WD, 384)
    start_k(0, 0)
    for c in range(NVC):
        start_v(0, 0, c)

    wq_u, wo_u, wg_u, wu_u, wd_u, k_u, v_u = (
        r.bitcast(U32) for r in (wq_s, wo_s, wg_s, wu_s, wd_s, kbuf, vbuf))

    def tile(ref_u, idx, start, size):
        x = ref_u[idx[:-1] + (pl.ds(start // 16, size // 16), idx[-1])]
        return pltpu.bitcast(x.reshape(size // 2, 128), BF16)

    def proj(a, w_u, tiles, start, size):
        return jnp.concatenate([_dot(a, tile(w_u, (j,), start, size)) for j in tiles], axis=1)

    def ln_lhs(x):
        return jnp.concatenate([x, jnp.ones_like(x)], axis=0).astype(BF16)

    def ln_proj(lhs, mean, rstd, w_u, tiles):
        z = proj(lhs, w_u, tiles, 0, D)
        return (z[0:8] - mean * z[8:16]) * rstd

    row = lax.broadcasted_iota(jnp.int32, (HG, GR), 0)
    col = lax.broadcasted_iota(jnp.int32, (HG, GR), 1)
    diag = (col >= row * DH) & (col < (row + 1) * DH)

    def qk_lhs(qg):
        return jnp.where(diag, qg, 0.0).astype(BF16)

    def softmax(s_tiles):
        s = jnp.concatenate(s_tiles, axis=1) * SCALE
        m = jnp.max(s, axis=-1, keepdims=True)
        e = jnp.exp(s - m)
        l = jnp.sum(e, axis=-1, keepdims=True)
        return e * (1.0 / l)

    def moe(x):
        lhs = ln_lhs(x)
        mean, rstd, xn = _ln_stats(x)
        r = jnp.sum(xn * wr_s[...], axis=-1, keepdims=True)
        g = ln_proj(lhs, mean, rstd, wg_u, range(F // 128))
        u = ln_proj(lhs, mean, rstd, wu_u, range(F // 128))
        h = (g * jax.nn.sigmoid(g) * u).astype(BF16)
        y = proj(h, wd_u, range(D // 128), 0, F)
        return _round(x + (xn + y * jax.nn.sigmoid(r)))

    x_cp.wait()
    wr_cp.wait()
    wr_s[...] = wr_in[...].astype(F32).reshape(1, D)
    x_s[...] = jnp.zeros_like(x_s)
    x_s[0:B, :] = x_in[...].astype(F32)
    out_s[...] = jnp.zeros_like(out_s)
    xn0 = _ln_stats(x_s[...])[2].astype(BF16)
    wait_w(wq_s, SEM_WQ)
    q1_s[...] = proj(xn0, wq_u, range(H * DH // 128), 0, D)
    wait_w(wo_s, SEM_WO)
    wait_w(wg_s, SEM_WG)
    wait_w(wu_s, SEM_WU)
    wait_w(wd_s, SEM_WD)

    srow = lax.broadcasted_iota(jnp.int32, (HG, SR), 0)
    scol = lax.broadcasted_iota(jnp.int32, (HG, SR), 1)
    shead = srow - (scol >= DH).astype(jnp.int32)

    def batch_body(b, carry):
        slot = b % 2
        more = b + 1 < B

        def wait_v(c):
            wait_chunk(vbuf, SEM_V + slot * NVC + c, slot, *V_CHUNKS[c])

            @pl.when(more)
            def _():
                start_v(b + 1, 1 - slot, c)

        wait_chunk(kbuf, SEM_K + slot, slot, 0, H * DH, 0, NJ)

        @pl.when(more)
        def _():
            start_k(b + 1, 1 - slot)

        def qk1(g, c):
            off = pl.multiple_of(g * GR, GR)
            qg = jnp.broadcast_to(q1_s[pl.ds(b, 1), pl.ds(off, GR)], (HG, GR))
            lhs = qk_lhs(qg)
            p_s[g] = softmax([_dot(lhs, tile(k_u, (slot, j), off, GR)) for j in range(NJ)])
            return c
        lax.fori_loop(0, NG, qk1, 0)

        def pv_tiles(pb, off, js):
            o = None
            for j in js:
                t = _dot_nt(pb[:, j * 128:(j + 1) * 128], tile(v_u, (slot, j), off, SR))
                o = t if o is None else o + t
            return o

        def wo_pair(o, s, off):
            o = jnp.where(shead == 2 * (s % PG), o, 0.0).astype(BF16)
            return proj(o, wo_u, range(D // 128), off, SR)

        def pv1(s, y):
            for c in range(NVC - 3):
                @pl.when(s == V_CHUNKS[c][0] // SR)
                def _():
                    wait_v(c)
            off = pl.multiple_of(s * SR, SR)
            pb = p_s[s // PG].astype(BF16)
            return y + wo_pair(pv_tiles(pb, off, range(NJ)), s, off)
        y1 = lax.fori_loop(0, NS - 1, pv1, jnp.zeros((HG, D), F32))

        off = (NS - 1) * SR
        pb = p_s[NG - 1].astype(BF16)
        o = None
        for c in range(NVC - 3, NVC):
            wait_v(c)
            t = pv_tiles(pb, off, range(V_CHUNKS[c][2], V_CHUNKS[c][2] + V_CHUNKS[c][3]))
            o = t if o is None else o + t
        y1 = y1 + wo_pair(o, NS - 1, off)

        x0 = jnp.broadcast_to(x_s[pl.ds(b, 1), :], (HG, D))
        x1 = _round(x0 + jnp.sum(y1, axis=0, keepdims=True))
        x2 = moe(x1)

        lhs2 = ln_lhs(x2)
        mean2, rstd2, _ = _ln_stats(x2)
        nt = GR // 128

        nd = D // 128
        q_t, s_t, p_g, pj_h, o_t = {}, {}, {}, {}, {}
        y_tiles = [jnp.where(srow[:, 0:128] == 0, x2[:, n * 128:(n + 1) * 128], 0.0)
                   for n in range(nd)]
        true8 = (srow[:, 0:128] + b) >= 0
        res = {}
        lhs_g = {}

        def job_a(job, g, t):
            res[job] = q_t[g, t] = ln_proj(lhs2, mean2, rstd2, wq_u, [g * nt + t])

        def job_b(job, g, j):
            if g not in lhs_g:
                lhs_g[g] = qk_lhs(jnp.concatenate([q_t[g, t] for t in range(nt)], axis=1))
            res[job] = s_t[g, j] = _dot(lhs_g[g], tile(k_u, (slot, j), g * GR, GR))

        def job_e(job, g, t, gate):
            if g not in p_g:
                p_g[g] = softmax([s_t[g, j] for j in range(NJ)])
            accs = []
            for c in range(8):
                r = t * 128 + c * 16
                m = r // DH
                if (g, m) not in pj_h:
                    pj_h[g, m] = [
                        jnp.broadcast_to(p_g[g][m:m + 1, j * 128:(j + 1) * 128], (16, 128))
                        for j in range(NJ)]
                pj = pj_h[g, m]
                acc = tile(v_u, (slot, 0), g * GR + r, 16).astype(F32) * pj[0]
                for j in range(1, NJ):
                    acc = acc + tile(v_u, (slot, j), g * GR + r, 16).astype(F32) * pj[j]
                if c == 0 and gate is not None:
                    acc = jnp.concatenate([jnp.where(true8, acc[0:8], res[gate]), acc[8:16]],
                                          axis=0)
                accs.append(acc)
            a = jnp.concatenate(accs, axis=0)
            o_t[g, t] = a.T.reshape(16, 8, 128).sum(axis=0)

        def job_f(job, g, t0, t1, n):
            o = jnp.concatenate([o_t[g, t] for t in range(t0, t1)], axis=1).astype(BF16)
            y = _dot(o, tile(wo_u, (n,), g * GR + t0 * 128, (t1 - t0) * 128))
            res[job] = y_tiles[n] = y + y_tiles[n]

        for job in _l2_schedule():
            {'a': job_a, 'b': job_b, 'e': job_e, 'f': job_f}[job[0]](job, *job[1:])

        x3 = _round(jnp.broadcast_to(jnp.sum(jnp.concatenate(y_tiles, axis=1), axis=0, keepdims=True), (8, D)))
        x4 = moe(x3)
        out_s[pl.ds(b, 1), :] = x4[0:1, :]
        return carry

    lax.fori_loop(0, B, batch_body, 0)
    o_ref[...] = out_s[0:B, :].astype(o_ref.dtype)


def _tile_view(t):
    *lead, r, c = t.shape
    n = len(lead)
    t = t.reshape(*lead, r // 16, 2, 8, c // 128, 128)
    return t.transpose(*range(n), n, n + 1, n + 3, n + 2, n + 4)


@jax.jit
def pallas_interleave_layers__sliding_block_cached__moe_arch_mod__decode_kernel(
    A_x: jax.Array,
    A_k_cache: jax.Array,
    A_v_cache: jax.Array,
    A_wq: jax.Array,
    A_wo: jax.Array,
    B_x: jax.Array,
    B_w_r: jax.Array,
    B_w_gate: jax.Array,
    B_w_up: jax.Array,
    B_w_down: jax.Array,
):
    x = A_x.reshape(B, D)
    kt = _tile_view(jnp.swapaxes(A_k_cache, 2, 3).reshape(B, H * DH, SK))
    vt = _tile_view(jnp.swapaxes(A_v_cache, 2, 3).reshape(B, H * DH, SK))

    out = pl.pallas_call(
        _kernel,
        in_specs=[pl.BlockSpec(memory_space=pl.ANY)] * 9,
        out_specs=pl.BlockSpec(memory_space=pltpu.VMEM),
        out_shape=jax.ShapeDtypeStruct((B, D), BF16),
        scratch_shapes=[
            pltpu.VMEM((B, D), BF16),
            pltpu.VMEM((D,), BF16),
            pltpu.VMEM((D // 16, H * DH // 128, 16, 128), BF16),
            pltpu.VMEM((H * DH // 16, D // 128, 16, 128), BF16),
            pltpu.VMEM((D // 16, F // 128, 16, 128), BF16),
            pltpu.VMEM((D // 16, F // 128, 16, 128), BF16),
            pltpu.VMEM((F // 16, D // 128, 16, 128), BF16),
            pltpu.VMEM((2, H * DH // 16, NJ, 16, 128), BF16),
            pltpu.VMEM((2, H * DH // 16, NJ, 16, 128), BF16),
            pltpu.VMEM((8, D), F32),
            pltpu.VMEM((8, H * DH), F32),
            pltpu.VMEM((NG, HG, W), F32),
            pltpu.VMEM((8, D), F32),
            pltpu.VMEM((1, D), F32),
            pltpu.SemaphoreType.DMA((NSEM,)),
        ],
        compiler_params=pltpu.CompilerParams(
            vmem_limit_bytes=100 * 1024 * 1024,
            disable_bounds_checks=True,
            disable_semaphore_checks=True,
        ),
    )(x, kt, vt, _tile_view(A_wq), _tile_view(A_wo), B_w_r,
      _tile_view(B_w_gate), _tile_view(B_w_up), _tile_view(B_w_down))
    return out.reshape(B, 1, D)
```

```python
import jax
import jax.numpy as jnp
from jax import lax
import jax.experimental.pallas as pl
import jax.experimental.pallas.tpu as pltpu

B, D = 4, 640
H, DH, SK = 32, 192, 4096
W = 1024
F = 1536
NJ = W // 128
HG = 8
NG = H // HG
GR = HG * DH
SR = 2 * DH
NS = H // 2
PG = HG // 2
JW0 = (SK - W) // 128
JW = 4
LN_EPS = 1e-5
SCALE = DH ** -0.5
F32 = jnp.float32
BF16 = jnp.bfloat16
U32 = jnp.uint32

V_CHUNKS = ([(g * GR, GR, 0, NJ) for g in range(NG - 1)]
            + [(s * SR, SR, 0, NJ) for s in range(NS - PG, NS - 1)]
            + [((NS - 1) * SR, SR, 0, 3), ((NS - 1) * SR, SR, 3, 3), ((NS - 1) * SR, SR, 6, 2)])
NVC = len(V_CHUNKS)

SEM_X, SEM_WR, SEM_WQ, SEM_WO, SEM_WG, SEM_WU, SEM_WD = range(7)
SEM_K = 7
SEM_V = SEM_K + 2
NSEM = SEM_V + 2 * NVC


NT = H * DH // 128
L2_PAIRS = [2] * 8
L2_T0 = [3 * sum(L2_PAIRS[:g]) for g in range(len(L2_PAIRS) + 1)]

KU = 12
KQ0 = 6
KQ = 15
VG = 3
OL = 0
EP = 2


def _l2_schedule():
    nd = D // 128
    ng = len(L2_PAIRS)
    t_d = 106
    t_x = 150
    t_soft = 270
    t_pop = 130
    t_g = 30
    t_v = 45
    a_jobs = [[('a', t) for t in range(L2_T0[g], L2_T0[g + 1]) if not KQ0 <= t < KQ0 + KQ]
              for g in range(ng)]
    mx = list(a_jobs[0])
    nxt = [g for g in range(1, ng) if a_jobs[g]]
    for g in range(ng):
        if nxt and (g == 0 or nxt[0] <= g + 1):
            mx += a_jobs[nxt.pop(0)]
        mx += [('b', g, j) for j in range(NJ)]
    es = [(g, t, k) for g in range(ng) for t in range(L2_T0[g], L2_T0[g + 1]) for k in range(EP)]
    cuts = [0, 12, 24, 32, 36, 40, 42, 44, 46, 48]
    fs = [('f', c0, c1, n) for c0, c1 in zip(cuts[:-1], cuts[1:]) for n in range(nd)]
    order, now, vpu = [('v', t) for t in range(KQ0, KQ0 + KQ)], 0, KQ * t_v
    b_end, avail, o_at = {}, [], {}

    def start(e):
        return max(vpu, b_end[e[0]] + t_soft)

    while mx or es or fs:
        while es and es[0][0] in b_end and (
                start(es[0]) + t_g <= now + t_pop or not (mx or fs[0][2] - 1 in o_at)):
            e = es.pop(0)
            st = start(e)
            gate = None
            if vpu > b_end[e[0]] + t_soft:
                cand = [j for (tt, j) in avail if tt <= st + t_g]
                gate = cand[-1] if cand else None
            order.append(('e',) + e + (gate,))
            vpu = st + t_d // EP
            if e[2] == EP - 1:
                o_at[e[1]] = vpu + t_x
        if mx:
            job = mx.pop(0)
            now += 40 if job[0] == 'a' else 24 * L2_PAIRS[job[1]]
            if job[0] == 'b' and job[2] == NJ - 1:
                b_end[job[1]] = now
        else:
            job = fs.pop(0)
            now = max(now, o_at[job[2] - 1]) + 8 * (job[2] - job[1])
        order.append(job)
        avail.append((now + t_pop, job))
    return order


def _dot(a, b):
    return jnp.dot(a, b, preferred_element_type=F32)


def _dot_nt(a, b):
    return lax.dot_general(a, b, (((1,), (1,)), ((), ())), preferred_element_type=F32)


def _ln_stats(x):
    m = jnp.mean(x, axis=-1, keepdims=True)
    c = x - m
    c2 = c * c
    part = c2[:, 0:128]
    for kt in range(1, D // 128):
        part = part + c2[:, kt * 128:(kt + 1) * 128]
    v = jnp.sum(part, axis=-1, keepdims=True) * (1.0 / D)
    r = lax.rsqrt(v + LN_EPS)
    return m, r, c * r, part


def _round(x):
    return x.astype(BF16).astype(F32)


def _kernel(x_hbm, k_hbm, v_hbm, wq_hbm, wo_hbm, wr_hbm, wg_hbm, wu_hbm, wd_hbm,
            o_ref,
            x_in, wr_in, wq_s, wo_s, wg_s, wu_s, wd_s, kbuf, vbuf,
            x_s, q1_s, p_s, out_s, wr_s, csq_s, csg_s, csu_s, wqt_s, wut_s, wgt_s,
            sems):

    def start_rows(src, dst, sem, r0, nr, j_src, j0, nj, jw):
        rows = pl.ds(r0 // 16, nr // 16)
        for par in range(2):
            for j in range(j0, j0 + nj, jw):
                n = min(jw, j0 + nj - j)
                pltpu.make_async_copy(src.at[rows, par, pl.ds(j_src + j, n)],
                                      dst.at[rows, pl.ds(j, n), pl.ds(par * 8, 8)],
                                      sems.at[sem]).start()

    def start_w(src, dst, sem, nr):
        for r0 in range(0, dst.shape[0] * 16, nr):
            start_rows(src, dst, sem, r0, nr, 0, 0, dst.shape[1], dst.shape[1])

    def wait_w(dst, sem):
        pltpu.make_async_copy(dst, dst, sems.at[sem]).wait()

    def wait_chunk(dst, sem, slot, r0, nr, j0, nj):
        view = dst.at[slot, pl.ds(r0 // 16, nr // 16), pl.ds(j0, nj)]
        pltpu.make_async_copy(view, view, sems.at[sem]).wait()

    def start_k(b, slot):
        for g in range(NG):
            start_rows(k_hbm.at[b], kbuf.at[slot], SEM_K + slot, g * GR, GR, JW0, 0, NJ, JW)

    def start_v(b, slot, c):
        r0, nr, j0, nj = V_CHUNKS[c]
        start_rows(v_hbm.at[b], vbuf.at[slot], SEM_V + slot * NVC + c, r0, nr, JW0, j0, nj, JW)

    x_cp = pltpu.make_async_copy(x_hbm, x_in, sems.at[SEM_X])
    wr_cp = pltpu.make_async_copy(wr_hbm, wr_in, sems.at[SEM_WR])
    x_cp.start()
    wr_cp.start()
    start_w(wq_hbm, wq_s, SEM_WQ, D)
    start_w(wo_hbm, wo_s, SEM_WO, 384)
    start_w(wg_hbm, wg_s, SEM_WG, D)
    start_w(wu_hbm, wu_s, SEM_WU, D)
    start_w(wd_hbm, wd_s, SEM_WD, 384)
    start_k(0, 0)
    for c in range(NVC):
        start_v(0, 0, c)

    wq_u, wo_u, wg_u, wu_u, wd_u, k_u, v_u = (
        r.bitcast(U32) for r in (wq_s, wo_s, wg_s, wu_s, wd_s, kbuf, vbuf))

    def tile(ref_u, idx, start, size):
        x = ref_u[idx[:-1] + (pl.ds(start // 16, size // 16), idx[-1])]
        return pltpu.bitcast(x.reshape(size // 2, 128), BF16)

    def proj(a, w_u, tiles, start, size):
        return jnp.concatenate([_dot(a, tile(w_u, (j,), start, size)) for j in tiles], axis=1)

    def ln_fix(z, mean, rstd, cs_s, t):
        return (z - mean * cs_s[:, t * 128:(t + 1) * 128]) * rstd

    lane8 = lax.broadcasted_iota(jnp.int32, (8, 128), 1)
    sub8 = lax.broadcasted_iota(jnp.int32, (8, 128), 0)

    def lane_sums(accs):
        vs = [jnp.broadcast_to(jnp.sum(a, axis=-1, keepdims=True), (8, 128)) for a in accs]
        bit = 8
        while len(vs) > 1:
            hi = (lane8 & bit) != 0
            vs = [jnp.where(hi, vs[i + 1], vs[i]) for i in range(0, len(vs), 2)]
            bit *= 2
        return jnp.where((lane8 & 7) == sub8, vs[0], 0.0)

    def after(true8, x, dep):
        return jnp.concatenate([jnp.where(true8, x[:, k:k + 128], dep)
                                for k in range(0, x.shape[1], 128)], axis=1)

    def vpu_tile(x, wt_s, i):
        accs = []
        for c in range(16):
            acc = wt_s[i, c * 8:(c + 1) * 8, 0:128] * x[:, 0:128]
            for kt in range(1, D // 128):
                ks = slice(kt * 128, (kt + 1) * 128)
                acc = acc + wt_s[i, c * 8:(c + 1) * 8, ks] * x[:, ks]
            accs.append(acc)
        return jnp.broadcast_to(jnp.sum(lane_sums(accs), axis=0, keepdims=True), (8, 128))

    def transpose_tiles(w_u, wt_s, t0, n):
        def body(i, c):
            for kt in range(D // 128):
                wt_s[i, :, kt * 128:(kt + 1) * 128] = (
                    tile(w_u, (t0 + i,), kt * 128, 128).astype(F32).T)
            return c
        lax.fori_loop(0, n, body, 0)

    row = lax.broadcasted_iota(jnp.int32, (HG, GR), 0)
    col = lax.broadcasted_iota(jnp.int32, (HG, GR), 1)
    diag = (col >= row * DH) & (col < (row + 1) * DH)

    def qk_lhs(qg):
        return jnp.where(diag, qg, 0.0).astype(BF16)

    def softmax(s_tiles):
        s = jnp.concatenate(s_tiles, axis=1) * SCALE
        m = jnp.max(s, axis=-1, keepdims=True)
        e = jnp.exp(s - m)
        l = jnp.sum(e, axis=-1, keepdims=True)
        return e * (1.0 / l)

    def moe(x, true8, swap):
        nf = F // 128
        xb = x.astype(BF16)
        mean, rstd, xn, part = _ln_stats(x)
        r = jnp.sum(xn * wr_s[...], axis=-1, keepdims=True)
        xl = after(true8, x, part)
        wv, wvt, wm = (wg_u, wgt_s, wu_u) if swap else (wu_u, wut_s, wg_u)
        u = [_dot(xb, tile(wv, (t,), 0, D)) for t in range(nf - KU)]
        u += [vpu_tile(x if i < VG else xl, wvt, i) for i in range(KU)]
        g = [_dot(xb, tile(wm, (t,), 0, D)) for t in range(nf)]
        if swap:
            g, u = u, g
        h = []
        for t in range(nf):
            gt = ln_fix(g[t], mean, rstd, csg_s, t)
            h.append(gt * jax.nn.sigmoid(gt) * ln_fix(u[t], mean, rstd, csu_s, t))
        dk = 3
        y = None
        for t0 in range(0, nf, dk):
            hb = jnp.concatenate(h[t0:t0 + dk], axis=1).astype(BF16)
            yt = proj(hb, wd_u, range(D // 128), t0 * 128, dk * 128)
            y = yt if y is None else yt + y
        return _round(x + (xn + y * jax.nn.sigmoid(r)))

    x_cp.wait()
    wr_cp.wait()
    wr_s[...] = wr_in[...].astype(F32).reshape(1, D)
    x_s[...] = jnp.zeros_like(x_s)
    x_s[0:B, :] = x_in[...].astype(F32)
    out_s[...] = jnp.zeros_like(out_s)
    xn0 = _ln_stats(x_s[...])[2]
    ones = jnp.ones((8, D), F32)
    wait_w(wq_s, SEM_WQ)
    z = proj(jnp.concatenate([xn0, ones], axis=0).astype(BF16), wq_u, range(H * DH // 128), 0, D)
    q1_s[...] = z[0:8]
    csq_s[...] = z[8:16]
    transpose_tiles(wq_u, wqt_s, KQ0, KQ)
    wait_w(wo_s, SEM_WO)
    wait_w(wg_s, SEM_WG)
    wait_w(wu_s, SEM_WU)
    csg_s[...] = proj(ones.astype(BF16), wg_u, range(F // 128), 0, D)
    csu_s[...] = proj(ones.astype(BF16), wu_u, range(F // 128), 0, D)
    transpose_tiles(wu_u, wut_s, F // 128 - KU, KU)
    transpose_tiles(wg_u, wgt_s, F // 128 - KU, KU)
    wait_w(wd_s, SEM_WD)

    srow = lax.broadcasted_iota(jnp.int32, (HG, SR), 0)
    scol = lax.broadcasted_iota(jnp.int32, (HG, SR), 1)
    shead = srow - (scol >= DH).astype(jnp.int32)

    def batch_body(b, carry):
        slot = b % 2
        more = b + 1 < B

        def wait_v(c):
            wait_chunk(vbuf, SEM_V + slot * NVC + c, slot, *V_CHUNKS[c])

            @pl.when(more)
            def _():
                start_v(b + 1, 1 - slot, c)

        wait_chunk(kbuf, SEM_K + slot, slot, 0, H * DH, 0, NJ)

        @pl.when(more)
        def _():
            start_k(b + 1, 1 - slot)

        def qk1(g, c):
            off = pl.multiple_of(g * GR, GR)
            qg = jnp.broadcast_to(q1_s[pl.ds(b, 1), pl.ds(off, GR)], (HG, GR))
            lhs = qk_lhs(qg)
            p_s[g] = softmax([_dot(lhs, tile(k_u, (slot, j), off, GR)) for j in range(NJ)])
            return c
        lax.fori_loop(0, NG, qk1, 0)

        def pv_tiles(pb, off, js):
            o = None
            for j in js:
                t = _dot_nt(pb[:, j * 128:(j + 1) * 128], tile(v_u, (slot, j), off, SR))
                o = t if o is None else o + t
            return o

        def wo_pair(o, s, off):
            o = jnp.where(shead == 2 * (s % PG), o, 0.0).astype(BF16)
            return proj(o, wo_u, range(D // 128), off, SR)

        def pv1(s, y):
            for c in range(NVC - 3):
                @pl.when(s == V_CHUNKS[c][0] // SR)
                def _():
                    wait_v(c)
            off = pl.multiple_of(s * SR, SR)
            pb = p_s[s // PG].astype(BF16)
            return y + wo_pair(pv_tiles(pb, off, range(NJ)), s, off)
        y1 = lax.fori_loop(0, NS - 1, pv1, jnp.zeros((HG, D), F32))

        off = (NS - 1) * SR
        pb = p_s[NG - 1].astype(BF16)
        o = None
        for c in range(NVC - 3, NVC):
            wait_v(c)
            t = pv_tiles(pb, off, range(V_CHUNKS[c][2], V_CHUNKS[c][2] + V_CHUNKS[c][3]))
            o = t if o is None else o + t
        y1 = y1 + wo_pair(o, NS - 1, off)

        x0 = jnp.broadcast_to(x_s[pl.ds(b, 1), :], (HG, D))
        x1 = _round(x0 + jnp.sum(y1, axis=0, keepdims=True))
        true8 = (srow[:, 0:128] + b) >= 0
        x2 = moe(x1, true8, False)

        lhs2 = x2.astype(BF16)
        mean2, rstd2, _, part2 = _ln_stats(x2)
        nd = D // 128
        q_t, s_t, p_g, pj_h, o_t, il_h = {}, {}, {}, {}, {}, {}
        y_tiles = [jnp.where(srow[:, 0:128] == 0, x2[:, n * 128:(n + 1) * 128], 0.0)
                   for n in range(nd)]
        res = {}
        x2l = after(true8, x2, part2)
        lhs_g = {}

        def job_a(job, t):
            res[job] = _dot(lhs2, tile(wq_u, (t,), 0, D))
            q_t[t] = ln_fix(res[job], mean2, rstd2, csq_s, t)

        def job_v(job, t):
            q_t[t] = ln_fix(vpu_tile(x2 if t - KQ0 < VG else x2l, wqt_s, t - KQ0), mean2, rstd2, csq_s, t)

        def job_b(job, g, j):
            t0, t1 = L2_T0[g], L2_T0[g + 1]
            if g not in lhs_g:
                q = jnp.concatenate([q_t[t] for t in range(t0, t1)], axis=1)
                lhs_g[g] = jnp.where(diag[:, 0:(t1 - t0) * 128], q, 0.0).astype(BF16)
            res[job] = s_t[g, j] = _dot(lhs_g[g], tile(k_u, (slot, j), t0 * 128, (t1 - t0) * 128))

        acc_t = {}
        JG = 7

        def job_e(job, g, t, part, gate):
            if g not in p_g:
                sc = jnp.concatenate([s_t[g, j] for j in range(NJ)], axis=1) * SCALE
                e = jnp.exp(sc - jnp.max(sc, axis=-1, keepdims=True))
                il = 1.0 / jnp.sum(e, axis=-1, keepdims=True)
                p_g[g] = (e, jnp.broadcast_to(il, (8, 128)))
            e, il = p_g[g]
            accs = acc_t.setdefault(t, [])
            gated = {}
            for c in range(part * 8 // EP, (part + 1) * 8 // EP):
                r = t * 128 + c * 16
                m = r // DH - L2_T0[g] * 128 // DH
                if (g, m) not in pj_h:
                    pj_h[g, m] = [jnp.broadcast_to(e[m:m + 1, j * 128:(j + 1) * 128], (8, 128))
                                  for j in range(NJ)]
                    il_h[g, m] = jnp.broadcast_to(il[m:m + 1, :], (8, 128))
                pj = list(pj_h[g, m])
                if gate is not None:
                    if m not in gated:
                        gated[m] = jnp.where(true8, pj[JG], res[gate])
                        if OL and part == EP - 1 and t - OL in o_t:
                            gated[m] = jnp.where(true8, gated[m], o_t[t - OL])
                    pj[JG] = gated[m]
                pj = [jnp.concatenate([x, x], axis=0) for x in pj]
                acc = tile(v_u, (slot, 0), r, 16).astype(F32) * pj[0]
                for j in range(1, NJ):
                    acc = acc + tile(v_u, (slot, j), r, 16).astype(F32) * pj[j]
                accs += [acc[0:8], acc[8:16]]
            if part == EP - 1:
                m0 = t * 128 // DH - L2_T0[g] * 128 // DH
                scale = il_h[g, m0]
                if t % 3 == 1:
                    scale = jnp.where(lane8 < 64, scale, il_h[g, m0 + 1])
                o_t[t] = lane_sums(accs) * scale

        def job_f(job, t0, t1, n):
            o = jnp.concatenate([o_t[t] for t in range(t0, t1)], axis=1).astype(BF16)
            y = _dot(o, tile(wo_u, (n,), t0 * 128, (t1 - t0) * 128))
            res[job] = y_tiles[n] = y + y_tiles[n]

        for job in _l2_schedule():
            {'a': job_a, 'v': job_v, 'b': job_b, 'e': job_e, 'f': job_f}[job[0]](job, *job[1:])

        x3 = _round(jnp.broadcast_to(jnp.sum(jnp.concatenate(y_tiles, axis=1), axis=0, keepdims=True), (8, D)))
        x4 = moe(x3, true8, True)
        out_s[pl.ds(b, 1), :] = x4[0:1, :]
        return carry

    lax.fori_loop(0, B, batch_body, 0)
    o_ref[...] = out_s[0:B, :].astype(o_ref.dtype)


def _tile_view(t):
    *lead, r, c = t.shape
    n = len(lead)
    t = t.reshape(*lead, r // 16, 2, 8, c // 128, 128)
    return t.transpose(*range(n), n, n + 1, n + 3, n + 2, n + 4)


@jax.jit
def pallas_interleave_layers__sliding_block_cached__moe_arch_mod__decode_kernel(
    A_x: jax.Array,
    A_k_cache: jax.Array,
    A_v_cache: jax.Array,
    A_wq: jax.Array,
    A_wo: jax.Array,
    B_x: jax.Array,
    B_w_r: jax.Array,
    B_w_gate: jax.Array,
    B_w_up: jax.Array,
    B_w_down: jax.Array,
):
    x = A_x.reshape(B, D)
    kt = _tile_view(jnp.swapaxes(A_k_cache, 2, 3).reshape(B, H * DH, SK))
    vt = _tile_view(jnp.swapaxes(A_v_cache, 2, 3).reshape(B, H * DH, SK))

    out = pl.pallas_call(
        _kernel,
        in_specs=[pl.BlockSpec(memory_space=pl.ANY)] * 9,
        out_specs=pl.BlockSpec(memory_space=pltpu.VMEM),
        out_shape=jax.ShapeDtypeStruct((B, D), BF16),
        scratch_shapes=[
            pltpu.VMEM((B, D), BF16),
            pltpu.VMEM((D,), BF16),
            pltpu.VMEM((D // 16, H * DH // 128, 16, 128), BF16),
            pltpu.VMEM((H * DH // 16, D // 128, 16, 128), BF16),
            pltpu.VMEM((D // 16, F // 128, 16, 128), BF16),
            pltpu.VMEM((D // 16, F // 128, 16, 128), BF16),
            pltpu.VMEM((F // 16, D // 128, 16, 128), BF16),
            pltpu.VMEM((2, H * DH // 16, NJ, 16, 128), BF16),
            pltpu.VMEM((2, H * DH // 16, NJ, 16, 128), BF16),
            pltpu.VMEM((8, D), F32),
            pltpu.VMEM((8, H * DH), F32),
            pltpu.VMEM((NG, HG, W), F32),
            pltpu.VMEM((8, D), F32),
            pltpu.VMEM((1, D), F32),
            pltpu.VMEM((8, H * DH), F32),
            pltpu.VMEM((8, F), F32),
            pltpu.VMEM((8, F), F32),
            pltpu.VMEM((max(KQ, 1), 128, D), F32),
            pltpu.VMEM((max(KU, 1), 128, D), F32),
            pltpu.VMEM((max(KU, 1), 128, D), F32),
            pltpu.SemaphoreType.DMA((NSEM,)),
        ],
        compiler_params=pltpu.CompilerParams(
            vmem_limit_bytes=100 * 1024 * 1024,
            disable_bounds_checks=True,
            disable_semaphore_checks=True,
        ),
    )(x, kt, vt, _tile_view(A_wq), _tile_view(A_wo), B_w_r,
      _tile_view(B_w_gate), _tile_view(B_w_up), _tile_view(B_w_down))
    return out.reshape(B, 1, D)
```

```python
import jax
import jax.numpy as jnp
from jax import lax
import jax.experimental.pallas as pl
import jax.experimental.pallas.tpu as pltpu

B, D = 4, 640
H, DH, SK = 32, 192, 4096
W = 1024
F = 1536
NJ = W // 128
HG = 8
NG = H // HG
GR = HG * DH
SR = 2 * DH
NS = H // 2
PG = HG // 2
JW0 = (SK - W) // 128
JW = 4
LN_EPS = 1e-5
SCALE = DH ** -0.5
F32 = jnp.float32
BF16 = jnp.bfloat16
U32 = jnp.uint32

V_CHUNKS = ([(g * GR, GR, 0, NJ) for g in range(NG - 1)]
            + [(s * SR, SR, 0, NJ) for s in range(NS - PG, NS - 1)]
            + [((NS - 1) * SR, 256, 0, 4), ((NS - 1) * SR, 256, 4, 4),
               (H * DH - 128, 128, 0, 4), (H * DH - 128, 128, 4, 4)])
NVC = len(V_CHUNKS)

SEM_X, SEM_WR, SEM_WQ, SEM_WO, SEM_WG, SEM_WU, SEM_WD = range(7)
SEM_K = 7
SEM_V = SEM_K + 2
NSEM = SEM_V + 2 * NVC


NT = H * DH // 128
L2_PAIRS = [2, 2, 2, 2, 2, 2, 2, 2]
L2_T0 = [3 * sum(L2_PAIRS[:g]) for g in range(len(L2_PAIRS) + 1)]

KU = 12
KQ0 = 6
KQ = 19
KL = 10
VQ = list(range(KQ0, KQ0 + KQ)) + list(range(NT - KL, NT))
PAD = 1
NJF = 6
VG = 3
EP = 8


def _l2_schedule():
    nd = D // 128
    ng = len(L2_PAIRS)
    t_d = 83
    t_x = 150
    t_soft = 270
    t_pop = 130
    t_d2 = t_d
    t_g = 30
    t_v = 45
    a_jobs = [[('a', t) for t in range(L2_T0[g], L2_T0[g + 1]) if t not in VQ]
              for g in range(ng)]
    mx = list(a_jobs[0])
    nxt = [g for g in range(1, ng) if a_jobs[g]]
    for g in range(ng):
        if nxt and (g == 0 or nxt[0] <= g + 1):
            mx += a_jobs[nxt.pop(0)]
        mx += [('b', g, j) for j in range(NJ)]
    es = [(g, t, k) for g in range(ng) for t in range(L2_T0[g], L2_T0[g + 1]) for k in range(EP)]
    cuts = [0, 2, 4, 6, 8, 10, 12, 14, 16, 18, 20, 22, 24, 26, 28, 30, 32, 34, 36, 38, 40, 42, 44, 46, 48]
    fs = [('f', c0, c1, n) for c0, c1 in zip(cuts[:-1], cuts[1:]) for n in range(nd)]
    order, now, vpu = [('v', t, None) for t in range(KQ0, KQ0 + KQ)], 0, KQ * t_v
    every = 16
    for i, t in enumerate(range(NT - KL, NT)):
        pos = 2 + i * (every + 1)
        es.insert(pos, (es[pos][0], t, 'v'))
    b_end, avail, o_at = {}, [], {}
    lead = 300

    def start(e):
        return max(vpu, b_end[e[0]] + t_soft)

    def cost(job):
        return {'a': 40, 'b': 24 * L2_PAIRS[job[1]] if job[0] == 'b' else 0,
                'f': 8 * (job[2] - job[1]) if job[0] == 'f' else 0}[job[0]]

    def urgent(extra):
        t = now + extra
        for job in mx:
            t += cost(job)
            if job[0] == 'b' and job[2] == NJ - 1:
                n_before = sum(1 for e in es if e[0] < job[1])
                if t + t_soft + lead > vpu + n_before * (t_d / EP):
                    return True
        return False

    while mx or es or fs:
        while es and es[0][0] in b_end and (
                start(es[0]) + t_g <= now + t_pop or not (mx or fs[0][2] - 1 in o_at)):
            e = es.pop(0)
            st = start(e)
            gate = None
            if vpu > b_end[e[0]] + t_soft:
                cand = [j for (tt, j) in avail if tt <= st + t_g]
                gate = cand[-1] if cand else None
            if e[2] == 'v':
                order.append(('v', e[1], gate))
                vpu = st + 45
                continue
            order.append(('e',) + e + (gate,))
            vpu = st + (t_d if mx else t_d2) / EP
            if e[2] == EP - 1:
                o_at[e[1]] = vpu + t_x
        f_ready = fs and o_at.get(fs[0][2] - 1, 1 << 30) <= now
        if mx and not (f_ready and not urgent(cost(fs[0]))):
            job = mx.pop(0)
            now += cost(job)
            if job[0] == 'b' and job[2] == NJ - 1:
                b_end[job[1]] = now
        else:
            job = fs.pop(0)
            now = max(now, o_at[job[2] - 1]) + cost(job)
        order.append(job)
        avail.append((now + t_pop, job))
    return order


def _dot(a, b):
    return jnp.dot(a, b, preferred_element_type=F32)


def _dot_nt(a, b):
    return lax.dot_general(a, b, (((1,), (1,)), ((), ())), preferred_element_type=F32)


def _ln_stats(x):
    m = jnp.mean(x, axis=-1, keepdims=True)
    c = x - m
    c2 = c * c
    part = c2[:, 0:128]
    for kt in range(1, D // 128):
        part = part + c2[:, kt * 128:(kt + 1) * 128]
    v = jnp.sum(part, axis=-1, keepdims=True) * (1.0 / D)
    r = lax.rsqrt(v + LN_EPS)
    return m, r, c * r, part


def _round(x):
    return x.astype(BF16).astype(F32)


def _kernel(x_hbm, k_hbm, v_hbm, wq_hbm, wo_hbm, wr_hbm, wg_hbm, wu_hbm, wd_hbm,
            o_ref,
            x_in, wr_in, wq_s, wo_s, wg_s, wu_s, wd_s, kbuf, vbuf,
            x_s, q1_s, p_s, out_s, wr_s, csq_s, csg_s, csu_s, wqt_s, wut_s, wgt_s, vf_s,
            sems):

    def start_rows(src, dst, sem, r0, nr, j_src, j0, nj, jw):
        rows = pl.ds(r0 // 16, nr // 16)
        for par in range(2):
            for j in range(j0, j0 + nj, jw):
                n = min(jw, j0 + nj - j)
                pltpu.make_async_copy(src.at[rows, par, pl.ds(j_src + j, n)],
                                      dst.at[rows, pl.ds(j, n), pl.ds(par * 8, 8)],
                                      sems.at[sem]).start()

    def start_w(src, dst, sem, nr):
        for r0 in range(0, dst.shape[0] * 16, nr):
            start_rows(src, dst, sem, r0, nr, 0, 0, src.shape[2], src.shape[2])

    def wait_w(src, dst, sem):
        view = dst.at[:, pl.ds(0, src.shape[2])]
        pltpu.make_async_copy(view, view, sems.at[sem]).wait()

    def wait_chunk(dst, sem, slot, r0, nr, j0, nj):
        view = dst.at[slot, pl.ds(r0 // 16, nr // 16), pl.ds(j0, nj)]
        pltpu.make_async_copy(view, view, sems.at[sem]).wait()

    def start_k(b, slot):
        for g in range(NG):
            start_rows(k_hbm.at[b], kbuf.at[slot], SEM_K + slot, g * GR, GR, JW0, 0, NJ, JW)

    def start_v(b, slot, c):
        r0, nr, j0, nj = V_CHUNKS[c]
        start_rows(v_hbm.at[b], vbuf.at[slot], SEM_V + slot * NVC + c, r0, nr, JW0, j0, nj, JW)

    x_cp = pltpu.make_async_copy(x_hbm, x_in, sems.at[SEM_X])
    wr_cp = pltpu.make_async_copy(wr_hbm, wr_in, sems.at[SEM_WR])
    start_w(wq_hbm, wq_s, SEM_WQ, D)
    x_cp.start()
    wr_cp.start()
    start_w(wo_hbm, wo_s, SEM_WO, 384)
    start_w(wg_hbm, wg_s, SEM_WG, D)
    start_w(wu_hbm, wu_s, SEM_WU, D)
    start_w(wd_hbm, wd_s, SEM_WD, 384)
    start_k(0, 0)
    for c in range(NVC):
        start_v(0, 0, c)

    wq_u, wo_u, wg_u, wu_u, wd_u, k_u, v_u = (
        r.bitcast(U32) for r in (wq_s, wo_s, wg_s, wu_s, wd_s, kbuf, vbuf))

    def tile(ref_u, idx, start, size):
        x = ref_u[idx[:-1] + (pl.ds(start // 16, size // 16), idx[-1])]
        return pltpu.bitcast(x.reshape(size // 2, 128), BF16)

    def proj(a, w_u, tiles, start, size):
        return jnp.concatenate([_dot(a, tile(w_u, (j,), start, size)) for j in tiles], axis=1)

    def ln_fix(z, mean, rstd, cs_s, t):
        return (z - mean * cs_s[:, t * 128:(t + 1) * 128]) * rstd

    lane8 = lax.broadcasted_iota(jnp.int32, (8, 128), 1)
    sub8 = lax.broadcasted_iota(jnp.int32, (8, 128), 0)

    def lane_sums(accs):
        vs = [jnp.broadcast_to(jnp.sum(a, axis=-1, keepdims=True), (8, 128)) for a in accs]
        bit = 8
        while len(vs) > 1:
            hi = (lane8 & bit) != 0
            vs = [jnp.where(hi, vs[i + 1], vs[i]) for i in range(0, len(vs), 2)]
            bit *= 2
        return jnp.where((lane8 & 7) == sub8, vs[0], 0.0)

    def after(true8, x, dep):
        return jnp.concatenate([jnp.where(true8, x[:, k:k + 128], dep)
                                for k in range(0, x.shape[1], 128)], axis=1)

    def vpu_tile(x, wt_s, i):
        accs = []
        for c in range(16):
            acc = wt_s[i, c * 8:(c + 1) * 8, 0:128] * x[:, 0:128]
            for kt in range(1, D // 128):
                ks = slice(kt * 128, (kt + 1) * 128)
                acc = acc + wt_s[i, c * 8:(c + 1) * 8, ks] * x[:, ks]
            accs.append(acc)
        return jnp.broadcast_to(jnp.sum(lane_sums(accs), axis=0, keepdims=True), (8, 128))

    def transpose_tiles(w_u, wt_s, t0, n, i0=0):
        def body(i, c):
            for kt in range(D // 128):
                wt_s[i0 + i, :, kt * 128:(kt + 1) * 128] = (
                    tile(w_u, (t0 + i,), kt * 128, 128).astype(F32).T)
            return c
        lax.fori_loop(0, n, body, 0)

    row = lax.broadcasted_iota(jnp.int32, (HG, GR), 0)
    col = lax.broadcasted_iota(jnp.int32, (HG, GR), 1)
    diag = (col >= row * DH) & (col < (row + 1) * DH)

    def qk_lhs(qg):
        return jnp.where(diag, qg, 0.0).astype(BF16)

    def softmax(s_tiles):
        s = jnp.concatenate(s_tiles, axis=1) * SCALE
        m = jnp.max(s, axis=-1, keepdims=True)
        e = jnp.exp(s - m)
        l = jnp.sum(e, axis=-1, keepdims=True)
        return e * (1.0 / l)

    def moe(x, true8, swap):
        nf = F // 128
        xb = x.astype(BF16)
        mean, rstd, xn, part = _ln_stats(x)
        r = jnp.sum(xn * wr_s[...], axis=-1, keepdims=True)
        xl = after(true8, x, part)
        wv, wvt, wm = (wg_u, wgt_s, wu_u) if swap else (wu_u, wut_s, wg_u)
        u = [_dot(xb, tile(wv, (t,), 0, D)) for t in range(nf - KU)]
        u += [vpu_tile(x if i < VG else xl, wvt, i) for i in range(KU)]
        g = [_dot(xb, tile(wm, (t,), 0, D)) for t in range(nf)]
        if swap:
            g, u = u, g
        h = []
        for t in range(nf):
            gt = ln_fix(g[t], mean, rstd, csg_s, t)
            h.append(gt * jax.nn.sigmoid(gt) * ln_fix(u[t], mean, rstd, csu_s, t))
        dk = 3
        y = None
        for t0 in range(0, nf, dk):
            hb = jnp.concatenate(h[t0:t0 + dk], axis=1).astype(BF16)
            yt = proj(hb, wd_u, range(D // 128), t0 * 128, dk * 128)
            y = yt if y is None else yt + y
        return _round(x + (xn + y * jax.nn.sigmoid(r)))

    x_cp.wait()
    wr_cp.wait()
    wr_s[...] = wr_in[...].astype(F32).reshape(1, D)
    x_s[...] = jnp.zeros_like(x_s)
    x_s[0:B, :] = x_in[...].astype(F32)
    out_s[...] = jnp.zeros_like(out_s)
    xn0 = _ln_stats(x_s[...])[2]
    ones = jnp.ones((8, D), F32)
    wait_w(wq_hbm, wq_s, SEM_WQ)
    z = proj(jnp.concatenate([xn0, ones], axis=0).astype(BF16), wq_u, range(H * DH // 128), 0, D)
    q1_s[...] = z[0:8]
    csq_s[...] = z[8:16]
    transpose_tiles(wq_u, wqt_s, KQ0, KQ)
    transpose_tiles(wq_u, wqt_s, NT - KL, KL, KQ)
    wait_w(wo_hbm, wo_s, SEM_WO)
    wait_w(wg_hbm, wg_s, SEM_WG)
    wait_w(wu_hbm, wu_s, SEM_WU)
    csg_s[...] = proj(ones.astype(BF16), wg_u, range(F // 128), 0, D)
    csu_s[...] = proj(ones.astype(BF16), wu_u, range(F // 128), 0, D)
    transpose_tiles(wu_u, wut_s, F // 128 - KU, KU)
    transpose_tiles(wg_u, wgt_s, F // 128 - KU, KU)
    wait_w(wd_hbm, wd_s, SEM_WD)

    srow = lax.broadcasted_iota(jnp.int32, (HG, SR), 0)
    scol = lax.broadcasted_iota(jnp.int32, (HG, SR), 1)
    shead = srow - (scol >= DH).astype(jnp.int32)

    def batch_body(b, carry):
        slot = b % 2
        more = b + 1 < B

        def wait_v(c):
            wait_chunk(vbuf, SEM_V + slot * NVC + c, slot, *V_CHUNKS[c])

            if c < NVC - 1:
                @pl.when(more)
                def _():
                    start_v(b + 1, 1 - slot, c)
                    if c == NVC - 2:
                        start_v(b + 1, 1 - slot, c + 1)

        wait_chunk(kbuf, SEM_K + slot, slot, 0, H * DH, 0, NJ)

        @pl.when(more)
        def _():
            start_k(b + 1, 1 - slot)

        def qk1(g, c):
            off = pl.multiple_of(g * GR, GR)
            qg = jnp.broadcast_to(q1_s[pl.ds(b, 1), pl.ds(off, GR)], (HG, GR))
            lhs = qk_lhs(qg)
            p_s[g] = softmax([_dot(lhs, tile(k_u, (slot, j), off, GR)) for j in range(NJ)])
            return c
        lax.fori_loop(0, NG, qk1, 0)

        def v_tile(j, off, nr, keep):
            vj = tile(v_u, (slot, j), off, nr)
            if keep:
                vf_s[pl.ds(off // 16, nr // 16), j] = vj.astype(F32).reshape(nr // 16, 16, 128)
            return vj

        def pv_tiles(pb, off, nr, js):
            o = None
            for j in js:
                t = _dot_nt(pb[:, j * 128:(j + 1) * 128], v_tile(j, off, nr, j < NJF))
                o = t if o is None else o + t
            return o

        def wo_pair(o, s, off, nr):
            o = jnp.where(shead[:, 0:nr] == 2 * (s % PG), o, 0.0).astype(BF16)
            return proj(o, wo_u, range(D // 128), off, nr)

        def pv1(s, y):
            for c in range(NVC - 4):
                @pl.when(s == V_CHUNKS[c][0] // SR)
                def _():
                    wait_v(c)
            off = pl.multiple_of(s * SR, SR)
            pb = p_s[s // PG].astype(BF16)
            return y + wo_pair(pv_tiles(pb, off, SR, range(NJ)), s, off, SR)
        y1 = lax.fori_loop(0, NS - 1, pv1, jnp.zeros((HG, D), F32))

        off = (NS - 1) * SR
        pb = p_s[NG - 1].astype(BF16)
        wait_v(NVC - 4)
        o = pv_tiles(pb, off, 256, range(0, 4))
        wait_v(NVC - 3)
        o = o + pv_tiles(pb, off, 256, range(4, NJ))

        off = H * DH - 128
        acc = None
        for c in (NVC - 2, NVC - 1):
            wait_v(c)
            for j in range(V_CHUNKS[c][2], V_CHUNKS[c][2] + V_CHUNKS[c][3]):
                pj = p_s[NG - 1, HG - 1:HG, j * 128:(j + 1) * 128]
                t = v_tile(j, off, 128, j < min(NJF, 4)).astype(F32) * pj
                acc = t if acc is None else acc + t
        y1 = y1 + wo_pair(o, NS - 1, (NS - 1) * SR, 256)
        oc = jnp.sum(acc, axis=-1, keepdims=True)
        yv = [(tile(wo_u, (n,), off, 128).astype(F32) * oc).reshape(16, 8, 128).sum(axis=0)
              for n in range(D // 128)]
        y1 = y1 + jnp.concatenate(yv, axis=1)

        x0 = jnp.broadcast_to(x_s[pl.ds(b, 1), :], (HG, D))
        x1 = _round(x0 + jnp.sum(y1, axis=0, keepdims=True))
        true8 = (srow[:, 0:128] + b) >= 0
        x2 = moe(x1, true8, False)

        lhs2 = x2.astype(BF16)
        mean2, rstd2, _, part2 = _ln_stats(x2)
        nd = D // 128
        q_t, s_t, p_g, pj_h, o_t, il_h = {}, {}, {}, {}, {}, {}
        y_tiles = [jnp.where(srow[:, 0:128] == 0, x2[:, n * 128:(n + 1) * 128], 0.0)
                   for n in range(nd)]
        res = {}
        x2l = after(true8, x2, part2)
        lhs_g = {}

        def job_a(job, t):
            res[job] = _dot(lhs2, tile(wq_u, (t,), 0, D))
            q_t[t] = ln_fix(res[job], mean2, rstd2, csq_s, t)

        def job_v(job, t, gate):
            i = VQ.index(t)
            xv = x2 if i < VG else x2l
            if gate is not None:
                xv = jnp.concatenate([x2[:, 0:D - 128], after(true8, x2[:, D - 128:], res[gate])],
                                     axis=1)
            q_t[t] = ln_fix(vpu_tile(xv, wqt_s, i), mean2, rstd2, csq_s, t)

        def job_b(job, g, j):
            t0, t1 = L2_T0[g], L2_T0[g + 1]
            if g not in lhs_g:
                q = jnp.concatenate([q_t[t] for t in range(t0, t1)], axis=1)
                lhs_g[g] = jnp.where(diag[:, 0:(t1 - t0) * 128], q, 0.0).astype(BF16)
            res[job] = s_t[g, j] = _dot(lhs_g[g], tile(k_u, (slot, j), t0 * 128, (t1 - t0) * 128))

        acc_t = {}
        JG = 7

        def job_e(job, g, t, part, gate):
            if g not in p_g:
                sc = jnp.concatenate([s_t[g, j] for j in range(NJ)], axis=1) * SCALE
                e = jnp.exp(sc - jnp.max(sc, axis=-1, keepdims=True))
                il = 1.0 / jnp.sum(e, axis=-1, keepdims=True)
                p_g[g] = (e, jnp.broadcast_to(il, (8, 128)))
            e, il = p_g[g]
            accs = acc_t.setdefault(t, [])
            gated = {}
            for c in range(part * 8 // EP, (part + 1) * 8 // EP):
                r = t * 128 + c * 16
                m = r // DH - L2_T0[g] * 128 // DH
                if (g, m) not in pj_h:
                    pj_h[g, m] = [jnp.broadcast_to(e[m:m + 1, j * 128:(j + 1) * 128], (8, 128))
                                  for j in range(NJ)]
                    il_h[g, m] = jnp.broadcast_to(il[m:m + 1, :], (8, 128))
                pj = list(pj_h[g, m])
                if gate is not None:
                    if m not in gated:
                        gated[m] = jnp.where(true8, pj[JG], res[gate])
                    pj[JG] = gated[m]
                pj = [jnp.concatenate([x, x], axis=0) for x in pj]
                acc = None
                for j in range(NJ):
                    if j < (NJF if t < NT - 1 else min(NJF, 4)):
                        vj = vf_s[r // 16, j]
                    else:
                        vj = tile(v_u, (slot, j), r, 16).astype(F32)
                    acc = vj * pj[j] if acc is None else acc + vj * pj[j]
                accs += [acc[0:8], acc[8:16]]
            if part == EP - 1:
                m0 = t * 128 // DH - L2_T0[g] * 128 // DH
                scale = il_h[g, m0]
                if t % 3 == 1:
                    scale = jnp.where(lane8 < 64, scale, il_h[g, m0 + 1])
                o_t[t] = lane_sums(accs) * scale

        def job_f(job, t0, t1, n):
            o = jnp.concatenate([o_t[t] for t in range(t0, t1)], axis=1).astype(BF16)
            y = _dot(o, tile(wo_u, (n,), t0 * 128, (t1 - t0) * 128))
            res[job] = y_tiles[n] = y + y_tiles[n]

        for job in _l2_schedule():
            {'a': job_a, 'v': job_v, 'b': job_b, 'e': job_e, 'f': job_f}[job[0]](job, *job[1:])

        x3 = _round(jnp.broadcast_to(jnp.sum(jnp.concatenate(y_tiles, axis=1), axis=0, keepdims=True), (8, D)))
        x4 = moe(x3, true8, True)
        out_s[pl.ds(b, 1), :] = x4[0:1, :]
        return carry

    lax.fori_loop(0, B, batch_body, 0)
    o_ref[...] = out_s[0:B, :].astype(o_ref.dtype)


def _tile_view(t):
    *lead, r, c = t.shape
    n = len(lead)
    t = t.reshape(*lead, r // 16, 2, 8, c // 128, 128)
    return t.transpose(*range(n), n, n + 1, n + 3, n + 2, n + 4)


@jax.jit
def pallas_interleave_layers__sliding_block_cached__moe_arch_mod__decode_kernel(
    A_x: jax.Array,
    A_k_cache: jax.Array,
    A_v_cache: jax.Array,
    A_wq: jax.Array,
    A_wo: jax.Array,
    B_x: jax.Array,
    B_w_r: jax.Array,
    B_w_gate: jax.Array,
    B_w_up: jax.Array,
    B_w_down: jax.Array,
):
    x = A_x.reshape(B, D)
    kt = _tile_view(jnp.swapaxes(A_k_cache, 2, 3).reshape(B, H * DH, SK))
    vt = _tile_view(jnp.swapaxes(A_v_cache, 2, 3).reshape(B, H * DH, SK))

    out = pl.pallas_call(
        _kernel,
        in_specs=[pl.BlockSpec(memory_space=pl.ANY)] * 9,
        out_specs=pl.BlockSpec(memory_space=pltpu.VMEM),
        out_shape=jax.ShapeDtypeStruct((B, D), BF16),
        scratch_shapes=[
            pltpu.VMEM((B, D), BF16),
            pltpu.VMEM((D,), BF16),
            pltpu.VMEM((D // 16, H * DH // 128 + PAD, 16, 128), BF16),
            pltpu.VMEM((H * DH // 16, D // 128, 16, 128), BF16),
            pltpu.VMEM((D // 16, F // 128 + PAD, 16, 128), BF16),
            pltpu.VMEM((D // 16, F // 128 + PAD, 16, 128), BF16),
            pltpu.VMEM((F // 16, D // 128, 16, 128), BF16),
            pltpu.VMEM((2, H * DH // 16, NJ + PAD, 16, 128), BF16),
            pltpu.VMEM((2, H * DH // 16, NJ, 16, 128), BF16),
            pltpu.VMEM((8, D), F32),
            pltpu.VMEM((8, H * DH), F32),
            pltpu.VMEM((NG, HG, W), F32),
            pltpu.VMEM((8, D), F32),
            pltpu.VMEM((1, D), F32),
            pltpu.VMEM((8, H * DH), F32),
            pltpu.VMEM((8, F), F32),
            pltpu.VMEM((8, F), F32),
            pltpu.VMEM((max(KQ + KL, 1), 128, D), F32),
            pltpu.VMEM((max(KU, 1), 128, D), F32),
            pltpu.VMEM((max(KU, 1), 128, D), F32),
            pltpu.VMEM((H * DH // 16, max(NJF, 1), 16, 128), F32),
            pltpu.SemaphoreType.DMA((NSEM,)),
        ],
        compiler_params=pltpu.CompilerParams(
            vmem_limit_bytes=116 * 1024 * 1024,
            disable_bounds_checks=True,
            disable_semaphore_checks=True,
        ),
    )(x, kt, vt, _tile_view(A_wq), _tile_view(A_wo), B_w_r,
      _tile_view(B_w_gate), _tile_view(B_w_up), _tile_view(B_w_down))
    return out.reshape(B, 1, D)
```

```python
import jax
import jax.numpy as jnp
from jax import lax
import jax.experimental.pallas as pl
import jax.experimental.pallas.tpu as pltpu

B, D = 4, 640
H, DH, SK = 32, 192, 4096
W = 1024
F = 1536
NJ = W // 128
ND = D // 128
NF = F // 128
NT = H * DH // 128
HG = 8
NG = H // HG
GR = HG * DH
SR = 2 * DH
NS = H // 2
PG = HG // 2
JW0 = (SK - W) // 128
JW = 4
LN_EPS = 1e-5
SCALE = DH ** -0.5
F32 = jnp.float32
BF16 = jnp.bfloat16
U32 = jnp.uint32

V_CHUNKS = ([(g * GR, GR, 0, NJ) for g in range(NG - 1)]
            + [(s * SR, SR, 0, NJ) for s in range(NS - PG, NS - 1)]
            + [((NS - 1) * SR, 256, 0, 4), ((NS - 1) * SR, 256, 4, 4),
               (H * DH - 128, 128, 0, 4), (H * DH - 128, 128, 4, 4)])
NVC = len(V_CHUNKS)

SEM_X, SEM_WR, SEM_WQ, SEM_WO, SEM_WG, SEM_WU, SEM_WD = range(7)
SEM_K = 7
SEM_V = SEM_K + 2
NSEM = SEM_V + 2 * NVC

GT = 6
NG2 = NT // GT
KQ0, KQ, KL = 6, 19, 10
VQ = list(range(KQ0, KQ0 + KQ)) + list(range(NT - KL, NT))
NJF = 6
FV = 3
VG = 4
DK = 3


def _l2_schedule():
    t_e, t_v = 83 / 8, 45
    t_x, t_soft, t_pop, lead = 150, 270, 130, 300
    a_jobs = [[('a', t) for t in range(g * GT, (g + 1) * GT) if t not in VQ] for g in range(NG2)]
    mx = list(a_jobs[0])
    nxt = [g for g in range(1, NG2) if a_jobs[g]]
    for g in range(NG2):
        if nxt and (g == 0 or nxt[0] <= g + 1):
            mx += a_jobs[nxt.pop(0)]
        mx += [('b', g, j) for j in range(NJ)]
    es = [(t // GT, t, c) for t in range(NT) for c in range(8)]
    for i, t in enumerate(range(NT - KL, NT)):
        es.insert(2 + i * 17, (es[2 + i * 17][0], t, 'v'))
    cuts = list(range(0, NT - FV, 2)) + [NT - FV]
    fs = [('f', c0, c1, n) for c0, c1 in zip(cuts[:-1], cuts[1:]) for n in range(ND)]
    order, now, vpu = [('v', t, None) for t in range(KQ0, KQ0 + KQ)], 0, KQ * t_v
    b_end, avail, o_at = {}, [], {}

    def start(e):
        return max(vpu, b_end[e[0]] + t_soft)

    def cost(job):
        return 40 if job[0] == 'a' else 8 * GT if job[0] == 'b' else 8 * (job[2] - job[1])

    def urgent(extra):
        t = now + extra
        for job in mx:
            t += cost(job)
            if job[0] == 'b' and job[2] == NJ - 1:
                n_before = sum(1 for e in es if e[0] < job[1])
                if t + t_soft + lead > vpu + n_before * t_e:
                    return True
        return False

    while mx or es or fs:
        while es and es[0][0] in b_end and (
                start(es[0]) <= now + t_pop or not (mx or (fs and fs[0][2] - 1 in o_at))):
            e = es.pop(0)
            st = start(e)
            gate = None
            if vpu > b_end[e[0]] + t_soft:
                gate = [j for (tt, j) in avail if tt <= st][-1]
            if e[2] == 'v':
                order.append(('v', e[1], gate))
                vpu = st + t_v
                continue
            prev = order[-1]
            if (prev[0] == 'e' and prev[2] == e[1] and prev[5] == gate
                    and not (e[1] % 3 == 1 and e[2] == 4)):
                order[-1] = prev[:4] + (e[2] + 1, gate)
            else:
                order.append(('e', e[0], e[1], e[2], e[2] + 1, gate))
            vpu = st + t_e
            if e[2] == 7:
                o_at[e[1]] = vpu + t_x
        if not (mx or fs):
            continue
        f_ready = fs and o_at.get(fs[0][2] - 1, 1 << 30) <= now
        if mx and not (f_ready and not urgent(cost(fs[0]))):
            job = mx.pop(0)
            now += cost(job)
            if job[0] == 'b' and job[2] == NJ - 1:
                b_end[job[1]] = now
        else:
            job = fs.pop(0)
            now = max(now, o_at[job[2] - 1]) + cost(job)
        order.append(job)
        avail.append((now + t_pop, job))
    return order


def _dot(a, b):
    return jnp.dot(a, b, preferred_element_type=F32)


def _dot_nt(a, b):
    return lax.dot_general(a, b, (((1,), (1,)), ((), ())), preferred_element_type=F32)


def _round(x):
    return x.astype(BF16).astype(F32)


def _ln_stats(x):
    m = jnp.mean(x, axis=-1, keepdims=True)
    c = x - m
    c2 = c * c
    part = c2[:, 0:128]
    for kt in range(1, ND):
        part = part + c2[:, kt * 128:(kt + 1) * 128]
    v = jnp.sum(part, axis=-1, keepdims=True) * (1.0 / D)
    m = _round(m)
    r = lax.rsqrt(v + LN_EPS)
    return m, r, (x - m) * r, part


def _kernel(x_hbm, k_hbm, v_hbm, wq_hbm, wo_hbm, wr_hbm, wg_hbm, wu_hbm, wd_hbm,
            o_ref,
            x_in, wr_in, wq_s, wo_s, wg_s, wu_s, wd_s, kbuf, vbuf,
            x_s, q1_s, p_s, out_s, wr_s, csq_s, csg_s, csu_s, wqt_s, wut_s, wgt_s, vf_s,
            sems):
    def start_rows(src, dst, sem, r0, nr, j_src, j0, nj, jw):
        rows = pl.ds(r0 // 16, nr // 16)
        for half in range(2):
            for j in range(j0, j0 + nj, jw):
                n = min(jw, j0 + nj - j)
                pltpu.make_async_copy(src.at[rows, half, pl.ds(j_src + j, n)],
                                      dst.at[rows, pl.ds(j, n), pl.ds(half * 8, 8)],
                                      sems.at[sem]).start()

    def start_w(src, dst, sem, nr):
        for r0 in range(0, dst.shape[0] * 16, nr):
            start_rows(src, dst, sem, r0, nr, 0, 0, src.shape[2], src.shape[2])

    def wait_w(src, dst, sem):
        view = dst.at[:, pl.ds(0, src.shape[2])]
        pltpu.make_async_copy(view, view, sems.at[sem]).wait()

    def wait_chunk(dst, sem, slot, r0, nr, j0, nj):
        view = dst.at[slot, pl.ds(r0 // 16, nr // 16), pl.ds(j0, nj)]
        pltpu.make_async_copy(view, view, sems.at[sem]).wait()

    def start_k(b, slot):
        for g in range(NG):
            start_rows(k_hbm.at[b], kbuf.at[slot], SEM_K + slot, g * GR, GR, JW0, 0, NJ, JW)

    def start_v(b, slot, c):
        r0, nr, j0, nj = V_CHUNKS[c]
        start_rows(v_hbm.at[b], vbuf.at[slot], SEM_V + slot * NVC + c, r0, nr, JW0, j0, nj, JW)

    x_cp = pltpu.make_async_copy(x_hbm, x_in, sems.at[SEM_X])
    wr_cp = pltpu.make_async_copy(wr_hbm, wr_in, sems.at[SEM_WR])
    start_w(wq_hbm, wq_s, SEM_WQ, D)
    x_cp.start()
    wr_cp.start()
    start_w(wo_hbm, wo_s, SEM_WO, 384)
    start_w(wg_hbm, wg_s, SEM_WG, D)
    start_w(wu_hbm, wu_s, SEM_WU, D)
    start_w(wd_hbm, wd_s, SEM_WD, 384)
    start_k(0, 0)
    for c in range(NVC):
        start_v(0, 0, c)

    wq_u, wo_u, wg_u, wu_u, wd_u, k_u, v_u = (
        r.bitcast(U32) for r in (wq_s, wo_s, wg_s, wu_s, wd_s, kbuf, vbuf))

    def tile(ref_u, idx, start, size):
        x = ref_u[idx[:-1] + (pl.ds(start // 16, size // 16), idx[-1])]
        return pltpu.bitcast(x.reshape(size // 2, 128), BF16)

    def proj(a, w_u, tiles, start, size):
        return jnp.concatenate([_dot(a, tile(w_u, (j,), start, size)) for j in tiles], axis=1)

    def ln_fix(z, mean, rstd, cs_s, t):
        return (z - mean * cs_s[:, t * 128:(t + 1) * 128]) * rstd

    lane8 = lax.broadcasted_iota(jnp.int32, (8, 128), 1)
    sub8 = lax.broadcasted_iota(jnp.int32, (8, 128), 0)

    bits = [((lane8 & bit) != 0)[None] for bit in (8, 16, 32, 64)]
    on_diag = (lane8 & 7) == sub8

    def spread(sums):
        v = jnp.broadcast_to(sums, (16, 8, 128))
        for hi in bits:
            v = v.reshape(v.shape[0] // 2, 2, 8, 128)
            v = jnp.where(hi, v[:, 1], v[:, 0])
        return jnp.where(on_diag, v[0], 0.0)

    def after(true8, x, dep):
        return jnp.concatenate([jnp.where(true8, x[:, k:k + 128], dep)
                                for k in range(0, x.shape[1], 128)], axis=1)

    def vpu_tile(x, wt_s, i):
        sums = jnp.sum(wt_s[i].reshape(16, 8, D) * x[None], axis=-1, keepdims=True)
        return jnp.broadcast_to(jnp.sum(spread(sums), axis=0, keepdims=True), (8, 128))

    def transpose_tiles(w_u, wt_s, t0, n, i0=0):
        def body(i, c):
            for kt in range(ND):
                wt_s[i0 + i, :, kt * 128:(kt + 1) * 128] = (
                    tile(w_u, (t0 + i,), kt * 128, 128).astype(F32).T)
            return c
        lax.fori_loop(0, n, body, 0)

    row = lax.broadcasted_iota(jnp.int32, (HG, GR), 0)
    col = lax.broadcasted_iota(jnp.int32, (HG, GR), 1)
    diag = (col >= row * DH) & (col < (row + 1) * DH)

    def moe(x, true8, swap):
        xb = x.astype(BF16)
        mean, rstd, xn, part = _ln_stats(x)
        r = jnp.sum(xn * wr_s[...], axis=-1, keepdims=True)
        xl = after(true8, x, part)
        wvt, wm = (wgt_s, wu_u) if swap else (wut_s, wg_u)
        u = [vpu_tile(x if i < VG else xl, wvt, i) for i in range(NF)]
        g = [_dot(xb, tile(wm, (t,), 0, D)) for t in range(NF)]
        if swap:
            g, u = u, g
        h = []
        for t in range(NF):
            gt = ln_fix(g[t], mean, rstd, csg_s, t)
            h.append(gt * jax.nn.sigmoid(gt) * ln_fix(u[t], mean, rstd, csu_s, t))
        y = None
        for t0 in range(0, NF, DK):
            hb = jnp.concatenate(h[t0:t0 + DK], axis=1).astype(BF16)
            yt = proj(hb, wd_u, range(ND), t0 * 128, DK * 128)
            y = yt if y is None else yt + y
        return _round(x + (xn + y * jax.nn.sigmoid(r)))

    x_cp.wait()
    wr_cp.wait()
    wr_s[...] = wr_in[...].astype(F32).reshape(1, D)
    x_s[...] = jnp.zeros_like(x_s)
    x_s[0:B, :] = x_in[...].astype(F32)
    out_s[...] = jnp.zeros_like(out_s)
    xn0 = _ln_stats(x_s[...])[2]
    ones = jnp.ones((8, D), F32)
    wait_w(wq_hbm, wq_s, SEM_WQ)
    z = proj(jnp.concatenate([xn0, ones], axis=0).astype(BF16), wq_u, range(NT), 0, D)
    q1_s[...] = z[0:8]
    csq_s[...] = z[8:16]
    transpose_tiles(wq_u, wqt_s, KQ0, KQ)
    transpose_tiles(wq_u, wqt_s, NT - KL, KL, KQ)
    wait_w(wo_hbm, wo_s, SEM_WO)
    wait_w(wg_hbm, wg_s, SEM_WG)
    wait_w(wu_hbm, wu_s, SEM_WU)
    csg_s[...] = proj(ones.astype(BF16), wg_u, range(NF), 0, D)
    csu_s[...] = proj(ones.astype(BF16), wu_u, range(NF), 0, D)
    transpose_tiles(wu_u, wut_s, 0, NF)
    transpose_tiles(wg_u, wgt_s, 0, NF)
    wait_w(wd_hbm, wd_s, SEM_WD)

    srow = lax.broadcasted_iota(jnp.int32, (HG, SR), 0)
    scol = lax.broadcasted_iota(jnp.int32, (HG, SR), 1)
    shead = srow - (scol >= DH).astype(jnp.int32)

    def batch_body(b, carry):
        slot = b % 2
        more = b + 1 < B

        def wait_v(c):
            wait_chunk(vbuf, SEM_V + slot * NVC + c, slot, *V_CHUNKS[c])

            if c < NVC - 1:
                @pl.when(more)
                def _():
                    start_v(b + 1, 1 - slot, c)
                    if c == NVC - 2:
                        start_v(b + 1, 1 - slot, c + 1)

        wait_chunk(kbuf, SEM_K + slot, slot, 0, H * DH, 0, NJ)

        @pl.when(more)
        def _():
            start_k(b + 1, 1 - slot)

        def qk1(g, c):
            off = pl.multiple_of(g * GR, GR)
            qg = jnp.broadcast_to(q1_s[pl.ds(b, 1), pl.ds(off, GR)], (HG, GR))
            lhs = jnp.where(diag, qg, 0.0).astype(BF16)
            s = jnp.concatenate([_dot(lhs, tile(k_u, (slot, j), off, GR)) for j in range(NJ)],
                                axis=1) * SCALE
            e = jnp.exp(s - jnp.max(s, axis=-1, keepdims=True))
            p_s[g] = e * (1.0 / jnp.sum(e, axis=-1, keepdims=True))
            return c
        lax.fori_loop(0, NG, qk1, 0)

        def v_tile(j, off, nr, keep):
            vj = tile(v_u, (slot, j), off, nr)
            if keep:
                vf_s[pl.ds(off // 16, nr // 16), j] = vj.astype(F32).reshape(nr // 16, 16, 128)
            return vj

        def pv_tiles(pb, off, nr, js):
            o = None
            for j in js:
                t = _dot_nt(pb[:, j * 128:(j + 1) * 128], v_tile(j, off, nr, j < NJF))
                o = t if o is None else o + t
            return o

        def wo_pair(o, s, off, nr):
            o = jnp.where(shead[:, 0:nr] == 2 * (s % PG), o, 0.0).astype(BF16)
            return proj(o, wo_u, range(ND), off, nr)

        def pv1(s, y):
            for c in range(NVC - 4):
                @pl.when(s == V_CHUNKS[c][0] // SR)
                def _():
                    wait_v(c)
            off = pl.multiple_of(s * SR, SR)
            pb = p_s[s // PG].astype(BF16)
            return y + wo_pair(pv_tiles(pb, off, SR, range(NJ)), s, off, SR)
        y1 = lax.fori_loop(0, NS - 1, pv1, jnp.zeros((HG, D), F32))

        off = (NS - 1) * SR
        pb = p_s[NG - 1].astype(BF16)
        wait_v(NVC - 4)
        o = pv_tiles(pb, off, 256, range(0, 4))
        wait_v(NVC - 3)
        o = o + pv_tiles(pb, off, 256, range(4, NJ))

        off = H * DH - 128
        acc = None
        for c in (NVC - 2, NVC - 1):
            wait_v(c)
            for j in range(V_CHUNKS[c][2], V_CHUNKS[c][2] + V_CHUNKS[c][3]):
                pj = p_s[NG - 1, HG - 1:HG, j * 128:(j + 1) * 128]
                t = v_tile(j, off, 128, j < 4).astype(F32) * pj
                acc = t if acc is None else acc + t
        y1 = y1 + wo_pair(o, NS - 1, (NS - 1) * SR, 256)
        oc = jnp.sum(acc, axis=-1, keepdims=True)
        yv = [(tile(wo_u, (n,), off, 128).astype(F32) * oc).reshape(16, 8, 128).sum(axis=0)
              for n in range(ND)]
        y1 = y1 + jnp.concatenate(yv, axis=1)

        x0 = jnp.broadcast_to(x_s[pl.ds(b, 1), :], (HG, D))
        x1 = _round(x0 + jnp.sum(y1, axis=0, keepdims=True))
        true8 = (srow[:, 0:128] + b) >= 0
        x2 = moe(x1, true8, False)

        lhs2 = x2.astype(BF16)
        mean2, rstd2, _, part2 = _ln_stats(x2)
        q_t, s_t, p_g, pj_h, o_t, il_h, res, lhs_g, sum_t, yv_h = ({} for _ in range(10))
        y_tiles = [jnp.where(srow[:, 0:128] == 0, x2[:, n * 128:(n + 1) * 128], 0.0)
                   for n in range(ND)]
        x2l = after(true8, x2, part2)

        def job_a(job, t):
            res[job] = _dot(lhs2, tile(wq_u, (t,), 0, D))
            q_t[t] = ln_fix(res[job], mean2, rstd2, csq_s, t)

        def job_v(job, t, gate):
            i = VQ.index(t)
            xv = x2 if i < VG else x2l
            if gate is not None:
                xv = jnp.concatenate([x2[:, 0:D - 128], after(true8, x2[:, D - 128:], res[gate])],
                                     axis=1)
            q_t[t] = ln_fix(vpu_tile(xv, wqt_s, i), mean2, rstd2, csq_s, t)

        def job_b(job, g, j):
            if g not in lhs_g:
                q = jnp.concatenate([q_t[t] for t in range(g * GT, (g + 1) * GT)], axis=1)
                lhs_g[g] = jnp.where(diag[:, 0:GT * 128], q, 0.0).astype(BF16)
            res[job] = s_t[g, j] = _dot(lhs_g[g], tile(k_u, (slot, j), g * GT * 128, GT * 128))

        def job_e(job, g, t, c0, c1, gate):
            if g not in p_g:
                sc = jnp.concatenate([s_t[g, j] for j in range(NJ)], axis=1) * SCALE
                e = jnp.exp(sc - jnp.max(sc, axis=-1, keepdims=True))
                il = 1.0 / jnp.sum(e, axis=-1, keepdims=True)
                p_g[g] = (e, jnp.broadcast_to(il, (8, 128)))
            e, il = p_g[g]
            r0 = t * 8 + c0
            n = c1 - c0
            m = r0 * 16 // DH - g * GT * 128 // DH
            if (g, m) not in pj_h:
                pj_h[g, m] = [jnp.broadcast_to(e[m:m + 1, j * 128:(j + 1) * 128], (8, 128))
                              for j in range(NJ)]
                il_h[g, m] = jnp.broadcast_to(il[m:m + 1, :], (8, 128))
            pj = list(pj_h[g, m])
            if gate is not None:
                pj[NJ - 1] = after(true8, pj[NJ - 1], res[gate])
            nf = NJF if t < NT - 1 else 4
            if (g, m, nf) not in pj_h:
                pj_h[g, m, nf] = jnp.stack(pj[0:nf])[None, :, None]
            vf = vf_s[pl.ds(r0, n), pl.ds(0, nf)].reshape(n, nf, 2, 8, 128)
            acc = jnp.sum(vf * pj_h[g, m, nf], axis=1).reshape(2 * n, 8, 128)
            for j in range(nf, NJ):
                vj = tile(v_u, (slot, j), r0 * 16, n * 16).astype(F32)
                acc = acc + vj.reshape(2 * n, 8, 128) * pj[j][None]
            sums = jnp.sum(acc, axis=-1, keepdims=True)
            if t >= NT - FV:
                for k in range(ND):
                    w = tile(wo_u, (k,), r0 * 16, n * 16).astype(F32).reshape(2 * n, 8, 128)
                    yc = jnp.sum(w * sums, axis=0)
                    yv_h[g, m, k] = yc + yv_h[g, m, k] if (g, m, k) in yv_h else yc
                return
            sum_t.setdefault(t, []).append(jnp.broadcast_to(sums, (2 * n, 8, 128)))
            if c1 == 8:
                m0 = t * 128 // DH - g * GT * 128 // DH
                scale = il_h[g, m0]
                if t % 3 == 1:
                    scale = jnp.where(lane8 < 64, scale, il_h[g, m0 + 1])
                o_t[t] = spread(jnp.concatenate(sum_t[t], axis=0)) * scale

        def job_f(job, t0, t1, n):
            o = jnp.concatenate([o_t[t] for t in range(t0, t1)], axis=1).astype(BF16)
            y = _dot(o, tile(wo_u, (n,), t0 * 128, (t1 - t0) * 128))
            res[job] = y_tiles[n] = y + y_tiles[n]

        for job in _l2_schedule():
            {'a': job_a, 'v': job_v, 'b': job_b, 'e': job_e, 'f': job_f}[job[0]](job, *job[1:])

        for (g, m, n), yc in yv_h.items():
            y_tiles[n] = y_tiles[n] + yc * il_h[g, m]
        x3 = jnp.sum(jnp.concatenate(y_tiles, axis=1), axis=0, keepdims=True)
        x4 = moe(_round(jnp.broadcast_to(x3, (8, D))), true8, True)
        out_s[pl.ds(b, 1), :] = x4[0:1, :]
        return carry

    lax.fori_loop(0, B, batch_body, 0)
    o_ref[...] = out_s[0:B, :].astype(o_ref.dtype)


def _tile_view(t):
    *lead, r, c = t.shape
    n = len(lead)
    t = t.reshape(*lead, r // 16, 2, 8, c // 128, 128)
    return t.transpose(*range(n), n, n + 1, n + 3, n + 2, n + 4)


@jax.jit
def pallas_interleave_layers__sliding_block_cached__moe_arch_mod__decode_kernel(
    A_x: jax.Array,
    A_k_cache: jax.Array,
    A_v_cache: jax.Array,
    A_wq: jax.Array,
    A_wo: jax.Array,
    B_x: jax.Array,
    B_w_r: jax.Array,
    B_w_gate: jax.Array,
    B_w_up: jax.Array,
    B_w_down: jax.Array,
):
    x = A_x.reshape(B, D)
    kt = _tile_view(jnp.swapaxes(A_k_cache, 2, 3).reshape(B, H * DH, SK))
    vt = _tile_view(jnp.swapaxes(A_v_cache, 2, 3).reshape(B, H * DH, SK))

    out = pl.pallas_call(
        _kernel,
        in_specs=[pl.BlockSpec(memory_space=pl.ANY)] * 9,
        out_specs=pl.BlockSpec(memory_space=pltpu.VMEM),
        out_shape=jax.ShapeDtypeStruct((B, D), BF16),
        scratch_shapes=[
            pltpu.VMEM((B, D), BF16),
            pltpu.VMEM((D,), BF16),
            pltpu.VMEM((D // 16, NT + 1, 16, 128), BF16),
            pltpu.VMEM((H * DH // 16, ND, 16, 128), BF16),
            pltpu.VMEM((D // 16, NF + 1, 16, 128), BF16),
            pltpu.VMEM((D // 16, NF + 1, 16, 128), BF16),
            pltpu.VMEM((F // 16, ND, 16, 128), BF16),
            pltpu.VMEM((2, H * DH // 16, NJ + 1, 16, 128), BF16),
            pltpu.VMEM((2, H * DH // 16, NJ, 16, 128), BF16),
            pltpu.VMEM((8, D), F32),
            pltpu.VMEM((8, H * DH), F32),
            pltpu.VMEM((NG, HG, W), F32),
            pltpu.VMEM((8, D), F32),
            pltpu.VMEM((1, D), F32),
            pltpu.VMEM((8, H * DH), F32),
            pltpu.VMEM((8, F), F32),
            pltpu.VMEM((8, F), F32),
            pltpu.VMEM((KQ + KL, 128, D), F32),
            pltpu.VMEM((NF, 128, D), F32),
            pltpu.VMEM((NF, 128, D), F32),
            pltpu.VMEM((H * DH // 16, NJF, 16, 128), F32),
            pltpu.SemaphoreType.DMA((NSEM,)),
        ],
        compiler_params=pltpu.CompilerParams(
            vmem_limit_bytes=116 * 1024 * 1024,
            disable_bounds_checks=True,
            disable_semaphore_checks=True,
        ),
    )(x, kt, vt, _tile_view(A_wq), _tile_view(A_wo), B_w_r,
      _tile_view(B_w_gate), _tile_view(B_w_up), _tile_view(B_w_down))
    return out.reshape(B, 1, D)
```

```python
import jax
import jax.numpy as jnp
from jax import lax
import jax.experimental.pallas as pl
import jax.experimental.pallas.tpu as pltpu

B, D = 4, 640
H, DH, SK = 32, 192, 4096
W = 1024
F = 1536
NJ = W // 128
ND = D // 128
NF = F // 128
NT = H * DH // 128
HG = 8
NG = H // HG
GR = HG * DH
SR = 2 * DH
NS = H // 2
PG = HG // 2
JW0 = (SK - W) // 128
JW = 4
LN_EPS = 1e-5
SCALE = DH ** -0.5
F32 = jnp.float32
BF16 = jnp.bfloat16
U32 = jnp.uint32

V_CHUNKS = ([(g * GR, GR, 0, NJ) for g in range(NG - 1)]
            + [(s * SR, SR, 0, NJ) for s in range(NS - PG, NS - 1)]
            + [((NS - 1) * SR, 256, 0, 4), ((NS - 1) * SR, 256, 4, 4),
               (H * DH - 128, 128, 0, 4), (H * DH - 128, 128, 4, 4)])
NVC = len(V_CHUNKS)

SEM_X, SEM_WR, SEM_WQ, SEM_WO, SEM_WG, SEM_WU, SEM_WD = range(7)
SEM_K = 7
SEM_V = SEM_K + 2
NSEM = SEM_V + 2 * NVC

GT = 6
NG2 = NT // GT
KQ0, KQ, KL = 6, 19, 10
VQ = list(range(KQ0, KQ0 + KQ)) + list(range(NT - KL, NT))
NJF = 6
FV = 3
VG = 4
DK = 3


def _l2_schedule():
    t_e, t_v = 83 / 8, 45
    t_x, t_soft, t_pop, lead = 150, 270, 130, 300
    a_jobs = [[('a', t) for t in range(g * GT, (g + 1) * GT) if t not in VQ] for g in range(NG2)]
    mx = list(a_jobs[0])
    nxt = [g for g in range(1, NG2) if a_jobs[g]]
    for g in range(NG2):
        if nxt and (g == 0 or nxt[0] <= g + 1):
            mx += a_jobs[nxt.pop(0)]
        mx += [('b', g, j) for j in range(NJ)]
    es = [(t // GT, t, c) for t in range(NT) for c in range(8)]
    for i, t in enumerate(range(NT - KL, NT)):
        es.insert(2 + i * 17, (es[2 + i * 17][0], t, 'v'))
    cuts = list(range(0, NT - FV, 2)) + [NT - FV]
    fs = [('f', c0, c1, n) for c0, c1 in zip(cuts[:-1], cuts[1:]) for n in range(ND)]
    order, now, vpu = [('v', t, None) for t in range(KQ0, KQ0 + KQ)], 0, KQ * t_v
    b_end, avail, o_at = {}, [], {}

    def start(e):
        return max(vpu, b_end[e[0]] + t_soft)

    def cost(job):
        return 40 if job[0] == 'a' else 8 * GT if job[0] == 'b' else 8 * (job[2] - job[1])

    def urgent(extra):
        t = now + extra
        for job in mx:
            t += cost(job)
            if job[0] == 'b' and job[2] == NJ - 1:
                n_before = sum(1 for e in es if e[0] < job[1])
                if t + t_soft + lead > vpu + n_before * t_e:
                    return True
        return False

    while mx or es or fs:
        while es and es[0][0] in b_end and (
                start(es[0]) <= now + t_pop or not (mx or (fs and fs[0][2] - 1 in o_at))):
            e = es.pop(0)
            st = start(e)
            gate = None
            if vpu > b_end[e[0]] + t_soft:
                gate = [j for (tt, j) in avail if tt <= st][-1]
            if e[2] == 'v':
                order.append(('v', e[1], gate))
                vpu = st + t_v
                continue
            prev = order[-1]
            if (prev[0] == 'e' and prev[2] == e[1] and prev[5] == gate
                    and not (e[1] % 3 == 1 and e[2] == 4)):
                order[-1] = prev[:4] + (e[2] + 1, gate)
            else:
                order.append(('e', e[0], e[1], e[2], e[2] + 1, gate))
            vpu = st + t_e
            if e[2] == 7:
                o_at[e[1]] = vpu + t_x
        if not (mx or fs):
            continue
        f_ready = fs and o_at.get(fs[0][2] - 1, 1 << 30) <= now
        if mx and not (f_ready and not urgent(cost(fs[0]))):
            job = mx.pop(0)
            now += cost(job)
            if job[0] == 'b' and job[2] == NJ - 1:
                b_end[job[1]] = now
        else:
            job = fs.pop(0)
            now = max(now, o_at[job[2] - 1]) + cost(job)
        order.append(job)
        avail.append((now + t_pop, job))
    return order


def _dot(a, b):
    return jnp.dot(a, b, preferred_element_type=F32)


def _dot_nt(a, b):
    return lax.dot_general(a, b, (((1,), (1,)), ((), ())), preferred_element_type=F32)


def _round(x):
    return x.astype(BF16).astype(F32)


def _ln_stats(x):
    m = jnp.mean(x, axis=-1, keepdims=True)
    c = x - m
    c2 = c * c
    part = c2[:, 0:128]
    for kt in range(1, ND):
        part = part + c2[:, kt * 128:(kt + 1) * 128]
    v = jnp.sum(part, axis=-1, keepdims=True) * (1.0 / D)
    m = _round(m)
    r = lax.rsqrt(v + LN_EPS)
    return m, r, (x - m) * r, part


def _kernel(x_hbm, k_hbm, v_hbm, wq_hbm, wo_hbm, wr_hbm, wg_hbm, wu_hbm, wd_hbm,
            o_ref,
            x_in, wr_in, wq_s, wo_s, wg_s, wu_s, wd_s, kbuf, vbuf,
            x_s, q1_s, p_s, out_s, wr_s, csq_s, csg_s, csu_s, wqt_s, wut_s, wgt_s, vf_s,
            sems):
    def row_copies(src, dst, sem, r0, nr, j_src, j0, nj, jw):
        rows = pl.ds(r0 // 16, nr // 16)
        return [pltpu.make_async_copy(src.at[rows, half, pl.ds(j_src + j, jw)],
                                      dst.at[rows, pl.ds(j, jw), pl.ds(half * 8, 8)],
                                      sems.at[sem])
                for half in range(2) for j in range(j0, j0 + nj, jw)]

    def w_copies(src, dst, sem, nr):
        return [c for r0 in range(0, dst.shape[0] * 16, nr)
                for c in row_copies(src, dst, sem, r0, nr, 0, 0, src.shape[2], src.shape[2])]

    def k_copies(b, slot):
        return [c for g in range(NG) for c in row_copies(
            k_hbm.at[b], kbuf.at[slot], SEM_K + slot, g * GR, GR, JW0, 0, NJ, JW)]

    def v_copies(b, slot, c):
        r0, nr, j0, nj = V_CHUNKS[c]
        return row_copies(v_hbm.at[b], vbuf.at[slot], SEM_V + slot * NVC + c,
                          r0, nr, JW0, j0, nj, JW)

    def start(copies):
        for c in copies:
            c.start()

    def wait(copies):
        for c in copies:
            c.wait()

    x_cp = pltpu.make_async_copy(x_hbm, x_in, sems.at[SEM_X])
    wr_cp = pltpu.make_async_copy(wr_hbm, wr_in, sems.at[SEM_WR])
    wq_cp = w_copies(wq_hbm, wq_s, SEM_WQ, D)
    wo_cp = w_copies(wo_hbm, wo_s, SEM_WO, 384)
    wg_cp = w_copies(wg_hbm, wg_s, SEM_WG, D)
    wu_cp = w_copies(wu_hbm, wu_s, SEM_WU, D)
    wd_cp = w_copies(wd_hbm, wd_s, SEM_WD, 384)
    start(wq_cp + [x_cp, wr_cp] + wo_cp + wg_cp + wu_cp + wd_cp + k_copies(0, 0))
    for c in range(NVC):
        start(v_copies(0, 0, c))

    wq_u, wo_u, wg_u, wu_u, wd_u, k_u, v_u = (
        r.bitcast(U32) for r in (wq_s, wo_s, wg_s, wu_s, wd_s, kbuf, vbuf))

    def tile(ref_u, idx, start, size):
        x = ref_u[idx[:-1] + (pl.ds(start // 16, size // 16), idx[-1])]
        return pltpu.bitcast(x.reshape(size // 2, 128), BF16)

    def proj(a, w_u, tiles, start, size):
        return jnp.concatenate([_dot(a, tile(w_u, (j,), start, size)) for j in tiles], axis=1)

    def ln_fix(z, mean, rstd, cs_s, t):
        return (z - mean * cs_s[:, t * 128:(t + 1) * 128]) * rstd

    lane8 = lax.broadcasted_iota(jnp.int32, (8, 128), 1)
    sub8 = lax.broadcasted_iota(jnp.int32, (8, 128), 0)

    bits = [((lane8 & bit) != 0)[None] for bit in (8, 16, 32, 64)]
    on_diag = (lane8 & 7) == sub8

    def spread(sums):
        v = jnp.broadcast_to(sums, (16, 8, 128))
        for hi in bits:
            v = v.reshape(v.shape[0] // 2, 2, 8, 128)
            v = jnp.where(hi, v[:, 1], v[:, 0])
        return jnp.where(on_diag, v[0], 0.0)

    def after(true8, x, dep):
        return jnp.concatenate([jnp.where(true8, x[:, k:k + 128], dep)
                                for k in range(0, x.shape[1], 128)], axis=1)

    def vpu_tile(x, wt_s, i):
        sums = jnp.sum(wt_s[i].reshape(16, 8, D) * x[None], axis=-1, keepdims=True)
        return jnp.broadcast_to(jnp.sum(spread(sums), axis=0, keepdims=True), (8, 128))

    def transpose_tiles(w_u, wt_s, t0, n, i0=0):
        def body(i, c):
            for kt in range(ND):
                wt_s[i0 + i, :, kt * 128:(kt + 1) * 128] = (
                    tile(w_u, (t0 + i,), kt * 128, 128).astype(F32).T)
            return c
        lax.fori_loop(0, n, body, 0)

    row = lax.broadcasted_iota(jnp.int32, (HG, GR), 0)
    col = lax.broadcasted_iota(jnp.int32, (HG, GR), 1)
    diag = (col >= row * DH) & (col < (row + 1) * DH)

    def moe(x, true8, swap):
        xb = x.astype(BF16)
        mean, rstd, xn, part = _ln_stats(x)
        r = jnp.sum(xn * wr_s[...], axis=-1, keepdims=True)
        xl = after(true8, x, part)
        wvt, wm = (wgt_s, wu_u) if swap else (wut_s, wg_u)
        u = [vpu_tile(x if i < VG else xl, wvt, i) for i in range(NF)]
        g = [_dot(xb, tile(wm, (t,), 0, D)) for t in range(NF)]
        if swap:
            g, u = u, g
        h = []
        for t in range(NF):
            gt = ln_fix(g[t], mean, rstd, csg_s, t)
            h.append(gt * jax.nn.sigmoid(gt) * ln_fix(u[t], mean, rstd, csu_s, t))
        y = None
        for t0 in range(0, NF, DK):
            hb = jnp.concatenate(h[t0:t0 + DK], axis=1).astype(BF16)
            yt = proj(hb, wd_u, range(ND), t0 * 128, DK * 128)
            y = yt if y is None else yt + y
        return _round(x + (xn + y * jax.nn.sigmoid(r)))

    x_cp.wait()
    wr_cp.wait()
    wr_s[...] = wr_in[...].astype(F32).reshape(1, D)
    x_s[...] = jnp.zeros_like(x_s)
    x_s[0:B, :] = x_in[...].astype(F32)
    out_s[...] = jnp.zeros_like(out_s)
    xn0 = _ln_stats(x_s[...])[2]
    ones = jnp.ones((8, D), F32)
    wait(wq_cp)
    z = proj(jnp.concatenate([xn0, ones], axis=0).astype(BF16), wq_u, range(NT), 0, D)
    q1_s[...] = z[0:8]
    csq_s[...] = z[8:16]
    transpose_tiles(wq_u, wqt_s, KQ0, KQ)
    transpose_tiles(wq_u, wqt_s, NT - KL, KL, KQ)
    wait(wo_cp)
    wait(wg_cp)
    wait(wu_cp)
    csg_s[...] = proj(ones.astype(BF16), wg_u, range(NF), 0, D)
    csu_s[...] = proj(ones.astype(BF16), wu_u, range(NF), 0, D)
    transpose_tiles(wu_u, wut_s, 0, NF)
    transpose_tiles(wg_u, wgt_s, 0, NF)
    wait(wd_cp)

    srow = lax.broadcasted_iota(jnp.int32, (HG, SR), 0)
    scol = lax.broadcasted_iota(jnp.int32, (HG, SR), 1)
    shead = srow - (scol >= DH).astype(jnp.int32)

    def batch_body(b, carry):
        slot = b % 2
        more = b + 1 < B

        def wait_v(c):
            wait(v_copies(b, slot, c))

            if c < NVC - 1:
                @pl.when(more)
                def _():
                    start(v_copies(b + 1, 1 - slot, c))
                    if c == NVC - 2:
                        start(v_copies(b + 1, 1 - slot, c + 1))

        wait(k_copies(b, slot))

        @pl.when(more)
        def _():
            start(k_copies(b + 1, 1 - slot))

        def qk1(g, c):
            off = pl.multiple_of(g * GR, GR)
            qg = jnp.broadcast_to(q1_s[pl.ds(b, 1), pl.ds(off, GR)], (HG, GR))
            lhs = jnp.where(diag, qg, 0.0).astype(BF16)
            s = jnp.concatenate([_dot(lhs, tile(k_u, (slot, j), off, GR)) for j in range(NJ)],
                                axis=1) * SCALE
            e = jnp.exp(s - jnp.max(s, axis=-1, keepdims=True))
            p_s[g] = e * (1.0 / jnp.sum(e, axis=-1, keepdims=True))
            return c
        lax.fori_loop(0, NG, qk1, 0)

        def v_tile(j, off, nr, keep):
            vj = tile(v_u, (slot, j), off, nr)
            if keep:
                vf_s[pl.ds(off // 16, nr // 16), j] = vj.astype(F32).reshape(nr // 16, 16, 128)
            return vj

        def pv_tiles(pb, off, nr, js):
            o = None
            for j in js:
                t = _dot_nt(pb[:, j * 128:(j + 1) * 128], v_tile(j, off, nr, j < NJF))
                o = t if o is None else o + t
            return o

        def wo_pair(o, s, off, nr):
            o = jnp.where(shead[:, 0:nr] == 2 * (s % PG), o, 0.0).astype(BF16)
            return proj(o, wo_u, range(ND), off, nr)

        def pv1(s, y):
            for c in range(NVC - 4):
                @pl.when(s == V_CHUNKS[c][0] // SR)
                def _():
                    wait_v(c)
            off = pl.multiple_of(s * SR, SR)
            pb = p_s[s // PG].astype(BF16)
            return y + wo_pair(pv_tiles(pb, off, SR, range(NJ)), s, off, SR)
        y1 = lax.fori_loop(0, NS - 1, pv1, jnp.zeros((HG, D), F32))

        off = (NS - 1) * SR
        pb = p_s[NG - 1].astype(BF16)
        wait_v(NVC - 4)
        o = pv_tiles(pb, off, 256, range(0, 4))
        wait_v(NVC - 3)
        o = o + pv_tiles(pb, off, 256, range(4, NJ))

        off = H * DH - 128
        acc = None
        for c in (NVC - 2, NVC - 1):
            wait_v(c)
            for j in range(V_CHUNKS[c][2], V_CHUNKS[c][2] + V_CHUNKS[c][3]):
                pj = p_s[NG - 1, HG - 1:HG, j * 128:(j + 1) * 128]
                t = v_tile(j, off, 128, j < 4).astype(F32) * pj
                acc = t if acc is None else acc + t
        y1 = y1 + wo_pair(o, NS - 1, (NS - 1) * SR, 256)
        oc = jnp.sum(acc, axis=-1, keepdims=True)
        yv = [(tile(wo_u, (n,), off, 128).astype(F32) * oc).reshape(16, 8, 128).sum(axis=0)
              for n in range(ND)]
        y1 = y1 + jnp.concatenate(yv, axis=1)

        x0 = jnp.broadcast_to(x_s[pl.ds(b, 1), :], (HG, D))
        x1 = _round(x0 + jnp.sum(y1, axis=0, keepdims=True))
        true8 = (srow[:, 0:128] + b) >= 0
        x2 = moe(x1, true8, False)

        lhs2 = x2.astype(BF16)
        mean2, rstd2, _, part2 = _ln_stats(x2)
        q_t, s_t, p_g, pj_h, o_t, il_h, res, lhs_g, sum_t, yv_h = ({} for _ in range(10))
        y_tiles = [jnp.where(srow[:, 0:128] == 0, x2[:, n * 128:(n + 1) * 128], 0.0)
                   for n in range(ND)]
        x2l = after(true8, x2, part2)

        def job_a(job, t):
            res[job] = _dot(lhs2, tile(wq_u, (t,), 0, D))
            q_t[t] = ln_fix(res[job], mean2, rstd2, csq_s, t)

        def job_v(job, t, gate):
            i = VQ.index(t)
            xv = x2 if i < VG else x2l
            if gate is not None:
                xv = jnp.concatenate([x2[:, 0:D - 128], after(true8, x2[:, D - 128:], res[gate])],
                                     axis=1)
            q_t[t] = ln_fix(vpu_tile(xv, wqt_s, i), mean2, rstd2, csq_s, t)

        def job_b(job, g, j):
            if g not in lhs_g:
                q = jnp.concatenate([q_t[t] for t in range(g * GT, (g + 1) * GT)], axis=1)
                lhs_g[g] = jnp.where(diag[:, 0:GT * 128], q, 0.0).astype(BF16)
            res[job] = s_t[g, j] = _dot(lhs_g[g], tile(k_u, (slot, j), g * GT * 128, GT * 128))

        def job_e(job, g, t, c0, c1, gate):
            if g not in p_g:
                sc = jnp.concatenate([s_t[g, j] for j in range(NJ)], axis=1) * SCALE
                e = jnp.exp(sc - jnp.max(sc, axis=-1, keepdims=True))
                il = 1.0 / jnp.sum(e, axis=-1, keepdims=True)
                p_g[g] = (e, jnp.broadcast_to(il, (8, 128)))
            e, il = p_g[g]
            r0 = t * 8 + c0
            n = c1 - c0
            m = r0 * 16 // DH - g * GT * 128 // DH
            if (g, m) not in pj_h:
                pj_h[g, m] = [jnp.broadcast_to(e[m:m + 1, j * 128:(j + 1) * 128], (8, 128))
                              for j in range(NJ)]
                il_h[g, m] = jnp.broadcast_to(il[m:m + 1, :], (8, 128))
            pj = list(pj_h[g, m])
            if gate is not None:
                pj[NJ - 1] = after(true8, pj[NJ - 1], res[gate])
            nf = NJF if t < NT - 1 else 4
            if (g, m, nf) not in pj_h:
                pj_h[g, m, nf] = jnp.stack(pj[0:nf])[None, :, None]
            vf = vf_s[pl.ds(r0, n), pl.ds(0, nf)].reshape(n, nf, 2, 8, 128)
            acc = jnp.sum(vf * pj_h[g, m, nf], axis=1).reshape(2 * n, 8, 128)
            for j in range(nf, NJ):
                vj = tile(v_u, (slot, j), r0 * 16, n * 16).astype(F32)
                acc = acc + vj.reshape(2 * n, 8, 128) * pj[j][None]
            sums = jnp.sum(acc, axis=-1, keepdims=True)
            if t >= NT - FV:
                for k in range(ND):
                    w = tile(wo_u, (k,), r0 * 16, n * 16).astype(F32).reshape(2 * n, 8, 128)
                    yc = jnp.sum(w * sums, axis=0)
                    yv_h[g, m, k] = yc + yv_h[g, m, k] if (g, m, k) in yv_h else yc
                return
            sum_t.setdefault(t, []).append(jnp.broadcast_to(sums, (2 * n, 8, 128)))
            if c1 == 8:
                m0 = t * 128 // DH - g * GT * 128 // DH
                scale = il_h[g, m0]
                if t % 3 == 1:
                    scale = jnp.where(lane8 < 64, scale, il_h[g, m0 + 1])
                o_t[t] = spread(jnp.concatenate(sum_t[t], axis=0)) * scale

        def job_f(job, t0, t1, n):
            o = jnp.concatenate([o_t[t] for t in range(t0, t1)], axis=1).astype(BF16)
            y = _dot(o, tile(wo_u, (n,), t0 * 128, (t1 - t0) * 128))
            res[job] = y_tiles[n] = y + y_tiles[n]

        for job in _l2_schedule():
            {'a': job_a, 'v': job_v, 'b': job_b, 'e': job_e, 'f': job_f}[job[0]](job, *job[1:])

        for (g, m, n), yc in yv_h.items():
            y_tiles[n] = y_tiles[n] + yc * il_h[g, m]
        x3 = jnp.sum(jnp.concatenate(y_tiles, axis=1), axis=0, keepdims=True)
        x4 = moe(_round(jnp.broadcast_to(x3, (8, D))), true8, True)
        out_s[pl.ds(b, 1), :] = x4[0:1, :]
        return carry

    lax.fori_loop(0, B, batch_body, 0)
    o_ref[...] = out_s[0:B, :].astype(o_ref.dtype)


def _tile_view(t):
    *lead, r, c = t.shape
    n = len(lead)
    t = t.reshape(*lead, r // 16, 2, 8, c // 128, 128)
    return t.transpose(*range(n), n, n + 1, n + 3, n + 2, n + 4)


@jax.jit
def pallas_interleave_layers__sliding_block_cached__moe_arch_mod__decode_kernel(
    A_x: jax.Array,
    A_k_cache: jax.Array,
    A_v_cache: jax.Array,
    A_wq: jax.Array,
    A_wo: jax.Array,
    B_x: jax.Array,
    B_w_r: jax.Array,
    B_w_gate: jax.Array,
    B_w_up: jax.Array,
    B_w_down: jax.Array,
):
    x = A_x.reshape(B, D)
    kt = _tile_view(jnp.swapaxes(A_k_cache, 2, 3).reshape(B, H * DH, SK))
    vt = _tile_view(jnp.swapaxes(A_v_cache, 2, 3).reshape(B, H * DH, SK))

    out = pl.pallas_call(
        _kernel,
        in_specs=[pl.BlockSpec(memory_space=pl.ANY)] * 9,
        out_specs=pl.BlockSpec(memory_space=pltpu.VMEM),
        out_shape=jax.ShapeDtypeStruct((B, D), BF16),
        scratch_shapes=[
            pltpu.VMEM((B, D), BF16),
            pltpu.VMEM((D,), BF16),
            pltpu.VMEM((D // 16, NT + 1, 16, 128), BF16),
            pltpu.VMEM((H * DH // 16, ND, 16, 128), BF16),
            pltpu.VMEM((D // 16, NF + 1, 16, 128), BF16),
            pltpu.VMEM((D // 16, NF + 1, 16, 128), BF16),
            pltpu.VMEM((F // 16, ND, 16, 128), BF16),
            pltpu.VMEM((2, H * DH // 16, NJ + 1, 16, 128), BF16),
            pltpu.VMEM((2, H * DH // 16, NJ, 16, 128), BF16),
            pltpu.VMEM((8, D), F32),
            pltpu.VMEM((8, H * DH), F32),
            pltpu.VMEM((NG, HG, W), F32),
            pltpu.VMEM((8, D), F32),
            pltpu.VMEM((1, D), F32),
            pltpu.VMEM((8, H * DH), F32),
            pltpu.VMEM((8, F), F32),
            pltpu.VMEM((8, F), F32),
            pltpu.VMEM((KQ + KL, 128, D), F32),
            pltpu.VMEM((NF, 128, D), F32),
            pltpu.VMEM((NF, 128, D), F32),
            pltpu.VMEM((H * DH // 16, NJF, 16, 128), F32),
            pltpu.SemaphoreType.DMA((NSEM,)),
        ],
        compiler_params=pltpu.CompilerParams(
            vmem_limit_bytes=116 * 1024 * 1024,
            disable_bounds_checks=True,
            disable_semaphore_checks=True,
        ),
    )(x, kt, vt, _tile_view(A_wq), _tile_view(A_wo), B_w_r,
      _tile_view(B_w_gate), _tile_view(B_w_up), _tile_view(B_w_down))
    return out.reshape(B, 1, D)
```

```python
import jax
import jax.numpy as jnp
from jax import lax
import jax.experimental.pallas as pl
import jax.experimental.pallas.tpu as pltpu

B, D = 4, 640
H, DH, SK = 32, 192, 4096
W = 1024
F = 1536
NJ = W // 128
ND = D // 128
NF = F // 128
NT = H * DH // 128
HG = 8
NG = H // HG
GR = HG * DH
SR = 2 * DH
NS = H // 2
PG = HG // 2
JW0 = (SK - W) // 128
JW = 4
LN_EPS = 1e-5
SCALE = DH ** -0.5
F32 = jnp.float32
BF16 = jnp.bfloat16
U32 = jnp.uint32

V_CHUNKS = ([(g * GR, GR, 0, NJ) for g in range(NG - 1)]
            + [(s * SR, SR, 0, NJ) for s in range(NS - PG, NS - 1)]
            + [((NS - 1) * SR, 256, 0, 4), ((NS - 1) * SR, 256, 4, 4),
               (H * DH - 128, 128, 0, 4), (H * DH - 128, 128, 4, 4)])
NVC = len(V_CHUNKS)

SEM_X, SEM_WR, SEM_WQ, SEM_WO, SEM_WG, SEM_WU, SEM_WD = range(7)
SEM_K = 7
SEM_V = SEM_K + 2
NSEM = SEM_V + 2 * NVC

GT = 6
NG2 = NT // GT
KQ0, KQ, KL = 6, 19, 10
VQ = list(range(KQ0, KQ0 + KQ)) + list(range(NT - KL, NT))
NJF = 6
FV = 3
VG = 4
DK = 3


def _l2_schedule():
    t_e, t_v = 83 / 8, 45
    t_x, t_soft, t_pop, lead = 150, 270, 130, 225
    a_jobs = [[('a', t) for t in range(g * GT, (g + 1) * GT) if t not in VQ] for g in range(NG2)]
    mx = list(a_jobs[0])
    nxt = [g for g in range(1, NG2) if a_jobs[g]]
    for g in range(NG2):
        if nxt and (g == 0 or nxt[0] <= g + 1):
            mx += a_jobs[nxt.pop(0)]
        mx += [('b', g, j) for j in range(NJ)]
    es = [(t // GT, t, c) for t in range(NT) for c in range(8)]
    for i, t in enumerate(range(NT - KL, NT)):
        es.insert(9 + i * 14, (es[9 + i * 14][0], t, 'v'))
    cuts = list(range(0, NT - FV, 2)) + [NT - FV]
    fs = [('f', c0, c1, n) for c0, c1 in zip(cuts[:-1], cuts[1:]) for n in range(ND)]
    order, now, vpu = [('v', t, None) for t in range(KQ0, KQ0 + KQ)], 0, KQ * t_v
    b_end, avail, o_at = {}, [], {}

    def start(e):
        return max(vpu, b_end[e[0]] + t_soft)

    def cost(job):
        return 40 if job[0] == 'a' else 8 * GT if job[0] == 'b' else 8 * (job[2] - job[1])

    def urgent(extra):
        t = now + extra
        for job in mx:
            t += cost(job)
            if job[0] == 'b' and job[2] == NJ - 1:
                n_before = sum(1 for e in es if e[0] < job[1])
                if t + t_soft + lead > vpu + n_before * t_e:
                    return True
        return False

    while mx or es or fs:
        while es and es[0][0] in b_end and (
                start(es[0]) <= now + t_pop or not (mx or (fs and fs[0][2] - 1 in o_at))):
            e = es.pop(0)
            st = start(e)
            gate = None
            if vpu > b_end[e[0]] + t_soft:
                gate = [j for (tt, j) in avail if tt <= st][-1]
            if e[2] == 'v':
                order.append(('v', e[1], gate))
                vpu = st + t_v
                continue
            prev = order[-1]
            if (prev[0] == 'e' and prev[2] == e[1] and prev[5] == gate
                    and not (e[1] % 3 == 1 and e[2] == 4)):
                order[-1] = prev[:4] + (e[2] + 1, gate)
            else:
                order.append(('e', e[0], e[1], e[2], e[2] + 1, gate))
            vpu = st + t_e
            if e[2] == 7:
                o_at[e[1]] = vpu + t_x
        if not (mx or fs):
            continue
        f_ready = fs and o_at.get(fs[0][2] - 1, 1 << 30) <= now
        if mx and not (f_ready and not urgent(cost(fs[0]))):
            job = mx.pop(0)
            now += cost(job)
            if job[0] == 'b' and job[2] == NJ - 1:
                b_end[job[1]] = now
        else:
            job = fs.pop(0)
            now = max(now, o_at[job[2] - 1]) + cost(job)
        order.append(job)
        avail.append((now + t_pop, job))
    return order


def _dot(a, b):
    return jnp.dot(a, b, preferred_element_type=F32)


def _dot_nt(a, b):
    return lax.dot_general(a, b, (((1,), (1,)), ((), ())), preferred_element_type=F32)


def _round(x):
    return x.astype(BF16).astype(F32)


def _ln_stats(x):
    m = jnp.mean(x, axis=-1, keepdims=True)
    c = x - m
    c2 = c * c
    part = c2[:, 0:128]
    for kt in range(1, ND):
        part = part + c2[:, kt * 128:(kt + 1) * 128]
    v = jnp.sum(part, axis=-1, keepdims=True) * (1.0 / D)
    m = _round(m)
    r = lax.rsqrt(v + LN_EPS)
    return m, r, (x - m) * r, part


def _kernel(x_hbm, k_hbm, v_hbm, wq_hbm, wo_hbm, wr_hbm, wg_hbm, wu_hbm, wd_hbm,
            o_ref,
            x_in, wr_in, wq_s, wo_s, wg_s, wu_s, wd_s, kbuf, vbuf,
            x_s, q1_s, p_s, out_s, wr_s, csq_s, csg_s, csu_s, wqt_s, wut_s, wgt_s, vf_s,
            sems):
    def row_copies(src, dst, sem, r0, nr, j_src, j0, nj, jw):
        rows = pl.ds(r0 // 16, nr // 16)
        return [pltpu.make_async_copy(src.at[rows, half, pl.ds(j_src + j, jw)],
                                      dst.at[rows, pl.ds(j, jw), pl.ds(half * 8, 8)],
                                      sems.at[sem])
                for half in range(2) for j in range(j0, j0 + nj, jw)]

    def w_copies(src, dst, sem, nr):
        return [c for r0 in range(0, dst.shape[0] * 16, nr)
                for c in row_copies(src, dst, sem, r0, nr, 0, 0, src.shape[2], src.shape[2])]

    def k_copies(b, slot):
        return [c for g in range(NG) for c in row_copies(
            k_hbm.at[b], kbuf.at[slot], SEM_K + slot, g * GR, GR, JW0, 0, NJ, JW)]

    def v_copies(b, slot, c):
        r0, nr, j0, nj = V_CHUNKS[c]
        return row_copies(v_hbm.at[b], vbuf.at[slot], SEM_V + slot * NVC + c,
                          r0, nr, JW0, j0, nj, JW)

    def start(copies):
        for c in copies:
            c.start()

    def wait(copies):
        for c in copies:
            c.wait()

    x_cp = pltpu.make_async_copy(x_hbm, x_in, sems.at[SEM_X])
    wr_cp = pltpu.make_async_copy(wr_hbm, wr_in, sems.at[SEM_WR])
    wq_cp = w_copies(wq_hbm, wq_s, SEM_WQ, D)
    wo_cp = w_copies(wo_hbm, wo_s, SEM_WO, 384)
    wg_cp = w_copies(wg_hbm, wg_s, SEM_WG, D)
    wu_cp = w_copies(wu_hbm, wu_s, SEM_WU, D)
    wd_cp = w_copies(wd_hbm, wd_s, SEM_WD, 384)
    start(wq_cp + [x_cp, wr_cp] + wo_cp + wg_cp + wu_cp + wd_cp + k_copies(0, 0))
    for c in range(NVC):
        start(v_copies(0, 0, c))

    wq_u, wo_u, wg_u, wu_u, wd_u, k_u, v_u = (
        r.bitcast(U32) for r in (wq_s, wo_s, wg_s, wu_s, wd_s, kbuf, vbuf))

    def tile(ref_u, idx, start, size):
        x = ref_u[idx[:-1] + (pl.ds(start // 16, size // 16), idx[-1])]
        return pltpu.bitcast(x.reshape(size // 2, 128), BF16)

    def proj(a, w_u, tiles, start, size):
        return jnp.concatenate([_dot(a, tile(w_u, (j,), start, size)) for j in tiles], axis=1)

    def ln_fix(z, mean, rstd, cs_s, t):
        return (z - mean * cs_s[:, t * 128:(t + 1) * 128]) * rstd

    lane8 = lax.broadcasted_iota(jnp.int32, (8, 128), 1)
    sub8 = lax.broadcasted_iota(jnp.int32, (8, 128), 0)

    bits = [((lane8 & bit) != 0)[None] for bit in (8, 16, 32, 64)]
    on_diag = (lane8 & 7) == sub8

    def spread(sums):
        v = jnp.broadcast_to(sums, (16, 8, 128))
        for hi in bits:
            v = v.reshape(v.shape[0] // 2, 2, 8, 128)
            v = jnp.where(hi, v[:, 1], v[:, 0])
        return jnp.where(on_diag, v[0], 0.0)

    def after(true8, x, dep):
        return jnp.concatenate([jnp.where(true8, x[:, k:k + 128], dep)
                                for k in range(0, x.shape[1], 128)], axis=1)

    def vpu_tile(x, wt_s, i):
        sums = jnp.sum(wt_s[i].reshape(16, 8, D) * x[None], axis=-1, keepdims=True)
        return jnp.broadcast_to(jnp.sum(spread(sums), axis=0, keepdims=True), (8, 128))

    def transpose_tiles(w_u, wt_s, t0, n, i0=0):
        def body(i, c):
            for kt in range(ND):
                wt_s[i0 + i, :, kt * 128:(kt + 1) * 128] = (
                    tile(w_u, (t0 + i,), kt * 128, 128).astype(F32).T)
            return c
        lax.fori_loop(0, n, body, 0)

    row = lax.broadcasted_iota(jnp.int32, (HG, GR), 0)
    col = lax.broadcasted_iota(jnp.int32, (HG, GR), 1)
    diag = (col >= row * DH) & (col < (row + 1) * DH)

    def moe(x, true8, swap):
        xb = x.astype(BF16)
        mean, rstd, xn, part = _ln_stats(x)
        r = jnp.sum(xn * wr_s[...], axis=-1, keepdims=True)
        xl = after(true8, x, part)
        wvt, wm = (wgt_s, wu_u) if swap else (wut_s, wg_u)
        u = [vpu_tile(x if i < VG else xl, wvt, i) for i in range(NF)]
        g = [_dot(xb, tile(wm, (t,), 0, D)) for t in range(NF)]
        if swap:
            g, u = u, g
        h = []
        for t in range(NF):
            gt = ln_fix(g[t], mean, rstd, csg_s, t)
            h.append(gt * jax.nn.sigmoid(gt) * ln_fix(u[t], mean, rstd, csu_s, t))
        y = None
        for t0 in range(0, NF, DK):
            hb = jnp.concatenate(h[t0:t0 + DK], axis=1).astype(BF16)
            yt = proj(hb, wd_u, range(ND), t0 * 128, DK * 128)
            y = yt if y is None else yt + y
        return _round(x + (xn + y * jax.nn.sigmoid(r)))

    x_cp.wait()
    wr_cp.wait()
    wr_s[...] = wr_in[...].astype(F32).reshape(1, D)
    x_s[...] = jnp.zeros_like(x_s)
    x_s[0:B, :] = x_in[...].astype(F32)
    out_s[...] = jnp.zeros_like(out_s)
    xn0 = _ln_stats(x_s[...])[2]
    ones = jnp.ones((8, D), F32)
    wait(wq_cp)
    z = proj(jnp.concatenate([xn0, ones], axis=0).astype(BF16), wq_u, range(NT), 0, D)
    q1_s[...] = z[0:8]
    csq_s[...] = z[8:16]
    transpose_tiles(wq_u, wqt_s, KQ0, KQ)
    transpose_tiles(wq_u, wqt_s, NT - KL, KL, KQ)
    wait(wo_cp)
    wait(wg_cp)
    wait(wu_cp)
    csg_s[...] = proj(ones.astype(BF16), wg_u, range(NF), 0, D)
    csu_s[...] = proj(ones.astype(BF16), wu_u, range(NF), 0, D)
    transpose_tiles(wu_u, wut_s, 0, NF)
    transpose_tiles(wg_u, wgt_s, 0, NF)
    wait(wd_cp)

    srow = lax.broadcasted_iota(jnp.int32, (HG, SR), 0)
    scol = lax.broadcasted_iota(jnp.int32, (HG, SR), 1)
    shead = srow - (scol >= DH).astype(jnp.int32)

    def batch_body(b, carry):
        slot = b % 2
        more = b + 1 < B

        def wait_v(c):
            wait(v_copies(b, slot, c))

            if c < NVC - 1:
                @pl.when(more)
                def _():
                    start(v_copies(b + 1, 1 - slot, c))
                    if c == NVC - 2:
                        start(v_copies(b + 1, 1 - slot, c + 1))

        wait(k_copies(b, slot))

        @pl.when(more)
        def _():
            start(k_copies(b + 1, 1 - slot))

        def qk1(g, c):
            off = pl.multiple_of(g * GR, GR)
            qg = jnp.broadcast_to(q1_s[pl.ds(b, 1), pl.ds(off, GR)], (HG, GR))
            lhs = jnp.where(diag, qg, 0.0).astype(BF16)
            s = jnp.concatenate([_dot(lhs, tile(k_u, (slot, j), off, GR)) for j in range(NJ)],
                                axis=1) * SCALE
            e = jnp.exp(s - jnp.max(s, axis=-1, keepdims=True))
            p_s[g] = e * (1.0 / jnp.sum(e, axis=-1, keepdims=True))
            return c
        lax.fori_loop(0, NG, qk1, 0)

        def v_tile(j, off, nr, keep):
            vj = tile(v_u, (slot, j), off, nr)
            if keep:
                vf_s[pl.ds(off // 16, nr // 16), j] = vj.astype(F32).reshape(nr // 16, 16, 128)
            return vj

        def pv_tiles(pb, off, nr, js):
            o = None
            for j in js:
                t = _dot_nt(pb[:, j * 128:(j + 1) * 128], v_tile(j, off, nr, j < NJF))
                o = t if o is None else o + t
            return o

        def wo_pair(o, s, off, nr):
            o = jnp.where(shead[:, 0:nr] == 2 * (s % PG), o, 0.0).astype(BF16)
            return proj(o, wo_u, range(ND), off, nr)

        def pv1(s, y):
            for c in range(NVC - 4):
                @pl.when(s == V_CHUNKS[c][0] // SR)
                def _():
                    wait_v(c)
            off = pl.multiple_of(s * SR, SR)
            pb = p_s[s // PG].astype(BF16)
            return y + wo_pair(pv_tiles(pb, off, SR, range(NJ)), s, off, SR)
        y1 = lax.fori_loop(0, NS - 1, pv1, jnp.zeros((HG, D), F32))

        off = (NS - 1) * SR
        pb = p_s[NG - 1].astype(BF16)
        wait_v(NVC - 4)
        o = pv_tiles(pb, off, 256, range(0, 4))
        wait_v(NVC - 3)
        o = o + pv_tiles(pb, off, 256, range(4, NJ))

        off = H * DH - 128
        acc = None
        for c in (NVC - 2, NVC - 1):
            wait_v(c)
            for j in range(V_CHUNKS[c][2], V_CHUNKS[c][2] + V_CHUNKS[c][3]):
                pj = p_s[NG - 1, HG - 1:HG, j * 128:(j + 1) * 128]
                t = v_tile(j, off, 128, j < 4).astype(F32) * pj
                acc = t if acc is None else acc + t
        y1 = y1 + wo_pair(o, NS - 1, (NS - 1) * SR, 256)
        oc = jnp.sum(acc, axis=-1, keepdims=True)
        yv = [(tile(wo_u, (n,), off, 128).astype(F32) * oc).reshape(16, 8, 128).sum(axis=0)
              for n in range(ND)]
        y1 = y1 + jnp.concatenate(yv, axis=1)

        x0 = jnp.broadcast_to(x_s[pl.ds(b, 1), :], (HG, D))
        x1 = _round(x0 + jnp.sum(y1, axis=0, keepdims=True))
        true8 = (srow[:, 0:128] + b) >= 0
        x2 = moe(x1, true8, False)

        lhs2 = x2.astype(BF16)
        mean2, rstd2, _, part2 = _ln_stats(x2)
        q_t, s_t, p_g, pj_h, o_t, il_h, res, lhs_g, sum_t, yv_h = ({} for _ in range(10))
        y_tiles = [jnp.where(srow[:, 0:128] == 0, x2[:, n * 128:(n + 1) * 128], 0.0)
                   for n in range(ND)]
        x2l = after(true8, x2, part2)

        def job_a(job, t):
            res[job] = _dot(lhs2, tile(wq_u, (t,), 0, D))
            q_t[t] = ln_fix(res[job], mean2, rstd2, csq_s, t)

        def job_v(job, t, gate):
            i = VQ.index(t)
            xv = x2 if i < VG else x2l
            if gate is not None:
                xv = jnp.concatenate([x2[:, 0:D - 128], after(true8, x2[:, D - 128:], res[gate])],
                                     axis=1)
            q_t[t] = ln_fix(vpu_tile(xv, wqt_s, i), mean2, rstd2, csq_s, t)

        def job_b(job, g, j):
            if g not in lhs_g:
                q = jnp.concatenate([q_t[t] for t in range(g * GT, (g + 1) * GT)], axis=1)
                lhs_g[g] = jnp.where(diag[:, 0:GT * 128], q, 0.0).astype(BF16)
            res[job] = s_t[g, j] = _dot(lhs_g[g], tile(k_u, (slot, j), g * GT * 128, GT * 128))
            if j == NJ - 1:
                sc = jnp.concatenate([s_t[g, k] for k in range(NJ)], axis=1) * SCALE
                e = jnp.exp(sc - jnp.max(sc, axis=-1, keepdims=True))
                il = 1.0 / jnp.sum(e, axis=-1, keepdims=True)
                p_g[g] = (e, jnp.broadcast_to(il, (8, 128)))

        def job_e(job, g, t, c0, c1, gate):
            e, il = p_g[g]
            r0 = t * 8 + c0
            n = c1 - c0
            m = r0 * 16 // DH - g * GT * 128 // DH
            if (g, m) not in pj_h:
                pj_h[g, m] = [jnp.broadcast_to(e[m:m + 1, j * 128:(j + 1) * 128], (8, 128))
                              for j in range(NJ)]
                il_h[g, m] = jnp.broadcast_to(il[m:m + 1, :], (8, 128))
            pj = list(pj_h[g, m])
            if gate is not None:
                pj[NJ - 1] = after(true8, pj[NJ - 1], res[gate])
            nf = NJF if t < NT - 1 else 4
            if (g, m, nf) not in pj_h:
                pj_h[g, m, nf] = jnp.stack(pj[0:nf])[None, :, None]
            vf = vf_s[pl.ds(r0, n), pl.ds(0, nf)].reshape(n, nf, 2, 8, 128)
            acc = jnp.sum(vf * pj_h[g, m, nf], axis=1).reshape(2 * n, 8, 128)
            for j in range(nf, NJ):
                vj = tile(v_u, (slot, j), r0 * 16, n * 16).astype(F32)
                acc = acc + vj.reshape(2 * n, 8, 128) * pj[j][None]
            sums = jnp.sum(acc, axis=-1, keepdims=True)
            if t >= NT - FV:
                for k in range(ND):
                    w = tile(wo_u, (k,), r0 * 16, n * 16).astype(F32).reshape(2 * n, 8, 128)
                    yc = jnp.sum(w * sums, axis=0)
                    yv_h[g, m, k] = yc + yv_h[g, m, k] if (g, m, k) in yv_h else yc
                return
            sum_t.setdefault(t, []).append(jnp.broadcast_to(sums, (2 * n, 8, 128)))
            if c1 == 8:
                m0 = t * 128 // DH - g * GT * 128 // DH
                scale = il_h[g, m0]
                if t % 3 == 1:
                    scale = jnp.where(lane8 < 64, scale, il_h[g, m0 + 1])
                o_t[t] = spread(jnp.concatenate(sum_t[t], axis=0)) * scale

        def job_f(job, t0, t1, n):
            o = jnp.concatenate([o_t[t] for t in range(t0, t1)], axis=1).astype(BF16)
            y = _dot(o, tile(wo_u, (n,), t0 * 128, (t1 - t0) * 128))
            res[job] = y_tiles[n] = y + y_tiles[n]

        for job in _l2_schedule():
            {'a': job_a, 'v': job_v, 'b': job_b, 'e': job_e, 'f': job_f}[job[0]](job, *job[1:])

        for (g, m, n), yc in yv_h.items():
            y_tiles[n] = y_tiles[n] + yc * il_h[g, m]
        x3 = jnp.sum(jnp.concatenate(y_tiles, axis=1), axis=0, keepdims=True)
        x4 = moe(_round(jnp.broadcast_to(x3, (8, D))), true8, True)
        out_s[pl.ds(b, 1), :] = x4[0:1, :]
        return carry

    lax.fori_loop(0, B, batch_body, 0)
    o_ref[...] = out_s[0:B, :].astype(o_ref.dtype)


def _tile_view(t):
    *lead, r, c = t.shape
    n = len(lead)
    t = t.reshape(*lead, r // 16, 2, 8, c // 128, 128)
    return t.transpose(*range(n), n, n + 1, n + 3, n + 2, n + 4)


@jax.jit
def pallas_interleave_layers__sliding_block_cached__moe_arch_mod__decode_kernel(
    A_x: jax.Array,
    A_k_cache: jax.Array,
    A_v_cache: jax.Array,
    A_wq: jax.Array,
    A_wo: jax.Array,
    B_x: jax.Array,
    B_w_r: jax.Array,
    B_w_gate: jax.Array,
    B_w_up: jax.Array,
    B_w_down: jax.Array,
):
    x = A_x.reshape(B, D)
    kt = _tile_view(jnp.swapaxes(A_k_cache, 2, 3).reshape(B, H * DH, SK))
    vt = _tile_view(jnp.swapaxes(A_v_cache, 2, 3).reshape(B, H * DH, SK))

    out = pl.pallas_call(
        _kernel,
        in_specs=[pl.BlockSpec(memory_space=pl.ANY)] * 9,
        out_specs=pl.BlockSpec(memory_space=pltpu.VMEM),
        out_shape=jax.ShapeDtypeStruct((B, D), BF16),
        scratch_shapes=[
            pltpu.VMEM((B, D), BF16),
            pltpu.VMEM((D,), BF16),
            pltpu.VMEM((D // 16, NT + 1, 16, 128), BF16),
            pltpu.VMEM((H * DH // 16, ND, 16, 128), BF16),
            pltpu.VMEM((D // 16, NF + 1, 16, 128), BF16),
            pltpu.VMEM((D // 16, NF + 1, 16, 128), BF16),
            pltpu.VMEM((F // 16, ND, 16, 128), BF16),
            pltpu.VMEM((2, H * DH // 16, NJ + 1, 16, 128), BF16),
            pltpu.VMEM((2, H * DH // 16, NJ, 16, 128), BF16),
            pltpu.VMEM((8, D), F32),
            pltpu.VMEM((8, H * DH), F32),
            pltpu.VMEM((NG, HG, W), F32),
            pltpu.VMEM((8, D), F32),
            pltpu.VMEM((1, D), F32),
            pltpu.VMEM((8, H * DH), F32),
            pltpu.VMEM((8, F), F32),
            pltpu.VMEM((8, F), F32),
            pltpu.VMEM((KQ + KL, 128, D), F32),
            pltpu.VMEM((NF, 128, D), F32),
            pltpu.VMEM((NF, 128, D), F32),
            pltpu.VMEM((H * DH // 16, NJF, 16, 128), F32),
            pltpu.SemaphoreType.DMA((NSEM,)),
        ],
        compiler_params=pltpu.CompilerParams(
            vmem_limit_bytes=116 * 1024 * 1024,
            disable_bounds_checks=True,
            disable_semaphore_checks=True,
        ),
    )(x, kt, vt, _tile_view(A_wq), _tile_view(A_wo), B_w_r,
      _tile_view(B_w_gate), _tile_view(B_w_up), _tile_view(B_w_down))
    return out.reshape(B, 1, D)
```

```python
import jax
import jax.numpy as jnp
from jax import lax
import jax.experimental.pallas as pl
import jax.experimental.pallas.tpu as pltpu

B, D = 4, 640
H, DH, SK = 32, 192, 4096
W = 1024
F = 1536
NJ = W // 128
ND = D // 128
NF = F // 128
NT = H * DH // 128
HG = 8
NG = H // HG
GR = HG * DH
SR = 2 * DH
NS = H // 2
PG = HG // 2
JW0 = (SK - W) // 128
JW = 4
LN_EPS = 1e-5
SCALE = DH ** -0.5
F32 = jnp.float32
BF16 = jnp.bfloat16
U32 = jnp.uint32

V_CHUNKS = ([(g * GR, GR, 0, NJ) for g in range(NG - 1)]
            + [(s * SR, SR, 0, NJ) for s in range(NS - PG, NS - 1)]
            + [((NS - 1) * SR, 256, 0, 4), ((NS - 1) * SR, 256, 4, 4),
               (H * DH - 128, 128, 0, 4), (H * DH - 128, 128, 4, 4)])
NVC = len(V_CHUNKS)

SEM_X, SEM_WR, SEM_WQ, SEM_WO, SEM_WG, SEM_WU, SEM_WD = range(7)
SEM_K = 7
SEM_V = SEM_K + 2
NSEM = SEM_V + 2 * NVC

GT = 6
NG2 = NT // GT
KQ0, KQ, KL = 6, 19, 10
VQ = list(range(KQ0, KQ0 + KQ)) + list(range(NT - KL, NT))
NJF = 6
FV = 3
VG = 4
DK = 3


def _l2_schedule():
    t_e, t_v = 83 / 8, 45
    t_x, t_soft, t_pop, lead = 150, 270, 130, 225
    a_jobs = [[('a', t) for t in range(g * GT, (g + 1) * GT) if t not in VQ] for g in range(NG2)]
    mx = list(a_jobs[0])
    nxt = [g for g in range(1, NG2) if a_jobs[g]]
    for g in range(NG2):
        if nxt and (g == 0 or nxt[0] <= g + 1):
            mx += a_jobs[nxt.pop(0)]
        mx += [('b', g, j) for j in range(NJ)]
    es = [(t // GT, t, c) for t in range(NT) for c in range(8)]
    for i, t in enumerate(range(NT - KL, NT)):
        es.insert(9 + i * 14, (es[9 + i * 14][0], t, 'v'))
    cuts = list(range(0, NT - FV, 2)) + [NT - FV]
    fs = [('f', c0, c1, n) for c0, c1 in zip(cuts[:-1], cuts[1:]) for n in range(ND)]
    order, now, vpu = [('v', t, None) for t in range(KQ0, KQ0 + KQ)], 0, KQ * t_v
    b_end, avail, o_at = {}, [], {}

    def start(e):
        return max(vpu, b_end[e[0]] + t_soft)

    def cost(job):
        return 40 if job[0] == 'a' else 8 * GT if job[0] == 'b' else 8 * (job[2] - job[1])

    def urgent(extra):
        t = now + extra
        for job in mx:
            t += cost(job)
            if job[0] == 'b' and job[2] == NJ - 1:
                n_before = sum(1 for e in es if e[0] < job[1])
                if t + t_soft + lead > vpu + n_before * t_e:
                    return True
        return False

    while mx or es or fs:
        while es and es[0][0] in b_end and (
                start(es[0]) <= now + t_pop or not (mx or (fs and fs[0][2] - 1 in o_at))):
            e = es.pop(0)
            st = start(e)
            gate = None
            if vpu > b_end[e[0]] + t_soft:
                gate = [j for (tt, j) in avail if tt <= st][-1]
            if e[2] == 'v':
                order.append(('v', e[1], gate))
                vpu = st + t_v
                continue
            prev = order[-1]
            if (prev[0] == 'e' and prev[2] == e[1] and prev[5] == gate
                    and not (e[1] % 3 == 1 and e[2] == 4)):
                order[-1] = prev[:4] + (e[2] + 1, gate)
            else:
                order.append(('e', e[0], e[1], e[2], e[2] + 1, gate))
            vpu = st + t_e
            if e[2] == 7:
                o_at[e[1]] = vpu + t_x
        if not (mx or fs):
            continue
        f_ready = fs and o_at.get(fs[0][2] - 1, 1 << 30) <= now
        if mx and not (f_ready and not urgent(cost(fs[0]))):
            job = mx.pop(0)
            now += cost(job)
            if job[0] == 'b' and job[2] == NJ - 1:
                b_end[job[1]] = now
        else:
            job = fs.pop(0)
            now = max(now, o_at[job[2] - 1]) + cost(job)
        order.append(job)
        avail.append((now + t_pop, job))
    return order


def _dot(a, b):
    return jnp.dot(a, b, preferred_element_type=F32)


def _dot_nt(a, b):
    return lax.dot_general(a, b, (((1,), (1,)), ((), ())), preferred_element_type=F32)


def _round(x):
    return x.astype(BF16).astype(F32)


def _ln_stats(x):
    m = jnp.mean(x, axis=-1, keepdims=True)
    c = x - m
    c2 = c * c
    part = c2[:, 0:128]
    for kt in range(1, ND):
        part = part + c2[:, kt * 128:(kt + 1) * 128]
    v = jnp.sum(part, axis=-1, keepdims=True) * (1.0 / D)
    m = _round(m)
    r = lax.rsqrt(v + LN_EPS)
    return m, r, (x - m) * r, part


def _kernel(x_hbm, k_hbm, v_hbm, wq_hbm, wo_hbm, wr_hbm, wg_hbm, wu_hbm, wd_hbm,
            o_ref,
            x_in, wr_in, wq_s, wo_s, wg_s, wu_s, wd_s, kbuf, vbuf,
            x_s, q1_s, p_s, out_s, wr_s, csq_s, csg_s, csu_s, wqt_s, wut_s, wgt_s, vf_s,
            sems):
    def row_copies(src, dst, sem, r0, nr, j_src, j0, nj, jw):
        rows = pl.ds(r0 // 16, nr // 16)
        return [pltpu.make_async_copy(src.at[rows, half, pl.ds(j_src + j, jw)],
                                      dst.at[rows, pl.ds(j, jw), pl.ds(half * 8, 8)],
                                      sems.at[sem])
                for half in range(2) for j in range(j0, j0 + nj, jw)]

    def w_copies(src, dst, sem, nr):
        return [c for r0 in range(0, dst.shape[0] * 16, nr)
                for c in row_copies(src, dst, sem, r0, nr, 0, 0, src.shape[2], src.shape[2])]

    def k_copies(b, slot):
        return [c for g in range(NG) for c in row_copies(
            k_hbm.at[b], kbuf.at[slot], SEM_K + slot, g * GR, GR, JW0, 0, NJ, JW)]

    def v_copies(b, slot, c):
        r0, nr, j0, nj = V_CHUNKS[c]
        return row_copies(v_hbm.at[b], vbuf.at[slot], SEM_V + slot * NVC + c,
                          r0, nr, JW0, j0, nj, JW)

    def start(copies):
        for c in copies:
            c.start()

    def wait(copies):
        for c in copies:
            c.wait()

    x_cp = pltpu.make_async_copy(x_hbm, x_in, sems.at[SEM_X])
    wr_cp = pltpu.make_async_copy(wr_hbm, wr_in, sems.at[SEM_WR])
    wq_cp = w_copies(wq_hbm, wq_s, SEM_WQ, D)
    wo_cp = w_copies(wo_hbm, wo_s, SEM_WO, 384)
    wg_cp = w_copies(wg_hbm, wg_s, SEM_WG, D)
    wu_cp = w_copies(wu_hbm, wu_s, SEM_WU, D)
    wd_cp = w_copies(wd_hbm, wd_s, SEM_WD, 384)
    start(wq_cp + [x_cp, wr_cp] + wo_cp + wg_cp + wu_cp + wd_cp + k_copies(0, 0))
    for c in range(NVC):
        start(v_copies(0, 0, c))

    def tile(ref, idx, start, size):
        view = ref.at[idx[:-1] + (pl.ds(start // 16, size // 16), idx[-1])]
        return pltpu.bitcast(view.bitcast(U32)[...].reshape(size // 2, 128), BF16)

    def proj(a, w_s, tiles, start, size):
        return jnp.concatenate([_dot(a, tile(w_s, (j,), start, size)) for j in tiles], axis=1)

    def ln_fix(z, mean, rstd, cs_s, t):
        return (z - mean * cs_s[:, t * 128:(t + 1) * 128]) * rstd

    lane8 = lax.broadcasted_iota(jnp.int32, (8, 128), 1)
    sub8 = lax.broadcasted_iota(jnp.int32, (8, 128), 0)

    bits = [((lane8 & bit) != 0)[None] for bit in (8, 16, 32, 64)]
    on_diag = (lane8 & 7) == sub8

    def spread(sums):
        v = jnp.broadcast_to(sums, (16, 8, 128))
        for hi in bits:
            v = v.reshape(v.shape[0] // 2, 2, 8, 128)
            v = jnp.where(hi, v[:, 1], v[:, 0])
        return jnp.where(on_diag, v[0], 0.0)

    def after(true8, x, dep):
        return jnp.concatenate([jnp.where(true8, x[:, k:k + 128], dep)
                                for k in range(0, x.shape[1], 128)], axis=1)

    def vpu_tile(x, wt_s, i):
        sums = jnp.sum(wt_s[i].reshape(16, 8, D) * x[None], axis=-1, keepdims=True)
        return jnp.broadcast_to(jnp.sum(spread(sums), axis=0, keepdims=True), (8, 128))

    def transpose_tiles(w_s, wt_s, t0, n, i0=0):
        def body(i, c):
            for kt in range(ND):
                wt_s[i0 + i, :, kt * 128:(kt + 1) * 128] = (
                    tile(w_s, (t0 + i,), kt * 128, 128).astype(F32).T)
            return c
        lax.fori_loop(0, n, body, 0)

    row = lax.broadcasted_iota(jnp.int32, (HG, GR), 0)
    col = lax.broadcasted_iota(jnp.int32, (HG, GR), 1)
    diag = (col >= row * DH) & (col < (row + 1) * DH)

    def moe(x, true8, swap):
        xb = x.astype(BF16)
        mean, rstd, xn, part = _ln_stats(x)
        r = jnp.sum(xn * wr_s[...], axis=-1, keepdims=True)
        xl = after(true8, x, part)
        wvt, wm = (wgt_s, wu_s) if swap else (wut_s, wg_s)
        u = [vpu_tile(x if i < VG else xl, wvt, i) for i in range(NF)]
        g = [_dot(xb, tile(wm, (t,), 0, D)) for t in range(NF)]
        if swap:
            g, u = u, g
        h = []
        for t in range(NF):
            gt = ln_fix(g[t], mean, rstd, csg_s, t)
            h.append(gt * jax.nn.sigmoid(gt) * ln_fix(u[t], mean, rstd, csu_s, t))
        y = None
        for t0 in range(0, NF, DK):
            hb = jnp.concatenate(h[t0:t0 + DK], axis=1).astype(BF16)
            yt = proj(hb, wd_s, range(ND), t0 * 128, DK * 128)
            y = yt if y is None else yt + y
        return _round(x + (xn + y * jax.nn.sigmoid(r)))

    x_cp.wait()
    wr_cp.wait()
    wr_s[...] = wr_in[...].astype(F32).reshape(1, D)
    x_s[...] = jnp.zeros_like(x_s)
    x_s[0:B, :] = x_in[...].astype(F32)
    out_s[...] = jnp.zeros_like(out_s)
    xn0 = _ln_stats(x_s[...])[2]
    ones = jnp.ones((8, D), F32)
    wait(wq_cp)
    z = proj(jnp.concatenate([xn0, ones], axis=0).astype(BF16), wq_s, range(NT), 0, D)
    q1_s[...] = z[0:8]
    csq_s[...] = z[8:16]
    transpose_tiles(wq_s, wqt_s, KQ0, KQ)
    transpose_tiles(wq_s, wqt_s, NT - KL, KL, KQ)
    wait(wo_cp)
    wait(wg_cp)
    wait(wu_cp)
    csg_s[...] = proj(ones.astype(BF16), wg_s, range(NF), 0, D)
    csu_s[...] = proj(ones.astype(BF16), wu_s, range(NF), 0, D)
    transpose_tiles(wu_s, wut_s, 0, NF)
    transpose_tiles(wg_s, wgt_s, 0, NF)
    wait(wd_cp)

    srow = lax.broadcasted_iota(jnp.int32, (HG, SR), 0)
    scol = lax.broadcasted_iota(jnp.int32, (HG, SR), 1)
    shead = srow - (scol >= DH).astype(jnp.int32)

    def batch_body(b, carry):
        slot = b % 2
        more = b + 1 < B

        def wait_v(c):
            wait(v_copies(b, slot, c))

            if c < NVC - 1:
                @pl.when(more)
                def _():
                    start(v_copies(b + 1, 1 - slot, c))
                    if c == NVC - 2:
                        start(v_copies(b + 1, 1 - slot, c + 1))

        wait(k_copies(b, slot))

        @pl.when(more)
        def _():
            start(k_copies(b + 1, 1 - slot))

        def qk1(g, c):
            off = pl.multiple_of(g * GR, GR)
            qg = jnp.broadcast_to(q1_s[pl.ds(b, 1), pl.ds(off, GR)], (HG, GR))
            lhs = jnp.where(diag, qg, 0.0).astype(BF16)
            s = jnp.concatenate([_dot(lhs, tile(kbuf, (slot, j), off, GR)) for j in range(NJ)],
                                axis=1) * SCALE
            e = jnp.exp(s - jnp.max(s, axis=-1, keepdims=True))
            p_s[g] = e * (1.0 / jnp.sum(e, axis=-1, keepdims=True))
            return c
        lax.fori_loop(0, NG, qk1, 0)

        def v_tile(j, off, nr, keep):
            vj = tile(vbuf, (slot, j), off, nr)
            if keep:
                vf_s[pl.ds(off // 16, nr // 16), j] = vj.astype(F32).reshape(nr // 16, 16, 128)
            return vj

        def pv_tiles(pb, off, nr, js):
            o = None
            for j in js:
                t = _dot_nt(pb[:, j * 128:(j + 1) * 128], v_tile(j, off, nr, j < NJF))
                o = t if o is None else o + t
            return o

        def wo_pair(o, s, off, nr):
            o = jnp.where(shead[:, 0:nr] == 2 * (s % PG), o, 0.0).astype(BF16)
            return proj(o, wo_s, range(ND), off, nr)

        def pv1(s, y):
            for c in range(NVC - 4):
                @pl.when(s == V_CHUNKS[c][0] // SR)
                def _():
                    wait_v(c)
            off = pl.multiple_of(s * SR, SR)
            pb = p_s[s // PG].astype(BF16)
            return y + wo_pair(pv_tiles(pb, off, SR, range(NJ)), s, off, SR)
        y1 = lax.fori_loop(0, NS - 1, pv1, jnp.zeros((HG, D), F32))

        off = (NS - 1) * SR
        pb = p_s[NG - 1].astype(BF16)
        wait_v(NVC - 4)
        o = pv_tiles(pb, off, 256, range(0, 4))
        wait_v(NVC - 3)
        o = o + pv_tiles(pb, off, 256, range(4, NJ))

        off = H * DH - 128
        acc = None
        for c in (NVC - 2, NVC - 1):
            wait_v(c)
            for j in range(V_CHUNKS[c][2], V_CHUNKS[c][2] + V_CHUNKS[c][3]):
                pj = p_s[NG - 1, HG - 1:HG, j * 128:(j + 1) * 128]
                t = v_tile(j, off, 128, j < 4).astype(F32) * pj
                acc = t if acc is None else acc + t
        y1 = y1 + wo_pair(o, NS - 1, (NS - 1) * SR, 256)
        oc = jnp.sum(acc, axis=-1, keepdims=True)
        yv = [(tile(wo_s, (n,), off, 128).astype(F32) * oc).reshape(16, 8, 128).sum(axis=0)
              for n in range(ND)]
        y1 = y1 + jnp.concatenate(yv, axis=1)

        x0 = jnp.broadcast_to(x_s[pl.ds(b, 1), :], (HG, D))
        x1 = _round(x0 + jnp.sum(y1, axis=0, keepdims=True))
        true8 = (srow[:, 0:128] + b) >= 0
        x2 = moe(x1, true8, False)

        lhs2 = x2.astype(BF16)
        mean2, rstd2, _, part2 = _ln_stats(x2)
        q_t, s_t, p_g, pj_h, o_t, il_h, res, lhs_g, sum_t, yv_h = ({} for _ in range(10))
        y_tiles = [jnp.where(srow[:, 0:128] == 0, x2[:, n * 128:(n + 1) * 128], 0.0)
                   for n in range(ND)]
        x2l = after(true8, x2, part2)

        def job_a(job, t):
            res[job] = _dot(lhs2, tile(wq_s, (t,), 0, D))
            q_t[t] = ln_fix(res[job], mean2, rstd2, csq_s, t)

        def job_v(job, t, gate):
            i = VQ.index(t)
            xv = x2 if i < VG else x2l
            if gate is not None:
                xv = jnp.concatenate([x2[:, 0:D - 128], after(true8, x2[:, D - 128:], res[gate])],
                                     axis=1)
            q_t[t] = ln_fix(vpu_tile(xv, wqt_s, i), mean2, rstd2, csq_s, t)

        def job_b(job, g, j):
            if g not in lhs_g:
                q = jnp.concatenate([q_t[t] for t in range(g * GT, (g + 1) * GT)], axis=1)
                lhs_g[g] = jnp.where(diag[:, 0:GT * 128], q, 0.0).astype(BF16)
            res[job] = s_t[g, j] = _dot(lhs_g[g], tile(kbuf, (slot, j), g * GT * 128, GT * 128))
            if j == NJ - 1:
                sc = jnp.concatenate([s_t[g, k] for k in range(NJ)], axis=1) * SCALE
                e = jnp.exp(sc - jnp.max(sc, axis=-1, keepdims=True))
                il = 1.0 / jnp.sum(e, axis=-1, keepdims=True)
                p_g[g] = (e, jnp.broadcast_to(il, (8, 128)))

        def job_e(job, g, t, c0, c1, gate):
            e, il = p_g[g]
            r0 = t * 8 + c0
            n = c1 - c0
            m = r0 * 16 // DH - g * GT * 128 // DH
            if (g, m) not in pj_h:
                pj_h[g, m] = [jnp.broadcast_to(e[m:m + 1, j * 128:(j + 1) * 128], (8, 128))
                              for j in range(NJ)]
                il_h[g, m] = jnp.broadcast_to(il[m:m + 1, :], (8, 128))
            pj = list(pj_h[g, m])
            if gate is not None:
                pj[NJ - 1] = after(true8, pj[NJ - 1], res[gate])
            nf = NJF if t < NT - 1 else 4
            if (g, m, nf) not in pj_h:
                pj_h[g, m, nf] = jnp.stack(pj[0:nf])[None, :, None]
            vf = vf_s[pl.ds(r0, n), pl.ds(0, nf)].reshape(n, nf, 2, 8, 128)
            acc = jnp.sum(vf * pj_h[g, m, nf], axis=1).reshape(2 * n, 8, 128)
            for j in range(nf, NJ):
                vj = tile(vbuf, (slot, j), r0 * 16, n * 16).astype(F32)
                acc = acc + vj.reshape(2 * n, 8, 128) * pj[j][None]
            sums = jnp.sum(acc, axis=-1, keepdims=True)
            if t >= NT - FV:
                for k in range(ND):
                    w = tile(wo_s, (k,), r0 * 16, n * 16).astype(F32).reshape(2 * n, 8, 128)
                    yc = jnp.sum(w * sums, axis=0)
                    yv_h[g, m, k] = yc + yv_h[g, m, k] if (g, m, k) in yv_h else yc
                return
            sum_t.setdefault(t, []).append(jnp.broadcast_to(sums, (2 * n, 8, 128)))
            if c1 == 8:
                m0 = t * 128 // DH - g * GT * 128 // DH
                scale = il_h[g, m0]
                if t % 3 == 1:
                    scale = jnp.where(lane8 < 64, scale, il_h[g, m0 + 1])
                o_t[t] = spread(jnp.concatenate(sum_t[t], axis=0)) * scale

        def job_f(job, t0, t1, n):
            o = jnp.concatenate([o_t[t] for t in range(t0, t1)], axis=1).astype(BF16)
            y = _dot(o, tile(wo_s, (n,), t0 * 128, (t1 - t0) * 128))
            res[job] = y_tiles[n] = y + y_tiles[n]

        for job in _l2_schedule():
            {'a': job_a, 'v': job_v, 'b': job_b, 'e': job_e, 'f': job_f}[job[0]](job, *job[1:])

        for (g, m, n), yc in yv_h.items():
            y_tiles[n] = y_tiles[n] + yc * il_h[g, m]
        x3 = jnp.sum(jnp.concatenate(y_tiles, axis=1), axis=0, keepdims=True)
        x4 = moe(_round(jnp.broadcast_to(x3, (8, D))), true8, True)
        out_s[pl.ds(b, 1), :] = x4[0:1, :]
        return carry

    lax.fori_loop(0, B, batch_body, 0)
    o_ref[...] = out_s[0:B, :].astype(o_ref.dtype)


def _tile_view(t):
    *lead, r, c = t.shape
    n = len(lead)
    t = t.reshape(*lead, r // 16, 2, 8, c // 128, 128)
    return t.transpose(*range(n), n, n + 1, n + 3, n + 2, n + 4)


@jax.jit
def pallas_interleave_layers__sliding_block_cached__moe_arch_mod__decode_kernel(
    A_x: jax.Array,
    A_k_cache: jax.Array,
    A_v_cache: jax.Array,
    A_wq: jax.Array,
    A_wo: jax.Array,
    B_x: jax.Array,
    B_w_r: jax.Array,
    B_w_gate: jax.Array,
    B_w_up: jax.Array,
    B_w_down: jax.Array,
):
    x = A_x.reshape(B, D)
    kt = _tile_view(jnp.swapaxes(A_k_cache, 2, 3).reshape(B, H * DH, SK))
    vt = _tile_view(jnp.swapaxes(A_v_cache, 2, 3).reshape(B, H * DH, SK))

    out = pl.pallas_call(
        _kernel,
        in_specs=[pl.BlockSpec(memory_space=pl.ANY)] * 9,
        out_specs=pl.BlockSpec(memory_space=pltpu.VMEM),
        out_shape=jax.ShapeDtypeStruct((B, D), BF16),
        scratch_shapes=[
            pltpu.VMEM((B, D), BF16),
            pltpu.VMEM((D,), BF16),
            pltpu.VMEM((D // 16, NT + 1, 16, 128), BF16),
            pltpu.VMEM((H * DH // 16, ND, 16, 128), BF16),
            pltpu.VMEM((D // 16, NF + 1, 16, 128), BF16),
            pltpu.VMEM((D // 16, NF + 1, 16, 128), BF16),
            pltpu.VMEM((F // 16, ND, 16, 128), BF16),
            pltpu.VMEM((2, H * DH // 16, NJ + 1, 16, 128), BF16),
            pltpu.VMEM((2, H * DH // 16, NJ, 16, 128), BF16),
            pltpu.VMEM((8, D), F32),
            pltpu.VMEM((8, H * DH), F32),
            pltpu.VMEM((NG, HG, W), F32),
            pltpu.VMEM((8, D), F32),
            pltpu.VMEM((1, D), F32),
            pltpu.VMEM((8, H * DH), F32),
            pltpu.VMEM((8, F), F32),
            pltpu.VMEM((8, F), F32),
            pltpu.VMEM((KQ + KL, 128, D), F32),
            pltpu.VMEM((NF, 128, D), F32),
            pltpu.VMEM((NF, 128, D), F32),
            pltpu.VMEM((H * DH // 16, NJF, 16, 128), F32),
            pltpu.SemaphoreType.DMA((NSEM,)),
        ],
        compiler_params=pltpu.CompilerParams(
            vmem_limit_bytes=116 * 1024 * 1024,
            disable_bounds_checks=True,
            disable_semaphore_checks=True,
        ),
    )(x, kt, vt, _tile_view(A_wq), _tile_view(A_wo), B_w_r,
      _tile_view(B_w_gate), _tile_view(B_w_up), _tile_view(B_w_down))
    return out.reshape(B, 1, D)
```
